```python
import jax
import jax.numpy as jnp

def _softmax(x, axis=-1):
    return jax.nn.softmax(x, axis=axis)

def _gelu(x):
    return jax.nn.gelu(x, approximate=True)

def _silu(x):
    return jax.nn.silu(x)

def _sigmoid(x):
    return jax.nn.sigmoid(x)

def _layernorm(x, axis=-1, eps=1e-05):
    m = jnp.mean(x, axis=axis, keepdims=True)
    v = jnp.var(x, axis=axis, keepdims=True)
    return (x - m) / jnp.sqrt(v + eps)

def _scatter_add(tgt, idx, src, axis=0):
    return tgt.at[idx].add(src)

def _segment_sum(src, seg, n):
    return jax.ops.segment_sum(src, seg, n)

class _Rng:

    def __init__(self, key):
        self._k = key

    def _next(self):
        self._k, sub = jax.random.split(self._k)
        return sub

    def normal(self, shape):
        return jax.random.normal(self._next(), shape, dtype=jnp.bfloat16)

    def randint(self, lo, hi, shape):
        return jax.random.randint(self._next(), shape, lo, hi, dtype=jnp.int32)

    def uniform(self, shape, lo=0.0, hi=1.0):
        return jax.random.uniform(self._next(), shape, jnp.bfloat16, lo, hi)

    def permutation(self, n):
        return jax.random.permutation(self._next(), n)
kernel_name = 'sequential_preLN__memory_aug_recurrent_mem_tr__mixer_s_mlp__prompt'

def setup_inputs():
    _rng = _Rng(jax.random.key(int.from_bytes(__import__("os").urandom(4), "little")))
    _w = lambda a: (lambda t: t.astype(jnp.bfloat16) if jnp.issubdtype(t.dtype, jnp.floating) else t)(jnp.asarray(a))

    def _A_setup():
        B, S, Dm = (1, 2048, 1024)
        H, Dh = (32, 128)
        M, seg = (8, 32)
        seg = min(seg, S)
        S = S // seg * seg
        return {'x': _w((lambda *s: _rng.normal(s) * 0.05)(B, S, Dm)), 'mem0': _w((lambda *s: _rng.normal(s) * 0.05)(B, M, Dm)), 'Wq': _w((lambda *s: _rng.normal(s) * 0.05)(Dm, H, Dh) * Dm ** (-0.5)), 'Wk': _w((lambda *s: _rng.normal(s) * 0.05)(Dm, H, Dh) * Dm ** (-0.5)), 'Wv': _w((lambda *s: _rng.normal(s) * 0.05)(Dm, H, Dh) * Dm ** (-0.5)), 'Wo': _w((lambda *s: _rng.normal(s) * 0.05)(H, Dh, Dm) * (H * Dh) ** (-0.5)), 'seg_len': seg}
    _A_in = _A_setup()

    def _B_setup():
        B, S, D, F = (1, 2048, 1024, 3584)
        return {'x': _w((lambda *s: _rng.normal(s) * 0.05)(B, S, D)), 'w1': _w((lambda *s: _rng.normal(s) * 0.05)(D, D) * D ** (-0.5)), 'w2': _w((lambda *s: _rng.normal(s) * 0.05)(D, D) * D ** (-0.5)), 'w3': _w((lambda *s: _rng.normal(s) * 0.05)(D, F) * D ** (-0.5)), 'w4': _w((lambda *s: _rng.normal(s) * 0.05)(F, D) * F ** (-0.5))}
    _B_in = _B_setup()
    return {'A_x': _A_in['x'], 'A_mem0': _A_in['mem0'], 'A_Wq': _A_in['Wq'], 'A_Wk': _A_in['Wk'], 'A_Wv': _A_in['Wv'], 'A_Wo': _A_in['Wo'], 'A_seg_len': _A_in['seg_len'], 'B_x': _B_in['x'], 'B_w1': _B_in['w1'], 'B_w2': _B_in['w2'], 'B_w3': _B_in['w3'], 'B_w4': _B_in['w4']}

def reference(A_x, A_mem0, A_Wq, A_Wk, A_Wv, A_Wo, A_seg_len, B_x, B_w1, B_w2, B_w3, B_w4):

    def _A_ref(x, mem0, Wq, Wk, Wv, Wo, seg_len):
        B, S, Dm = x.shape
        H, Dh = (Wq.shape[1], Wq.shape[2])
        M = mem0.shape[1]
        scale = Dh ** (-0.5)
        n_seg = S // seg_len
        L = M + seg_len
        idx = jnp.arange(L)
        mask = (idx[:, None] < M) | (idx[:, None] >= idx[None, :])
        mem = mem0
        outs = []
        for s in range(n_seg):
            xs = x[:, s * seg_len:(s + 1) * seg_len, :].copy()
            h = jnp.concatenate([mem, xs], axis=1)
            q = jnp.einsum('btd,dhe->bhte', h, Wq)
            k = jnp.einsum('btd,dhe->bhte', h, Wk)
            v = jnp.einsum('btd,dhe->bhte', h, Wv)
            scores = jnp.einsum('bhqe,bhke->bhqk', q, k) * scale
            scores = jnp.where(mask[None, None], scores, -1000000000.0)
            p = _softmax(scores, axis=-1)
            o = jnp.einsum('bhqk,bhke->bhqe', p, v)
            o = jnp.einsum('bhte,hed->btd', o, Wo)
            mem = o[:, :M, :].copy()
            outs.append(o[:, M:, :])
        return jnp.concatenate(outs, axis=1)

    def _B_ref(x, w1, w2, w3, w4):
        B, S, D = x.shape
        h = _gelu(_layernorm(x, axis=-1) @ w1)
        c = D // 4
        g0 = jnp.pad(h[:, :, 0 * c:1 * c], ((0, 0), (1, 0), (0, 0)))[:, :S, :]
        g1 = jnp.pad(h[:, :, 1 * c:2 * c], ((0, 0), (0, 1), (0, 0)))[:, 1:, :]
        g2 = jnp.pad(h[:, :, 2 * c:3 * c], ((0, 0), (2, 0), (0, 0)))[:, :S, :]
        g3 = jnp.pad(h[:, :, 3 * c:], ((0, 0), (0, 2), (0, 0)))[:, 2:, :]
        hs = jnp.concatenate([g0, g1, g2, g3], axis=-1) @ w2
        x1 = x + hs
        h2 = _gelu(_layernorm(x1, axis=-1) @ w3) @ w4
        return x1 + h2
    x = A_x
    h = x + _A_ref(_layernorm(x, axis=-1), A_mem0, A_Wq, A_Wk, A_Wv, A_Wo, A_seg_len)
    h2 = h + _B_ref(_layernorm(h, axis=-1), B_w1, B_w2, B_w3, B_w4)
    return h2
```

```python
import functools

import jax
import jax.numpy as jnp
from jax import lax
import jax.experimental.pallas as pl
import jax.experimental.pallas.tpu as pltpu

S = 2048
D = 1024
H = 32
DH = 128
MEM = 8
SEG = 32
F = 3584
NSEG = S // SEG
L = MEM + SEG
HS = SEG // 2
NP = H // 2
HD = D // 2
PAD = 2 * SEG
C4 = D // 4
HALO = 8
R = 64
RB = 4 * R
NB = S // RB
FC = 512
NC = F // FC
EPS = 1e-5
NEG = -1000000000.0

LAG_QK = 2
LAG_PV = 4
LAG_WO = 6
FILL_AT = 18
FILL_N = 2
WAIT_AT = 1
SKIP = 0

GROUPS = ((1, 3), (2, 4), (5, 6))
TARGETS = (((0, 1), (3, 1)), ((2, 1), (3, -1)), ((1, 1), (3, 1)), ((0, 1), (2, 1)),
           ((0, -1), (1, 1)), ((3, 1),), ((0, 1),))

bf16 = jnp.bfloat16
f32 = jnp.float32
u32 = jnp.uint32

SEM_X, SEM_W, SEM_WO, SEM_B, SEM_OUT = 0, 4, 16, 20, 24
NSEM = SEM_OUT + NB


def _mult(i, n):
    return i if isinstance(i, int) else pl.multiple_of(i, n)


def _ln(x):
    m = jnp.mean(x, axis=-1, keepdims=True)
    d = x - m
    v = jnp.mean(d * d, axis=-1, keepdims=True)
    return d * lax.rsqrt(v + EPS)


def _gelu(x):
    return jax.nn.gelu(x, approximate=True)


def _pack(x):
    return pltpu.bitcast(x.astype(bf16), u32)


def _unpack(x):
    return pltpu.bitcast(x, bf16)


def _dot(a, b):
    return jnp.dot(a, b, preferred_element_type=f32)


def _rows(*xs):
    return jnp.concatenate(xs, axis=0)


def _lhs(p, a):
    return (lambda: a(0) + a(3), lambda: a(2) + a(3), lambda: a(0), lambda: a(3),
            lambda: a(0) + a(1), lambda: a(2) - a(0), lambda: a(1) - a(3))[p]()


def _rhs(p, b):
    return (lambda: b(0) + b(3), lambda: b(0), lambda: b(1) - b(3), lambda: b(2) - b(0),
            lambda: b(3), lambda: b(0) + b(1), lambda: b(2) + b(3))[p]()


def _res(q, m):
    return (lambda: m(0) + m(3) - m(4) + m(6), lambda: m(2) + m(4),
            lambda: m(1) + m(3), lambda: m(0) - m(1) + m(2) + m(5))[q]()


def _pos(q, j):
    return 2 * (q >> 1) + (j >> 1), 2 * (q & 1) + (j & 1)


def _twice(side, blk):
    for p1 in range(7):
        outer = [side(p1, lambda q: blk[_pos(q, j)]) for j in range(4)]
        for p0 in range(7):
            yield 7 * p1 + p0, side(p0, outer.__getitem__)


def _row_lhs(p, a1, a2):
    return a1 + a2 if p in (1, 4) else a1 if p in (2, 5) else a2


def _row_res(t):
    if 0 not in t:
        return t[2] - t[1], t[1]
    if 1 not in t:
        return t[0], t[2] - t[0]
    return t[0], t[1]


def _interleave(*lists):
    order = sorted(((i + 0.5) / len(l), n, i)
                   for n, l in enumerate(lists) for i in range(len(l)))
    for _, n, i in order:
        lists[n][i]()


def _tasks(fn, *ranges):
    if len(ranges) == 2:
        return [functools.partial(fn, i, j) for i in ranges[0] for j in ranges[1]]
    return [functools.partial(fn, i) for i in ranges[0]]


def _scores(q, k):
    return lax.dot_general(q, k, (((1,), (1,)), ((), ())), preferred_element_type=f32)


def _attend(sc, v):
    ri = lax.broadcasted_iota(jnp.int32, (L, L), 0)
    ci = lax.broadcasted_iota(jnp.int32, (L, L), 1)
    sc = jnp.where((ri < MEM) | (ri >= ci), sc * (DH ** -0.5), NEG)
    mx = jnp.max(sc, axis=1, keepdims=True)
    e = jnp.exp(sc - mx)
    den = jnp.sum(e, axis=1, keepdims=True)
    inv = pl.reciprocal(den, approx=True)
    inv = inv * (2.0 - den * inv)
    return _dot(e, v) * inv


def _kernel(x_hbm, mem0_ref, wq_hbm, wk_hbm, wv_hbm, wo_hbm, w1_hbm, w2_hbm,
            w3_hbm, w4_hbm, out_hbm, hbuf, xg, wo_t, o1, ocar, w1b, w2b, w3b, sems):
    w_hbm = (wq_hbm, wk_hbm, wv_hbm)

    def b_copy(i, dst):
        src = (w1_hbm, w2_hbm, w3_hbm, w4_hbm)[i]
        return pltpu.make_async_copy(src.bitcast(u32), dst, sems.at[SEM_B + i])

    def seg_quads(s):
        r0 = HALO + s * SEG
        return [jnp.concatenate(
            [xg[2 * (q & 1) + c, pl.ds(_mult(r0 + (q >> 1) * HS, 8), HS), :]
             for c in range(2)], axis=1) for q in range(4)]

    def heads_of(c_mem, m):
        return [_rows(c_mem[n], _res(n, m.__getitem__), _res(2 + n, m.__getitem__))
                for n in range(2)]

    def wo_pass(phase, a, o, prev, o1_slot):
        whole, part = GROUPS[(phase + 1) % 3], GROUPS[(phase + 2) % 3]
        quad = lambda q: o[q & 1][MEM + (q >> 1) * HS:MEM + (q >> 1) * HS + HS]
        x = [_lhs(p, quad) for p in range(7)]
        o1[o1_slot, a] = x[0].astype(bf16)
        ocar[a] = _rows(*[x[p] for p in GROUPS[phase]], *[x[p][8:] for p in part])
        res = {}
        for k in range(2):
            for p, riders in ((whole[k], (prev[SEG + 8 * k:SEG + 8 * k + 8], x[whole[k]])),
                              (part[k], (x[part[k]][:8], prev[HS * k:HS * k + HS]))):
                lhs = _rows(_row_lhs(p, o[0][:MEM], o[1][:MEM]), *riders)
                res[p] = _dot(lhs.astype(bf16), _unpack(wo_t[p, a]))
        return res

    def add_h(s, terms):
        for q in range(4):
            for z in range(2):
                mine = [(sign, v) for p, zz, v in terms if zz == z
                        for qq, sign in TARGETS[p] if qq == q]
                if mine:
                    at = (pl.ds(_mult(PAD + s * SEG + (q >> 1) * HS + 8 * z, 8), 8),
                          pl.ds((q & 1) * HD, HD))
                    acc = hbuf[at]
                    for sign, v in mine:
                        acc = acc + v if sign > 0 else acc - v
                    hbuf[at] = acc

    def wo_finish(phase, s, tot, first=False):
        gw, gp = (phase + 1) % 3, (phase + 2) % 3
        whole, part = GROUPS[gw], GROUPS[gp]
        mem = _row_res({g: tot[GROUPS[g][0]][:MEM] + tot[GROUPS[g][1]][:MEM]
                        for g in (gw, gp)})
        if not first:
            add_h(s - 1, [(p, 1, tot[p][8:16]) for p in whole]
                  + [(p, z, tot[p][16 + 8 * z:24 + 8 * z]) for p in part for z in range(2)])
        add_h(s, [(p, 0, tot[p][8:16]) for p in part]
              + [(p, z, tot[p][16 + 8 * z:24 + 8 * z]) for p in whole for z in range(2)])
        return mem

    def wo_m1(slot, pairs):
        lhs = jnp.concatenate(
            [_rows(*[o1[slot + k, a] for k in range(3)]) for a in pairs], axis=1)
        return _dot(lhs, _rows(*[_unpack(wo_t[0, a]) for a in pairs]))

    def add_m1(s, r):
        for k in range(3):
            add_h(s + k, [(0, z, r[HS * k + 8 * z:HS * k + 8 * z + 8]) for z in range(2)])

    def prologue(wt, m1, qcar, stg0, stg1, stg2, stgo, xs, lhs1, lhs0, b1, qkv0, oacc):
        stg = (stg0, stg1, stg2)

        def x_copy(i):
            rows = pl.ds(_mult(i * (S // 4), S // 4), S // 4)
            return pltpu.make_async_copy(x_hbm.at[rows], xs.at[rows], sems.at[SEM_X + i])

        def wo_copy(g):
            rows = pl.ds(_mult(g * 512, 512), 512)
            return pltpu.make_async_copy(wo_hbm.bitcast(u32).at[rows], stgo,
                                         sems.at[SEM_WO + g])

        def start_chunk(g, m):
            src = w_hbm[m].bitcast(u32)
            dst = stg[m].reshape(D // 2, 8, DH)
            for par in range(2):
                pltpu.make_async_copy(
                    src.at[:, pl.ds(_mult(16 * par + 4 * g, 4), 4), :],
                    dst.at[:, pl.ds(4 * par, 4), :],
                    sems.at[SEM_W + 3 * g + m]).start()

        def wait_chunk(g, m):
            pltpu.make_async_copy(stg[m], stg[m], sems.at[SEM_W + 3 * g + m]).wait()

        def operands(g, m, pair, i):
            w = [stg[m][pl.ds(4 * (HD * k + 16 * i) + pair, 16, stride=4), :]
                 for k in range(2)]
            quad = [pltpu.bitcast(w[q >> 1] & jnp.uint32(0xFFFF0000) if q & 1
                                  else w[q >> 1] << 16, f32) for q in range(4)]
            b1[m, pair, pl.ds(16 * i, 16), :] = _rhs(0, quad.__getitem__).astype(bf16)
            for p in range(1, 7):
                wt[m][4 * g + pair, p - 1, pl.ds(8 * i, 8), :] = _pack(
                    _rhs(p, quad.__getitem__))

        def wo_operands(g, pair, i):
            w = [stgo[pl.ds(DH * pair + DH // 2 * (q >> 1) + 8 * i, 8),
                      pl.ds(HD * (q & 1), HD)] for q in range(4)]
            quad = [_unpack(v).astype(f32) for v in w]
            for p in range(7):
                wo_t[p, 4 * g + pair, pl.ds(8 * i, 8), :] = (
                    w[0] if p == 1 else w[3] if p == 4
                    else _pack(_rhs(p, quad.__getitem__)))

        start_chunk(0, 0)
        for i in range(4):
            x_copy(i).start()
        start_chunk(0, 1)
        start_chunk(0, 2)
        wo_copy(0).start()
        zero = jnp.zeros((HALO, C4), f32)
        for c in range(4):
            xg[c, pl.ds(0, HALO), :] = zero
            xg[c, pl.ds(HALO + S, HALO), :] = zero
        hbuf[pl.ds(0, PAD), :] = jnp.zeros((PAD, D), f32)
        for k in range(2):
            o1[k] = jnp.zeros((NP, HS, DH), bf16)
        oacc[...] = jnp.zeros(oacc.shape, f32)
        wait_chunk(0, 0)

        @pl.loop(0, 4)
        def _(pair):
            for i in range(HD // 16):
                operands(0, 0, pair, i)

        @pl.loop(0, 4)
        def _(i):
            x_copy(i).wait()

            @pl.loop(0, 4)
            def _(k):
                r0 = pl.multiple_of(i * (S // 4) + k * 128, 128)
                xv = xs[pl.ds(r0, 128), :].astype(f32)
                hbuf[pl.ds(PAD + r0, 128), :] = xv
                xn = _ln(xv)
                for c in range(4):
                    xg[c, pl.ds(HALO + r0, 128), :] = xn[:, c * C4:(c + 1) * C4]
                lhs1[pl.ds(pl.multiple_of(r0 // 4, 32), 32), :] = _pack(_rows(*[
                    xn[z:z + HS, :HD] + xn[z + HS:z + SEG, HD:]
                    for z in range(0, 128, SEG)]))

        mem = mem0_ref[...].astype(f32)
        cur, nxt = seg_quads(0), seg_quads(1)
        for p in range(1, 7):
            x0, x1 = _lhs(p, cur.__getitem__), _lhs(p, nxt.__getitem__)
            lhs0[p - 1] = _pack(
                _rows(x0, x1) if p in GROUPS[1]
                else _rows(_row_lhs(p, mem[:, :HD], mem[:, HD:]), x1[:8], x0))

        def project(g, m, pair):
            a = 4 * g + pair
            r = {p: _dot(_unpack(lhs0[p - 1]), _unpack(wt[m][a, p - 1]))
                 for p in range(1, 7)}
            first = _dot(_unpack(lhs1[...]), b1[m, pair])

            def keep():
                m1[NP * m + a] = first
                prod = {p: r[p][:HS] if p in GROUPS[1] else r[p][HS:] for p in r}
                prod[0] = first[:HS]
                qcar[m, a] = _rows(*[r[p][HS:] for p in GROUPS[1]],
                                   *[r[p][8:16] for p in GROUPS[2]])
                c_mem = _row_res({k: r[GROUPS[k][0]][:MEM] + r[GROUPS[k][1]][:MEM]
                                  for k in (0, 2)})
                for n, v in enumerate(heads_of(c_mem, prod)):
                    qkv0[m, a, n] = v
            return keep

        def step0(g):
            sc = [[_scores(qkv0[0, 4 * g + k, n], qkv0[1, 4 * g + k, n]) for n in range(2)]
                  for k in range(4)]
            o = [[_attend(sc[k][n], qkv0[2, 4 * g + k, n]) for n in range(2)]
                 for k in range(4)]
            none = jnp.zeros((3 * HS, DH), f32)
            res = [wo_pass(0, 4 * g + k, o[k], none, 2) for k in range(4)]
            for i, p in enumerate(res[0]):
                oacc[i] += res[0][p] + res[1][p] + res[2][p] + res[3][p]

        def stage(g, m):
            m2 = (m + 1) % 3
            g2 = jnp.minimum(g + (1 if m == 2 else 0), 3)
            work = _tasks(functools.partial(operands, g2, m2), range(4), range(HD // 16))
            extra = _tasks(functools.partial(wo_operands, g), range(4), range(8))
            span = 4 - WAIT_AT
            for j in range(4):
                if j >= WAIT_AT:
                    k = j - WAIT_AT
                    for w in (work, extra) if m == 2 else (work,):
                        for task in w[len(w) * k // span:len(w) * (k + 1) // span]:
                            task()
                keep = project(g, m, j)
                if j == WAIT_AT - 1:
                    @pl.when(g < 3)
                    def _():
                        start_chunk(g + 1, m)
                        if m == 2:
                            wait_chunk(g2, m2)
                    if m < 2:
                        wait_chunk(g2, m2)
                    if m == 2:
                        wo_copy(g).wait()
                if j == 3 and m == 2:
                    pl.when(g < 3)(lambda: wo_copy(g + 1).start())
                keep()

        @pl.loop(0, 4)
        def _(g):
            for m in range(3):
                stage(g, m)

        for i, dst in enumerate((w1b, w2b, w3b)):
            b_copy(i, dst).start()
        pl.loop(0, 4)(step0)
        order = [p for k in range(2) for p in (GROUPS[1][k], GROUPS[2][k])]
        return wo_finish(0, 0, {p: oacc[i] for i, p in enumerate(order)}, first=True)

    def step(wt, m1, qcar, s, phase, mem, o1_slot, fillers):
        gw, gp = (phase + 1) % 3, (phase + 2) % 3
        ahead, here = GROUPS[gw], GROUPS[gp]
        cur, nxt = seg_quads(s), seg_quads(jnp.minimum(s + 1, NSEG - 1))
        lhs = {}
        for p in ahead + here:
            x0, x1 = _lhs(p, cur.__getitem__), _lhs(p, nxt.__getitem__)
            riders = (x0[8:], x1) if p in ahead else (x1[:8], x0)
            lhs[p] = _rows(_row_lhs(p, *mem), *riders).astype(bf16)
        heads, scores, outs, tot = {}, {}, {}, {}

        def qkv(a):
            heads[a] = []
            for m in range(3):
                r = {p: _dot(lhs[p], _unpack(wt[m][a, p - 1])) for p in lhs}
                old = qcar[m, a]
                prod = {0: m1[NP * m + a, pl.ds(pl.multiple_of(s * HS, HS), HS), :]}
                for k in range(2):
                    prod[GROUPS[phase][k]] = old[HS * k:HS * k + HS]
                    prod[ahead[k]] = _rows(old[SEG + 8 * k:SEG + 8 * k + 8],
                                           r[ahead[k]][8:16])
                    prod[here[k]] = r[here[k]][HS:]
                qcar[m, a] = _rows(*[r[p][HS:] for p in ahead], *[r[p][8:16] for p in here])
                c_mem = _row_res({g: r[GROUPS[g][0]][:MEM] + r[GROUPS[g][1]][:MEM]
                                  for g in (gw, gp)})
                heads[a].append(heads_of(c_mem, prod))

        for t in range(NP + LAG_WO):
            a = t - LAG_QK
            if 0 <= a < NP:
                scores[a] = [_scores(heads[a][0][n], heads[a][1][n]) for n in range(2)]
            a = t - LAG_PV
            if 0 <= a < NP:
                outs[a] = [_attend(scores[a][n], heads[a][2][n]) for n in range(2)]
            if t < NP:
                qkv(t)
            if t == FILL_AT:
                fillers[0]()
            a = t - LAG_WO
            if 0 <= a < NP:
                for p, r in wo_pass(phase, a, outs[a], ocar[a], o1_slot).items():
                    tot[p] = tot[p] + r if p in tot else r
        fillers[1]()
        return wo_finish(phase, s, tot)

    def block_a(wt0, wt1, wt2, m1, qcar):
        wt = (wt0, wt1, wt2)
        stg = pltpu.VMEM((4 * D, DH), u32)
        if SKIP & 1:
            mem = (mem0_ref[:, :HD].astype(f32), mem0_ref[:, HD:].astype(f32))
        else:
            mem = pl.run_scoped(
                functools.partial(prologue, wt, m1, qcar), stg, stg, stg,
                pltpu.VMEM((512, D), u32),
                pltpu.VMEM((S, D), bf16),
                pltpu.VMEM((S // 4, HD), u32),
                pltpu.VMEM((6, HS, HD), u32),
                pltpu.VMEM((3, 4, HD, DH), bf16),
                pltpu.VMEM((3, NP, 2, L, DH), f32),
                pltpu.VMEM((4, SEG, HD), f32))

        def steps(i, mem):
            src = 3 * (i & 1)
            cuts = (0, 5, 10, NP)
            acc = []
            for k in range(3):
                c0, c1 = cuts[k], cuts[k + 1]
                fillers = [lambda lo=lo, hi=hi: acc.append(wo_m1(src, range(lo, hi)))
                           for lo, hi in ((c0, c0 + FILL_N), (c0 + FILL_N, c1))]
                mem = step(wt, m1, qcar, 3 * i + 1 + k, (1 + k) % 3, mem, 3 - src + k,
                           fillers)
            add_m1(3 * i - 2, functools.reduce(lambda u, v: u + v, acc))
            return mem

        if not SKIP & 2:
            lax.fori_loop(0, NSEG // 3, steps, mem)

    pl.run_scoped(block_a, *[pltpu.VMEM((NP, 6, HD // 2, DH), u32)] * 3,
                  pltpu.VMEM((3 * NP, S // 2, DH), f32),
                  pltpu.VMEM((3, NP, 3 * HS, DH), f32))

    def block_b(w4b, w3t, w4t, x1b, ya, pu, ta, pd, ob):
        b_copy(3, w4b).start()
        if not SKIP & 1:
            for i, dst in enumerate((w1b, w2b, w3b)):
                b_copy(i, dst).wait()

        def wo_last():
            phase = NSEG % 3
            terms = []
            for k in range(2):
                for p, r0, n in ((GROUPS[(phase + 2) % 3][k], HS * k, HS),
                                 (GROUPS[(phase + 1) % 3][k], SEG + 8 * k, 8)):
                    lhs = jnp.concatenate(
                        [ocar[a, pl.ds(r0, n), :] for a in range(NP)], axis=1)
                    r = _dot(lhs.astype(bf16),
                             _rows(*[_unpack(wo_t[p, a]) for a in range(NP)]))
                    terms += [(p, 1, r)] if n == 8 else [(p, 0, r[:8]), (p, 1, r[8:])]
            add_h(NSEG - 1, terms)
            add_m1(NSEG - 3, wo_m1(3 * (NSEG // 3 & 1), range(NP)))

        def w3_operands(c, i):
            blk = {(k, n): _unpack(w3b[pl.ds(128 * k + 8 * i, 8),
                                       pl.ds(FC * c + 128 * n, 128)]).astype(f32)
                   for k in range(4) for n in range(4)}
            for p, v in _twice(_rhs, blk):
                w3t[c, p, pl.ds(8 * i, 8), :] = _pack(v)

        def w4_operands(c, i):
            blk = {(k, n): _unpack(w4b[pl.ds(FC // 2 * c + 64 * k + 8 * (i >> 1), 8),
                                       pl.ds(C4 * n + 128 * (i & 1), 128)]).astype(f32)
                   for k in range(4) for n in range(4)}
            for p, v in _twice(_rhs, blk):
                w4t[c, p, pl.ds(8 * (i >> 1), 8), pl.ds(128 * (i & 1), 128)] = _pack(v)

        def mixer_norm(i):
            return _ln(_ln(hbuf[pl.ds(PAD + i * RB, RB), :])).astype(bf16)

        def mixer_in(i, u, c):
            xg[c, pl.ds(HALO + i * RB, RB), :] = _gelu(
                _dot(u, _unpack(w1b[:, pl.ds(c * C4, C4)])))

        def mixer_out(i, hs, c):
            off = (-1, 1, -2, 2)[c]
            win = xg[c, pl.ds(i * RB, RB + 2 * HALO), :]
            g = win[HALO + off:HALO + off + RB].astype(bf16)
            r = _dot(g, _unpack(w2b[pl.ds(c * C4 // 2, C4 // 2), :]))
            hs[i] = hs[i] + r if c else r

        def mixer_post(i, hs):
            hv = hbuf[pl.ds(PAD + i * RB, RB), :]
            x1 = _ln(hv) + hs
            x1b[pl.ds(i * RB, RB), :] = x1
            hbuf[pl.ds(PAD + i * RB, RB), :] = hv + x1

        def mlp_in(b, g):
            y = [_ln(x1b[pl.ds(_mult(b * RB + i * R + 16 * g, 16), 16), :])
                 for i in range(4)]
            blk = {(i, k): y[i][:, k * C4:(k + 1) * C4] for i in range(4) for k in range(4)}
            for p, v in _twice(_lhs, blk):
                ya[p, pl.ds(8 * g, 8), :] = _pack(v)

        def up(c, p1):
            m = [_dot(_unpack(ya[7 * p1 + p0]), _unpack(w3t[c, 7 * p1 + p0]))
                 for p0 in range(7)]
            for j in range(4):
                pu[c, p1, j] = _res(j, m.__getitem__)

        def mid(c, g, j):
            r = pl.ds(8 * g, 8)
            m = [pu[c, p1, j, r, :] for p1 in range(7)]
            y = [_gelu(_res(q, m.__getitem__)) for q in range(4)]
            for p1 in range(7):
                ta[c, p1, j, r, :] = _lhs(p1, y.__getitem__)

        def down(b, m, p1, p0):
            tot = None
            for c in range(NC):
                lhs = _lhs(p0, lambda j: ta[c, p1, j]).astype(bf16)
                r = _dot(lhs, _unpack(w4t[c, 7 * p1 + p0]))
                tot = r if tot is None else tot + r
            m[p0] = tot
            if p0 >= 3:
                j = (2, 1, 3, 0)[p0 - 3]
                v = _res(j, m.__getitem__)
                if p1 < 6:
                    pd[p1, j] = v
                if p1 >= 3:
                    q = (2, 1, 3, 0)[p1 - 3]
                    i, n = _pos(q, j)
                    r0, cols = _mult(b * RB + i * R, R), pl.ds(n * C4, C4)
                    v = _res(q, lambda k: v if k == p1 else pd[k, j])
                    ob[pl.ds(r0, R), cols] = (
                        hbuf[pl.ds(PAD + r0, R), cols] + v).astype(bf16)

        def out_copy(b):
            rows = pl.ds(_mult(b * RB, RB), RB)
            return pltpu.make_async_copy(ob.at[rows], out_hbm.at[rows],
                                         sems.at[SEM_OUT + b])

        if not SKIP & 4:
            u = mixer_norm(0)
            wo_last()
            for i in range(NB):
                nxt = mixer_norm(i + 1) if i + 1 < NB else None
                _interleave(_tasks(functools.partial(mixer_in, i, u), range(4)),
                            _tasks(functools.partial(w3_operands, i), range(16 * (i < NC))))
                u = nxt
        b_copy(3, w4b).wait()
        if not SKIP & 4:
            hs = {}
            for i in range(NB):
                if i:
                    mixer_post(i - 1, hs.pop(i - 1))
                _interleave(_tasks(functools.partial(mixer_out, i, hs), range(4)),
                            _tasks(functools.partial(w4_operands, i), range(16)) if i < NC
                            else _tasks(functools.partial(mlp_in, 0), range(R // 16)))
            _interleave(_tasks(functools.partial(up, 0), range(7)))
            mixer_post(NB - 1, hs.pop(NB - 1))

        @pl.loop(0, NB)
        def _(b):
            if SKIP & 8:
                out_copy(b).start()
                return
            for c in range(1, NC):
                _interleave(_tasks(functools.partial(up, c), range(7)),
                            _tasks(functools.partial(mid, c - 1), range(R // 8), range(4)))
            _interleave(_tasks(functools.partial(mid, NC - 1), range(R // 8), range(4)))
            _interleave(_tasks(functools.partial(down, b, {}), range(7), range(7)),
                        _tasks(functools.partial(mlp_in, jnp.minimum(b + 1, NB - 1)),
                               range(R // 16)))
            _interleave(_tasks(functools.partial(up, 0), range(7)))
            out_copy(b).start()

        for b in range(NB):
            out_copy(b).wait()

    pl.run_scoped(
        block_b,
        pltpu.VMEM((F // 2, D), u32),
        pltpu.VMEM((NC, 49, 128, 128), u32),
        pltpu.VMEM((NC, 49, 64, C4), u32),
        pltpu.VMEM((S, D), f32),
        pltpu.VMEM((49, R // 2, C4), u32),
        pltpu.VMEM((NC, 7, 4, R, 128), f32),
        pltpu.VMEM((NC, 7, 4, R, 128), f32),
        pltpu.VMEM((6, 4, R, C4), f32),
        pltpu.VMEM((S, D), bf16))


@jax.jit
def pallas_sequential_preLN__memory_aug_recurrent_mem_tr__mixer_s_mlp__prompt_kernel(
    A_x: jax.Array,
    A_mem0: jax.Array,
    A_Wq: jax.Array,
    A_Wk: jax.Array,
    A_Wv: jax.Array,
    A_Wo: jax.Array,
    A_seg_len: jax.Array,
    B_x: jax.Array,
    B_w1: jax.Array,
    B_w2: jax.Array,
    B_w3: jax.Array,
    B_w4: jax.Array,
):
    del A_seg_len, B_x
    hbm = pl.BlockSpec(memory_space=pl.ANY)
    vmem = pl.BlockSpec(memory_space=pltpu.VMEM)
    scratch = [
        pltpu.VMEM((PAD + S, D), f32),
        pltpu.VMEM((4, S + 2 * HALO, C4), f32),
        pltpu.VMEM((7, NP, DH // 2, HD), u32),
        pltpu.VMEM((6, NP, HS, DH), bf16),
        pltpu.VMEM((NP, 3 * HS, DH), f32),
        pltpu.VMEM((D // 2, D), u32),
        pltpu.VMEM((D // 2, D), u32),
        pltpu.VMEM((D // 2, F), u32),
        pltpu.SemaphoreType.DMA((NSEM,)),
    ]
    out = pl.pallas_call(
        _kernel,
        out_shape=jax.ShapeDtypeStruct((S, D), A_x.dtype),
        in_specs=[hbm, vmem] + [hbm] * 8,
        out_specs=hbm,
        scratch_shapes=scratch,
        compiler_params=pltpu.CompilerParams(vmem_limit_bytes=127 * 1024 * 1024),
    )(A_x.reshape(S, D), A_mem0.reshape(MEM, D),
      A_Wq.reshape(D // 2, 2 * H, DH), A_Wk.reshape(D // 2, 2 * H, DH),
      A_Wv.reshape(D // 2, 2 * H, DH),
      A_Wo.reshape(H * DH, D), B_w1, B_w2, B_w3, B_w4)
    return out.reshape(A_x.shape)
```

```python
import functools

import jax
import jax.numpy as jnp
from jax import lax
import jax.experimental.pallas as pl
import jax.experimental.pallas.tpu as pltpu

S = 2048
D = 1024
H = 32
DH = 128
MEM = 8
SEG = 32
F = 3584
NSEG = S // SEG
L = MEM + SEG
HS = SEG // 2
NP = H // 2
HD = D // 2
PAD = 2 * SEG
C4 = D // 4
HALO = 8
R = 64
RB = 4 * R
NB = S // RB
FC = 512
NC = F // FC
EPS = 1e-5
NEG = -1000000000.0

LAG_QK = 2
LAG_PV = 4
LAG_WO = 6
FILL_AT = 18
FILL_N = 2
UP_LAG = 8
DN_LAG = 20
MX_LAG = 4
CH0 = 3
CH = 1
AB = 4
AB2 = 1
MC = 21
G1 = 6
G2 = 12
G3 = 6
M1_CUT = 16
SKIP = 0

GROUPS = ((1, 3), (2, 4), (5, 6))
TARGETS = (((0, 1), (3, 1)), ((2, 1), (3, -1)), ((1, 1), (3, 1)), ((0, 1), (2, 1)),
           ((0, -1), (1, 1)), ((3, 1),), ((0, 1),))

bf16 = jnp.bfloat16
f32 = jnp.float32
u32 = jnp.uint32

SEM_X, SEM_W, SEM_WO, SEM_B, SEM_OUT = 0, 4, 16, 20, 24
NSEM = SEM_OUT + NB


def _mult(i, n):
    return i if isinstance(i, int) else pl.multiple_of(i, n)


def _ln(x):
    m = jnp.mean(x, axis=-1, keepdims=True)
    d = x - m
    v = jnp.mean(d * d, axis=-1, keepdims=True)
    return d * lax.rsqrt(v + EPS)


def _gelu2(x):
    c = 0.7978845608028654
    return x + x * jnp.tanh(x * (c + (c * 0.044715) * (x * x)))


def _get(ref, *idx, rows=None):
    rows = slice(None) if rows is None else pl.ds(rows[0] // 2, rows[1] // 2)
    return _unpack(ref.bitcast(u32)[idx + (rows, slice(None))])


def _cols(*xs):
    return jnp.concatenate(xs, axis=1)


def _unpack(x):
    return pltpu.bitcast(x, bf16)


def _dot(a, b):
    return jnp.dot(a, b, preferred_element_type=f32)


def _rows(*xs):
    return jnp.concatenate(xs, axis=0)


def _lhs(p, a):
    return (lambda: a(0) + a(3), lambda: a(2) + a(3), lambda: a(0), lambda: a(3),
            lambda: a(0) + a(1), lambda: a(2) - a(0), lambda: a(1) - a(3))[p]()


def _rhs(p, b):
    return (lambda: b(0) + b(3), lambda: b(0), lambda: b(1) - b(3), lambda: b(2) - b(0),
            lambda: b(3), lambda: b(0) + b(1), lambda: b(2) + b(3))[p]()


def _res(q, m):
    return (lambda: m(0) + m(3) - m(4) + m(6), lambda: m(2) + m(4),
            lambda: m(1) + m(3), lambda: m(0) - m(1) + m(2) + m(5))[q]()


def _pos(q, j):
    return 2 * (q >> 1) + (j >> 1), 2 * (q & 1) + (j & 1)


def _twice(side, blk, p1):
    outer = [side(p1, lambda q: blk(*_pos(q, j))) for j in range(4)]
    return [side(p0, outer.__getitem__) for p0 in range(7)]


def _ln_tasks(load, store):
    st = {}

    def mean():
        st["m"] = jnp.mean(load(), axis=-1, keepdims=True)
        return st["m"]

    def scale():
        d = load() - st["m"]
        st["r"] = lax.rsqrt(jnp.mean(d * d, axis=-1, keepdims=True) + EPS)
        return st["r"]

    return [mean, scale, lambda: store((load() - st["m"]) * st["r"])]


def _abreast(chains, n):
    return [t for i in range(0, len(chains), n) for ts in zip(*chains[i:i + n]) for t in ts]


def _token(x):
    x = x[-8:, -DH:] if x.shape[1] >= DH else jnp.broadcast_to(x[-8:], (8, DH))
    return pltpu.bitcast(x, u32)


def _row_lhs(p, a1, a2):
    return a1 + a2 if p in (1, 4) else a1 if p in (2, 5) else a2


def _row_res(t):
    if 0 not in t:
        return t[2] - t[1], t[1]
    if 1 not in t:
        return t[0], t[2] - t[0]
    return t[0], t[1]


def _merge(*lists):
    order = sorted(((i + 0.5) / len(l), n, i)
                   for n, l in enumerate(lists) for i in range(len(l)))
    return [lists[n][i] for _, n, i in order]


def _interleave(*lists):
    for task in _merge(*lists):
        task()


def _overlap(dots, side, release, lag):
    for i, dot in enumerate(dots):
        result = dot()
        mine = _share(side, i, len(dots) - lag)
        if mine:
            release(_token(result))
        for task in mine:
            task()


def _share(tasks, k, n):
    return tasks[len(tasks) * k // n:len(tasks) * (k + 1) // n] if k >= 0 else []


def _tasks(fn, *ranges):
    if len(ranges) == 2:
        return [functools.partial(fn, i, j) for i in ranges[0] for j in ranges[1]]
    return [functools.partial(fn, i) for i in ranges[0]]


def _start(copies):
    for c in copies:
        c.start()


def _wait(copies):
    for c in copies:
        c.wait()


def _scores(q, k):
    return lax.dot_general(q, k, (((1,), (1,)), ((), ())), preferred_element_type=f32)


def _attend(sc, v):
    ri = lax.broadcasted_iota(jnp.int32, (L, L), 0)
    ci = lax.broadcasted_iota(jnp.int32, (L, L), 1)
    sc = jnp.where((ri < MEM) | (ri >= ci), sc * (DH ** -0.5), NEG)
    mx = jnp.max(sc, axis=1, keepdims=True)
    e = jnp.exp(sc - mx)
    den = jnp.sum(e, axis=1, keepdims=True)
    inv = pl.reciprocal(den, approx=True)
    inv = inv * (2.0 - den * inv)
    return _dot(e, v) * inv


def _kernel(x_hbm, mem0_ref, wq_hbm, wk_hbm, wv_hbm, wo_hbm, w1_hbm, w2_hbm,
            w3_hbm, w4_hbm, out_hbm, hbuf, xg, wo_t, o1, late, ocar, m1, w12, sems):
    w_hbm = (wq_hbm, wk_hbm, wv_hbm)
    here = lax.fori_loop(0, 2, lambda i, z: z + (i >> 1), jnp.int32(0))

    def b_copies(raw):
        tile = lambda w, i: w.bitcast(u32).at[:, :, pl.ds(128 * i, 128)]
        for n in range(4):
            slabs = pl.ds(4 * n, 4)
            for i, w in enumerate((w1_hbm, w2_hbm)):
                for c in range(2):
                    yield pltpu.make_async_copy(
                        tile(w, 2 * n + c),
                        raw.at[slabs, pl.ds(128 * (NC + 2 * i + c), 128)],
                        sems.at[SEM_B])
            for c in range(NC):
                yield pltpu.make_async_copy(
                    tile(w3_hbm, 4 * c + n), raw.at[slabs, pl.ds(128 * c, 128)],
                    sems.at[SEM_B])

    def b_operands(raw, dst, r1, p1):
        for p0, v in enumerate(_twice(_rhs, lambda k, n: _unpack(raw(k, n)).astype(f32), p1)):
            if p1 in (1, 4) and p0 in (1, 4):
                k = 2 * (p1 // 4) + p0 // 4
                dst.bitcast(u32)[7 * p1 + p0, pl.ds(r1, 8), :] = raw(k, k)
            else:
                dst[7 * p1 + p0, pl.ds(_mult(2 * r1, 16), 16), :] = v.astype(bf16)

    def rows_of(r0, n):
        return pl.ds(pl.multiple_of(r0 + here, 8), n)

    def put(rows, x):
        for c in range(8):
            xg[c, rows, :] = x[:, DH * c:DH * (c + 1)]

    def mixer_norm(r0):
        store = functools.partial(put, rows_of(HALO + r0, HS))
        again = lambda: _cols(*[xg[c, rows_of(HALO + r0, HS), :] for c in range(8)])
        return (_ln_tasks(lambda: hbuf[rows_of(PAD + r0, HS), :], store)
                + _ln_tasks(again, store))

    def wo_tile(p, a):
        return _cols(*[_get(wo_t, p, a, c) for c in range(4)])

    def seg_quads(s):
        r0 = HALO + s * SEG
        return [jnp.concatenate(
            [xg[4 * (q & 1) + c, pl.ds(_mult(r0 + (q >> 1) * HS, 8), HS), :]
             for c in range(4)], axis=1) for q in range(4)]

    def heads_of(c_mem, m):
        return [_rows(c_mem[n], _res(n, m.__getitem__), _res(2 + n, m.__getitem__))
                for n in range(2)]

    def wo_pass(phase, a, o, prev, o1_slot):
        whole, part = GROUPS[(phase + 1) % 3], GROUPS[(phase + 2) % 3]
        quad = lambda q: o[q & 1][MEM + (q >> 1) * HS:MEM + (q >> 1) * HS + HS]
        x = [_lhs(p, quad) for p in range(7)]
        o1[o1_slot, a] = x[0].astype(bf16)
        ocar[a] = _rows(*[x[p] for p in GROUPS[phase]], *[x[p][8:] for p in part])
        res = {}
        for k in range(2):
            for p, riders in ((whole[k], (prev[SEG + 8 * k:SEG + 8 * k + 8], x[whole[k]])),
                              (part[k], (x[part[k]][:8], prev[HS * k:HS * k + HS]))):
                lhs = _rows(_row_lhs(p, o[0][:MEM], o[1][:MEM]), *riders)
                res[p] = _dot(lhs.astype(bf16), wo_tile(p, a))
        return res

    def add_h(s, terms):
        for q in range(4):
            for z in range(2):
                mine = [(sign, v) for p, zz, v in terms if zz == z
                        for qq, sign in TARGETS[p] if qq == q]
                if mine:
                    at = (pl.ds(_mult(PAD + s * SEG + (q >> 1) * HS + 8 * z, 8), 8),
                          pl.ds((q & 1) * HD, HD))
                    acc = hbuf[at]
                    for sign, v in mine:
                        acc = acc + v if sign > 0 else acc - v
                    hbuf[at] = acc

    def wo_finish(phase, s, tot, first=False):
        gw, gp = (phase + 1) % 3, (phase + 2) % 3
        whole, part = GROUPS[gw], GROUPS[gp]
        mem = _row_res({g: tot[GROUPS[g][0]][:MEM] + tot[GROUPS[g][1]][:MEM]
                        for g in (gw, gp)})
        if not first:
            add_h(s - 1, [(p, 1, tot[p][8:16]) for p in whole]
                  + [(p, z, tot[p][16 + 8 * z:24 + 8 * z]) for p in part for z in range(2)])
        add_h(s, [(p, 0, tot[p][8:16]) for p in part]
              + [(p, z, tot[p][16 + 8 * z:24 + 8 * z]) for p in whole for z in range(2)])
        return mem

    def wo_m1(slot, pairs):
        lhs = jnp.concatenate(
            [_rows(*[_get(o1, slot + k, a) for k in range(3)]) for a in pairs], axis=1)
        return _dot(lhs, _rows(*[wo_tile(0, a) for a in pairs]))

    def add_m1(s, r):
        for k in range(3):
            add_h(s + k, [(0, z, r[HS * k + 8 * z:HS * k + 8 * z + 8]) for z in range(2)])

    def prologue(wt, qcar, stg, lhs1, lhs0, qkv0):
        words = w12.bitcast(u32)

        def tile_copies(src, rows, n, dst, slab, sem):
            return [pltpu.make_async_copy(
                src.bitcast(u32).at[pl.ds(rows, n), pl.ds(128 * c, 128)],
                dst.at[slab + c, pl.ds(0, n)], sem) for c in range(8)]

        def x_copies(i):
            return tile_copies(x_hbm, _mult(i * (S // 8), S // 8), S // 8, words, 8 * i,
                               sems.at[SEM_X + i])

        def wo_copies(g):
            return tile_copies(wo_hbm, g * 512, 512, words, 8 * g, sems.at[SEM_WO + g])

        def start_chunk(g, m):
            src = w_hbm[m].bitcast(u32)
            dst = stg.reshape(3 * HD, 8, DH)
            for par in range(2):
                pltpu.make_async_copy(
                    src.at[:, pl.ds(_mult(16 * par + 4 * g, 4), 4), :],
                    dst.at[pl.ds(HD * m, HD), pl.ds(4 * par, 4), :],
                    sems.at[SEM_W + 3 * g + m]).start()

        def wait_chunk(g, m):
            part = stg.at[pl.ds(_mult(4 * D * m, 4 * D), 4 * D)]
            pltpu.make_async_copy(part, part, sems.at[SEM_W + 3 * g + m]).wait()

        def operands(g, m, pair, i):
            w = [stg[pl.ds(4 * (D * m + HD * k + 16 * i) + pair, 16, stride=4), :]
                 for k in range(2)]
            quad = [pltpu.bitcast(w[q >> 1] & jnp.uint32(0xFFFF0000) if q & 1
                                  else w[q >> 1] << 16, f32) for q in range(4)]
            wt[3 * NP + m, pair, pl.ds(16 * i, 16), :] = _rhs(0, quad.__getitem__).astype(bf16)
            for p in range(1, 7):
                wt[NP * m + 4 * g + pair, p - 1, pl.ds(16 * i, 16), :] = _rhs(
                    p, quad.__getitem__).astype(bf16)

        def wo_operands(g, pair, i):
            c, r0 = i & 3, 8 * (i >> 2)
            w = [words[8 * g + 4 * (q & 1) + c + here, pl.ds(DH * pair + DH // 2 * (q >> 1) + r0, 8), :]
                 for q in range(4)]
            quad = [_unpack(v).astype(f32) for v in w]
            for p in range(7):
                v = _rhs(p, quad.__getitem__).astype(bf16)
                wo_t[p, 4 * g + pair, c, pl.ds(2 * r0, 16), :] = v

        start_chunk(0, 0)
        for i in range(4):
            _start(x_copies(i))
        start_chunk(0, 1)
        start_chunk(0, 2)
        for r0 in (0, HALO + S):
            put(pl.ds(r0, HALO), jnp.zeros((HALO, D), f32))
        hbuf[pl.ds(0, PAD), :] = jnp.zeros((PAD, D), f32)
        for k in range(2):
            o1[k] = jnp.zeros((NP, HS, DH), bf16)
        wait_chunk(0, 0)

        @pl.loop(0, 4)
        def _(pair):
            for i in range(HD // 16):
                operands(0, 0, pair, i)

        @pl.loop(0, 4)
        def _(i):
            _wait(x_copies(i))

            @pl.loop(0, 4)
            def _(k):
                r0 = pl.multiple_of(i * (S // 4) + k * 128, 128)
                xv = jnp.concatenate(
                    [_unpack(words[8 * i + c, pl.ds(pl.multiple_of(k * 64, 64), 64), :])
                     for c in range(8)], axis=1).astype(f32)
                hbuf[pl.ds(PAD + r0, 128), :] = xv
                xn = _ln(xv)
                put(pl.ds(HALO + r0, 128), xn)
                v = _rows(*[xn[z:z + HS, :HD] + xn[z + HS:z + SEG, HD:]
                            for z in range(0, 128, SEG)])
                for c in range(4):
                    lhs1[c, pl.ds(pl.multiple_of(r0 // 2, 64), 64), :] = (
                        v[:, DH * c:DH * (c + 1)].astype(bf16))

        mem = mem0_ref[...].astype(f32)
        cur, nxt = seg_quads(0), seg_quads(1)
        for p in range(1, 7):
            x0, x1 = _lhs(p, cur.__getitem__), _lhs(p, nxt.__getitem__)
            v = (_rows(x0, x1) if p in GROUPS[1]
                 else _rows(_row_lhs(p, mem[:, :HD], mem[:, HD:]), x1[:8], x0))
            for c in range(4):
                lhs0[p - 1, c] = v[:, DH * c:DH * (c + 1)].astype(bf16)

        def first(g, m, pair, i):
            n = S // 2 // M1_CUT
            lhs = _cols(*[_get(lhs1, c, rows=(n * i, n)) for c in range(4)])
            r = pltpu.bitcast(_dot(lhs, _get(wt, 3 * NP + m + here, pair)), u32)
            m1.bitcast(u32)[NP * m + 4 * g + pair, pl.ds(n * i, n), :] = r
            return r

        def project(g, m, pair):
            a = 4 * g + pair
            r = {p: _dot(_cols(*[_get(lhs0, p - 1, c) for c in range(4)]),
                         _get(wt, NP * m + a, p - 1))
                 for p in range(1, 7)}
            prod = {p: r[p][:HS] if p in GROUPS[1] else r[p][HS:] for p in r}
            prod[0] = pltpu.bitcast(m1.bitcast(u32)[NP * m + a, pl.ds(0, HS), :], f32)
            qcar[m, a] = _rows(*[r[p][HS:] for p in GROUPS[1]],
                               *[r[p][8:16] for p in GROUPS[2]])
            c_mem = _row_res({k: r[GROUPS[k][0]][:MEM] + r[GROUPS[k][1]][:MEM]
                              for k in (0, 2)})
            for n, v in enumerate(heads_of(c_mem, prod)):
                qkv0[m, a, n] = v

        def wo_tasks(g):
            return _tasks(functools.partial(wo_operands, g), range(4), range(32))

        def dots(g, m):
            return _tasks(functools.partial(first, g, m), range(4), range(M1_CUT))

        @pl.loop(0, 11)
        def _(c):
            g, g2 = lax.div(c, 3), lax.div(c + 1, 3)
            m, m2 = c - 3 * g, c + 1 - 3 * g2
            for k in range(3):
                pl.when((m == k) & (g < 3))(functools.partial(start_chunk, g + 1, k))
            pl.when(c == 9)(lambda: _start([cp for k in range(4) for cp in wo_copies(k)]))
            wait_chunk(g2, m2)
            _interleave(_tasks(functools.partial(operands, g2, m2), range(4), range(HD // 16)),
                        dots(g, m))
            for pair in range(4):
                project(g, m, pair)

        def release(t):
            words[48, pl.ds(0, 8), :] = t

        for k in range(2):
            _wait(wo_copies(k))
            _overlap(_share(dots(3, 2), k, 2), wo_tasks(k), release, 2)

        scores, outs, tot = {}, {}, {}
        none = jnp.zeros((3 * HS, DH), f32)

        def step0(t):
            if t < NP:
                scores[t] = [_scores(qkv0[0, t, n], qkv0[1, t, n]) for n in range(2)]
            if 0 <= t - 2 < NP:
                outs[t - 2] = [_attend(scores[t - 2][n], qkv0[2, t - 2, n]) for n in range(2)]
            if 0 <= t - 4 < NP:
                for p, r in wo_pass(0, t - 4, outs[t - 4], none, 2).items():
                    tot[p] = tot[p] + r if p in tot else r
                return r
            project(3, 2, t)
            return qkv0[0, t, 0]

        for k, slots in ((2, range(12)), (3, range(12, 16))):
            _wait(wo_copies(k))
            _overlap(_tasks(step0, slots), wo_tasks(k), release, 1)
        _interleave(_tasks(step0, range(16, 20)))
        return wo_finish(0, 0, tot, first=True)

    def step(wt, qcar, s, phase, cur, nxt, first, mem, o1_slot, fillers, chores, release):
        gw, gp = (phase + 1) % 3, (phase + 2) % 3
        ahead, now = GROUPS[gw], GROUPS[gp]
        lhs = {}
        for p in ahead + now:
            x0, x1 = _lhs(p, cur.__getitem__), _lhs(p, nxt.__getitem__)
            riders = (x0[8:], x1) if p in ahead else (x1[:8], x0)
            lhs[p] = _rows(_row_lhs(p, *mem), *riders).astype(bf16)
        heads, scores, outs, tot = {}, {}, {}, {}

        def qkv(a):
            heads[a] = []
            for m in range(3):
                r = {p: _dot(lhs[p], _get(wt, NP * m + a, p - 1)) for p in lhs}
                mine = _share(chores, 3 * a + m, 3 * NP - CH0)
                if mine:
                    release(_token(r[now[1]]))
                for task in mine:
                    task()
                old = qcar[m, a]
                prod = {0: pltpu.bitcast(first(NP * m + a), f32)}
                for k in range(2):
                    prod[GROUPS[phase][k]] = old[HS * k:HS * k + HS]
                    prod[ahead[k]] = _rows(old[SEG + 8 * k:SEG + 8 * k + 8],
                                           r[ahead[k]][8:16])
                    prod[now[k]] = r[now[k]][HS:]
                qcar[m, a] = _rows(*[r[p][HS:] for p in ahead], *[r[p][8:16] for p in now])
                c_mem = _row_res({g: r[GROUPS[g][0]][:MEM] + r[GROUPS[g][1]][:MEM]
                                  for g in (gw, gp)})
                heads[a].append(heads_of(c_mem, prod))

        for t in range(NP + LAG_WO):
            a = t - LAG_QK
            if 0 <= a < NP:
                scores[a] = [_scores(heads[a][0][n], heads[a][1][n]) for n in range(2)]
            a = t - LAG_PV
            if 0 <= a < NP:
                outs[a] = [_attend(scores[a][n], heads[a][2][n]) for n in range(2)]
            if t < NP:
                qkv(t)
            if t == FILL_AT:
                fillers[0]()
            a = t - LAG_WO
            if 0 <= a < NP:
                for p, r in wo_pass(phase, a, outs[a], ocar[a], o1_slot).items():
                    tot[p] = tot[p] + r if p in tot else r
        fillers[1]()
        return wo_finish(phase, s, tot)

    def recurrence(wt, qcar, mem, raw, m1s):
        def m1_copy(i):
            rows = pl.ds(_mult((3 * i + 1) * HS, HS), 3 * HS)
            return pltpu.make_async_copy(m1.bitcast(u32).at[pl.ds(0, 3 * NP), rows], m1s.at[i & 1],
                                         sems.at[SEM_B + 2])

        m1_copy(0).start()
        late[...] = jnp.zeros(late.shape, f32)
        _start(b_copies(raw))
        spare = 128 * (NC + 4)
        raw[pl.ds(0, 16), pl.ds(spare, 8), :] = jnp.zeros((16, 8, DH), u32)

        def chores(i):
            def convert(dst, base, per, groups):
                tasks = []
                for k in range(per):
                    r = pl.multiple_of(8 * jnp.clip(per * (i - 1) + k, 0, groups - 1), 8)
                    r0 = pl.multiple_of(jnp.where(i > 0, base + r, spare), 8)
                    tasks += _tasks(functools.partial(
                        b_operands, lambda k, n, r0=r0: raw[4 * n + k, pl.ds(r0, 8), :],
                        dst, r), range(7))
                return tasks
            norm = _abreast([mixer_norm(jnp.maximum(3 * i - 5 + (k >> 1), 0) * SEG
                                        + (k & 1) * HS) for k in range(6)], AB2)
            norm.insert(0, lambda: add_m1(jnp.maximum(3 * i - 5, -2), late[...]))
            return _merge(convert(m1, 0, 6, 16 * NC) + convert(w12, 128 * NC, 4, 64), norm)

        def release(t):
            raw[16, pl.ds(0, 8), :] = t
            hbuf[pl.ds(0, 8), pl.ds(0, DH)] = pltpu.bitcast(t, f32)

        def steps(i, mem):
            pl.when(i < MC)(lambda: m1_copy(i).wait())
            pl.when(i + 1 < MC)(lambda: m1_copy(i + 1).start())
            pl.when(i == 1)(lambda: _wait(b_copies(raw)))
            src = 3 * (i & 1)
            cuts = (0, 5, 10, NP)
            acc = []
            todo = chores(i) if CH else []
            nxt = seg_quads(3 * i + 1)
            for k in range(3):
                c0, c1 = cuts[k], cuts[k + 1]
                fillers = [lambda lo=lo, hi=hi: acc.append(wo_m1(src, range(lo, hi)))
                           for lo, hi in ((c0, c0 + FILL_N), (c0 + FILL_N, c1))]
                cur, nxt = nxt, seg_quads(jnp.minimum(3 * i + 2 + k, NSEG - 1))
                mem = step(wt, qcar, 3 * i + 1 + k, (1 + k) % 3, cur, nxt,
                           lambda j: m1s[i & 1, j, pl.ds(HS * k, HS), :], mem,
                           3 - src + k, fillers, _share(todo, k, 3), release)
            late[...] = functools.reduce(lambda u, v: u + v, acc)
            return mem

        if not SKIP & 2:
            lax.fori_loop(0, NSEG // 3, steps, mem)
        else:
            m1_copy(0).wait()
            _wait(b_copies(raw))

    def block_a(wt, qcar):
        if SKIP & 1:
            mem = (mem0_ref[:, :HD].astype(f32), mem0_ref[:, HD:].astype(f32))
        else:
            mem = pl.run_scoped(
                functools.partial(prologue, wt, qcar),
                pltpu.VMEM((12 * D, DH), u32),
                pltpu.VMEM((4, S // 2, DH), bf16),
                pltpu.VMEM((6, 4, SEG, DH), bf16),
                pltpu.VMEM((3, NP, 2, L, DH), f32))

        pl.run_scoped(functools.partial(recurrence, wt, qcar, mem),
                      pltpu.VMEM((17, 128 * (NC + 4) + 8, DH), u32),
                      pltpu.VMEM((2, 3 * NP, 3 * HS, DH), u32))

    pl.run_scoped(block_a, pltpu.VMEM((3 * NP + 3, 6, HD, DH), bf16),
                  pltpu.VMEM((3, NP, 3 * HS, DH), f32))

    def block_b(w4t, x1b, yn, ya, *pu):
        pu = [pu[(0, 1, 2, 0, 1, 2, 1)[c]] for c in range(NC)]
        def wo_last():
            phase = NSEG % 3
            tot = {}

            def task(a0, p, r0=0, n=0):
                pairs = range(a0, a0 + 2)
                if p == 0:
                    r = wo_m1(3 * (NSEG // 3 & 1), pairs)
                else:
                    lhs = _cols(*[ocar[a, pl.ds(r0, n), :] for a in pairs])
                    r = _dot(lhs.astype(bf16), _rows(*[wo_tile(p, a) for a in pairs]))
                tot[p] = tot[p] + r if a0 else r
                if a0 == NP - 2 and p == 0:
                    add_m1(NSEG - 3, tot[p])
                elif a0 == NP - 2:
                    add_h(NSEG - 1, [(p, 1, tot[p][-8:])] + [(p, 0, tot[p][:8])] * (n > 8))
                return r

            todo = [(0,)] + [t for k in range(2) for t in (
                (GROUPS[(phase + 2) % 3][k], HS * k, HS),
                (GROUPS[(phase + 1) % 3][k], SEG + 8 * k, 8))]
            return [functools.partial(task, a0, *t) for t in todo for a0 in range(0, NP, 2)]

        def a_operands(load, dst):
            def task(g, p1):
                r0, c = 16 * (g >> 1), g & 1
                for p0, v in enumerate(_twice(
                        _lhs, lambda i, k: load(i * R + r0, 2 * k + c), p1)):
                    dst[7 * p1 + p0, c, pl.ds(r0, 16), :] = v.astype(bf16)
            return _tasks(task, range(R // 8), range(7))

        def products(src, at, w, r0, dst):
            m = {}

            def task(p1, p0):
                p = 7 * p1 + p0
                m[p0] = _dot(_cols(*[_get(src, *at(p), k) for k in range(2)]),
                             _get(w, p, rows=(r0, C4)))
                if p0 >= 3:
                    j = (2, 1, 3, 0)[p0 - 3]
                    dst[p1, j] = _res(j, m.__getitem__)
                return m[p0]
            return _tasks(task, range(7), range(7))

        def mlp_in(b, slot):
            def residual(r0, y):
                x1 = y + x1b[rows_of(b * RB + r0, 16), :]
                yn[pl.ds(r0, 16), :] = x1
                put(rows_of(b * RB + r0, 16), hbuf[rows_of(PAD + b * RB + r0, 16), :] + x1)

            def store(r0, y):
                yn[pl.ds(r0, 16), :] = y
                return y

            chains = [_ln_tasks(lambda r0=r0: hbuf[rows_of(PAD + b * RB + r0, 16), :],
                                functools.partial(residual, r0))
                      + _ln_tasks(lambda r0=r0: yn[rows_of(r0, 16), :],
                                  functools.partial(store, r0)) for r0 in range(0, RB, 16)]
            return _abreast(chains, AB) + a_operands(
                lambda r0, c: yn[rows_of(r0, 16), pl.ds(DH * c, DH)], ya.at[slot])

        def ups(b, c):
            return products(ya, lambda p: (b & 1, p), m1, C4 * c, pu[c])

        def mixer(raw, *bufs):
            sa, sp = bufs[:2], bufs[2:]
            w4_copies = [pltpu.make_async_copy(
                w4_hbm.bitcast(u32).at[pl.ds(c, n), :, :, pl.ds(DH * i, DH)],
                raw.at[i, pl.ds(c, n)], sems.at[SEM_B + s])
                for c, n, s in ((0, 2, 1), (2, NC - 2, 3)) for i in range(8)]
            _start(w4_copies)

            def pre(n, w, b):
                shift = lambda c: w * (-1, 1, -2, 2)[c >> 1]
                return a_operands(lambda r0, c: xg[c + here, pl.ds(
                    HALO + b * RB + r0 + shift(c), 16), :], sa[n & 1])

            def post(n, w, b):
                def task(g, j):
                    c = g & 1
                    m = [sp[n & 1][c + here, p1, j, pl.ds(8 * (g >> 1), 8), :]
                         for p1 in range(7)]
                    for q in range(4):
                        i, k = _pos(q, j)
                        r0 = _mult(b * RB + i * R + 8 * (g >> 1), 8)
                        v = _res(q, m.__getitem__)
                        if w == 0:
                            xg[2 * k + c, pl.ds(HALO + r0, 8), :] = _gelu2(v)
                        else:
                            x1b[pl.ds(r0, 8), pl.ds(DH * (2 * k + c), DH)] = 0.5 * v
                return _tasks(task, range(R // 4), range(4))

            def release(n, norms, t):
                raw[8, 0, 0, pl.ds(0, 8), :] = t
                t = pltpu.bitcast(t, f32)
                sp[1 - (n & 1)][0, 7, 0, pl.ds(0, 8), :] = t
                xg[0, pl.ds(S + 2 * HALO, 8), :] = t
                if norms:
                    hbuf[pl.ds(0, 8), pl.ds(0, DH)] = t
                    yn[pl.ds(RB, 8), pl.ds(0, DH)] = t

            def unit(n, w, *side, norms=False):
                dots = [t for c in range(2) for t in products(
                    sa[n & 1], lambda p: (p + here,), w12, C4 * (2 * w + c), sp[n & 1].at[c])]
                pairs = [lambda u=u, v=v: (u(), v())[1] for u, v in zip(dots[::2], dots[1::2])]
                _overlap(pairs, _merge(*side), functools.partial(release, n, norms), MX_LAG)

            def w4_work(k, n):
                def task(i, p1):
                    g = k + i
                    b_operands(lambda q, c: raw[2 * c + ((g >> 3) & 1) + here, g >> 4, q,
                                                pl.ds(_mult(8 * (g & 7), 8), 8), :],
                               w4t, _mult(8 * g, 8), p1)
                return _tasks(task, range(n), range(7))

            if not SKIP & 4:
                norms = lambda s: _abreast(
                    [mixer_norm(s * SEG + k * HS) for k in range(6)], 3)
                add_m1(NSEG - 6, late[...])
                _overlap(wo_last(), _merge(pre(0, 0, 0), norms(NSEG - 6)),
                         functools.partial(release, 0, True), MX_LAG)
                unit(0, 0, pre(1, 0, 1), norms(NSEG - 3), norms=True)
                unit(1, 0, pre(2, 0, 2), post(0, 0, 0))

                _wait(w4_copies[:8])

                @pl.loop(0, 2)
                def _(i):
                    for n in range(2):
                        b = 2 * i + 2 + n
                        unit(n, 0, pre(n + 1, 0, b + 1), post(n + 1, 0, b - 1),
                             w4_work(G1 * (b - 2), G1))

                _wait(w4_copies[8:])
                unit(0, 0, pre(1, 0, 7), post(1, 0, 5), w4_work(4 * G1, G1))
                unit(1, 0, pre(0, 1, 0), post(0, 0, 6), w4_work(5 * G1, G1))
                unit(0, 1, pre(1, 1, 1), post(1, 0, 7), w4_work(6 * G1, G1))
                unit(1, 1, pre(0, 1, 2), post(0, 1, 0), w4_work(7 * G1, G2))
                unit(0, 1, pre(1, 1, 3), post(1, 1, 1), w4_work(7 * G1 + G2, G2))
                done = 7 * G1 + 2 * G2

                @pl.loop(0, 2)
                def _(i):
                    ahead = mlp_in(i, i)
                    for n in range(2):
                        b = 2 * i + 3 + n
                        unit(n + 1, 1, pre(n, 1, b + 1), post(n, 1, b - 1),
                             _share(ahead, n, 2), w4_work(done + G3 * (b - 3), G3),
                             norms=True)

                done += 4 * G3
                rest = w4_work(done, 16 * NC - done)
                unit(1, 1, post(0, 1, 6), _share(rest, 0, 3) + _share(rest, 1, 3))
                _overlap(ups(0, 0), _merge(post(1, 1, 7), _share(rest, 2, 3)),
                         functools.partial(release, 0, False), MX_LAG)
            else:
                _wait(w4_copies)

        def mlp(ta, pd, ob):
            def mid(c, g, j):
                r = pl.ds(8 * g, 8)
                m = [pu[c][p1 + here, j, r, :] for p1 in range(7)]
                y = [_gelu2(_res(q, m.__getitem__)) for q in range(4)]
                for p1 in range(7):
                    v = _lhs(p1, y.__getitem__)
                    ta[c, p1, j, r, :] = v
                return v

            def down(b, m, p, c):
                p1, p0 = divmod(p, 7)
                lhs = _lhs(p0, lambda j: ta[c + here, p1, j]).astype(bf16)
                tot = _dot(lhs, jnp.concatenate(
                    [_get(w4t, p, rows=(C4 * c + 128 * k, 128)) for k in range(2)],
                    axis=1))
                m[p0] = m[p0] + tot if c else tot
                if c == NC - 1 and p0 >= 3:
                    j = (2, 1, 3, 0)[p0 - 3]
                    v = _res(j, m.__getitem__)
                    if p1 < 6:
                        pd[p1, j] = v
                    if p1 >= 3:
                        q = (2, 1, 3, 0)[p1 - 3]
                        i, n = _pos(q, j)
                        r0, cols = _mult(b * RB + i * R, R), pl.ds(n * C4, C4)
                        v = _res(q, lambda k: v if k == p1 else pd[k + here, j])
                        ob[pl.ds(r0, R), cols] = (
                            _cols(*[xg[2 * n + k, pl.ds(r0, R), :] for k in range(2)]) + 0.5 * v).astype(bf16)
                return tot

            def out_copy(b):
                rows = pl.ds(_mult(b * RB, RB), RB)
                return pltpu.make_async_copy(ob.at[rows], out_hbm.at[rows],
                                             sems.at[SEM_OUT + b])

            @pl.loop(0, NB)
            def _(b):
                if SKIP & 8:
                    ob[pl.ds(0, 16), pl.ds(0, DH)] = w4t[b, pl.ds(0, 16), :] + ya[0, b, 0, pl.ds(0, 16), :] + (pu[0][b, 0, pl.ds(0, 16), :] + x1b[rows_of(b * 8, 16), pl.ds(0, DH)] + xg[b, pl.ds(0, 16), :]).astype(bf16) + wo_t[b, 0, 0, pl.ds(0, 16), :] + w12[b, pl.ds(0, 16), :]
                    out_copy(b).start()
                    return
                mids = lambda c: _tasks(functools.partial(mid, c), range(R // 8), range(4))
                for c in range(NC):
                    def release(t):
                        pu[c][7, 0, pl.ds(0, 8), :] = pltpu.bitcast(t, f32)

                    _overlap(ups(b + (c + 1) // NC, (c + 1) % NC), mids(c), release, UP_LAG)

                def release(t):
                    hbuf[pl.ds(0, 8), pl.ds(0, DH)] = pltpu.bitcast(t, f32)
                    yn[pl.ds(RB, 8), pl.ds(0, DH)] = pltpu.bitcast(t, f32)

                _overlap(_tasks(functools.partial(down, b, {}), range(49), range(NC)),
                         mlp_in(jnp.minimum(b + 2, NB - 1), b & 1),
                         release, DN_LAG)
                out_copy(b).start()

            for b in range(NB):
                out_copy(b).wait()

        pl.run_scoped(mixer, pltpu.VMEM((9, NC, 4, 64, DH), u32),
                      *[pltpu.VMEM((49, 2, R, DH), bf16)] * 2,
                      *[pltpu.VMEM((2, 8, 4, R, DH), f32)] * 2)
        pl.run_scoped(mlp, pltpu.VMEM((NC, 7, 4, R, 128), f32),
                      pltpu.VMEM((6, 4, R, C4), f32), pltpu.VMEM((S, D), bf16))

    pl.run_scoped(
        block_b,
        pltpu.VMEM((49, C4 * NC, DH), bf16),
        pltpu.VMEM((S, D), f32),
        pltpu.VMEM((RB + 8, D), f32),
        pltpu.VMEM((2, 49, 2, R, DH), bf16),
        *[pltpu.VMEM((8, 4, R, 128), f32)] * 3)


@jax.jit
def pallas_sequential_preLN__memory_aug_recurrent_mem_tr__mixer_s_mlp__prompt_kernel(
    A_x: jax.Array,
    A_mem0: jax.Array,
    A_Wq: jax.Array,
    A_Wk: jax.Array,
    A_Wv: jax.Array,
    A_Wo: jax.Array,
    A_seg_len: jax.Array,
    B_x: jax.Array,
    B_w1: jax.Array,
    B_w2: jax.Array,
    B_w3: jax.Array,
    B_w4: jax.Array,
):
    del A_seg_len, B_x
    hbm = pl.BlockSpec(memory_space=pl.ANY)
    vmem = pl.BlockSpec(memory_space=pltpu.VMEM)
    scratch = [
        pltpu.VMEM((PAD + S, D), f32),
        pltpu.VMEM((8, S + 3 * HALO, DH), f32),
        pltpu.VMEM((7, NP, 4, DH, DH), bf16),
        pltpu.VMEM((6, NP, HS, DH), bf16),
        pltpu.VMEM((3 * HS, HD), f32),
        pltpu.VMEM((NP, 3 * HS, DH), f32),
        pltpu.VMEM((49, S, DH), bf16),
        pltpu.VMEM((49, D, DH), bf16),
        pltpu.SemaphoreType.DMA((NSEM,)),
    ]
    out = pl.pallas_call(
        _kernel,
        out_shape=jax.ShapeDtypeStruct((S, D), A_x.dtype),
        in_specs=[hbm, vmem] + [hbm] * 8,
        out_specs=hbm,
        scratch_shapes=scratch,
        compiler_params=pltpu.CompilerParams(vmem_limit_bytes=127 * 1024 * 1024),
    )(A_x.reshape(S, D), A_mem0.reshape(MEM, D),
      A_Wq.reshape(D // 2, 2 * H, DH), A_Wk.reshape(D // 2, 2 * H, DH),
      A_Wv.reshape(D // 2, 2 * H, DH),
      A_Wo.reshape(H * DH, D), B_w1.reshape(4, C4, D), B_w2.reshape(4, C4, D),
      B_w3.reshape(4, C4, F), B_w4.reshape(NC, 4, FC // 4, D))
    return out.reshape(A_x.shape)
```

```python
import functools

import jax
import jax.numpy as jnp
from jax import lax
import jax.experimental.pallas as pl
import jax.experimental.pallas.tpu as pltpu

S = 2048
D = 1024
H = 32
DH = 128
MEM = 8
SEG = 32
F = 3584
NSEG = S // SEG
L = MEM + SEG
HS = SEG // 2
NP = H // 2
HD = D // 2
PAD = 8
C4 = D // 4
HALO = 8
R = 64
RB = 4 * R
NB = S // RB
FC = 512
NC = F // FC
EPS = 1e-5
NEG = -1000000000.0

LAG_QK = 2
LAG_PV = 4
LAG_WO = 6
FILL_AT = 18
CUTS = (0,2,7,9,14,16,16)
UP_LAG = 8
DN_LAG = 20
MX_LAG = 8
CH0 = 20
CH = 7
DUE = 15
AB = 4
G1 = 7
G2 = 11
EARLY = 9
OUT_AT = 7
M1_CUT = 16
SKIP = 0

GROUPS = ((1, 3), (2, 4), (5, 6))
TARGETS = (((0, 1), (3, 1)), ((2, 1), (3, -1)), ((1, 1), (3, 1)), ((0, 1), (2, 1)),
           ((0, -1), (1, 1)), ((3, 1),), ((0, 1),))

bf16 = jnp.bfloat16
f32 = jnp.float32
u32 = jnp.uint32

SEM_X, SEM_W, SEM_WO, SEM_B, SEM_OUT = 0, 4, 16, 20, 24
NSEM = SEM_OUT + NB


def _mult(i, n):
    return i if isinstance(i, int) else pl.multiple_of(i, n)


def _ln(x):
    m = jnp.mean(x, axis=-1, keepdims=True)
    d = x - m
    v = jnp.mean(d * d, axis=-1, keepdims=True)
    return d * lax.rsqrt(v + EPS)


def _gelu2(x):
    c = 0.7978845608028654
    return x + x * jnp.tanh(x * (c + (c * 0.044715) * (x * x)))


def _get(ref, *idx, rows=None):
    rows = slice(None) if rows is None else pl.ds(rows[0] // 2, rows[1] // 2)
    return _unpack(ref.bitcast(u32)[idx + (rows, slice(None))])


def _cols(*xs):
    return jnp.concatenate(xs, axis=1)


def _unpack(x):
    return pltpu.bitcast(x, bf16)


def _dot(a, b):
    return jnp.dot(a, b, preferred_element_type=f32)


def _rows(*xs):
    return jnp.concatenate(xs, axis=0)


def _lhs(p, a):
    return (lambda: a(0) + a(3), lambda: a(2) + a(3), lambda: a(0), lambda: a(3),
            lambda: a(0) + a(1), lambda: a(2) - a(0), lambda: a(1) - a(3))[p]()


def _rhs(p, b):
    return (lambda: b(0) + b(3), lambda: b(0), lambda: b(1) - b(3), lambda: b(2) - b(0),
            lambda: b(3), lambda: b(0) + b(1), lambda: b(2) + b(3))[p]()


def _res(q, m):
    return (lambda: m(0) + m(3) - m(4) + m(6), lambda: m(2) + m(4),
            lambda: m(1) + m(3), lambda: m(0) - m(1) + m(2) + m(5))[q]()


def _pos(q, j):
    return 2 * (q >> 1) + (j >> 1), 2 * (q & 1) + (j & 1)


def _twice(side, blk, p1):
    outer = [side(p1, lambda q: blk(*_pos(q, j))) for j in range(4)]
    return [side(p0, outer.__getitem__) for p0 in range(7)]


def _ln_tasks(load, store, twice=False, keep=None):
    st = {}

    def fold(x):
        return functools.reduce(
            lambda u, v: u + v, [x[:, c:c + DH] for c in range(0, D, DH)])

    def part():
        st["s"] = fold(load())

    def mean():
        st["m"] = jnp.sum(st["s"], axis=-1, keepdims=True) * (1.0 / D)

    def square():
        d = load() - st["m"]
        st["s"] = fold(d * d)
        if keep:
            keep[...] = d

    def var():
        st["v"] = jnp.sum(st["s"], axis=-1, keepdims=True) * (1.0 / D)

    def scale():
        st["r"] = lax.rsqrt(st["v"] + EPS)

    def again():
        st["r"] = st["r"] * lax.rsqrt(st["v"] * st["r"] * st["r"] + EPS)

    def apply():
        store((keep[...] if keep else load() - st["m"]) * st["r"])

    if twice:
        return [part, mean, square, var, scale, again, apply]
    return [lambda: (part(), mean()), lambda: (square(), var(), scale()), apply]


def _abreast(chains, n):
    return [t for i in range(0, len(chains), n) for ts in zip(*chains[i:i + n]) for t in ts]


def _row_lhs(p, a1, a2):
    return a1 + a2 if p in (1, 4) else a1 if p in (2, 5) else a2


def _row_res(t):
    if 0 not in t:
        return t[2] - t[1], t[1]
    if 1 not in t:
        return t[0], t[2] - t[0]
    return t[0], t[1]


def _merge(*lists):
    order = sorted(((i + 0.5) / len(l), n, i)
                   for n, l in enumerate(lists) for i in range(len(l)))
    return [lists[n][i] for _, n, i in order]


def _interleave(*lists):
    for task in _merge(*lists):
        task()


def _held(spare, tasks):
    return [(spare, task) for task in tasks]


def _overlap(dots, side, lag):
    for i, dot in enumerate(dots):
        _release(dot(), _share(side, i, len(dots) - lag))


def _release(result, mine):
    for spare in {id(spare): spare for spare, _ in mine}.values():
        spare[...] = pltpu.bitcast(result[-8:, -DH:], spare.dtype)
    for _, task in mine:
        task()


def _share(tasks, k, n):
    return tasks[len(tasks) * k // n:len(tasks) * (k + 1) // n] if k >= 0 else []


def _tasks(fn, *ranges):
    if len(ranges) == 2:
        return [functools.partial(fn, i, j) for i in ranges[0] for j in ranges[1]]
    return [functools.partial(fn, i) for i in ranges[0]]


def _start(copies):
    for c in copies:
        c.start()


def _wait(copies):
    for c in copies:
        c.wait()


def _scores(q, k):
    return lax.dot_general(q, k, (((1,), (1,)), ((), ())), preferred_element_type=f32)


def _attend(sc, v):
    ri = lax.broadcasted_iota(jnp.int32, (L, L), 0)
    ci = lax.broadcasted_iota(jnp.int32, (L, L), 1)
    sc = jnp.where((ri < MEM) | (ri >= ci), sc * (DH ** -0.5), NEG)
    mx = jnp.max(sc, axis=1, keepdims=True)
    e = jnp.exp(sc - mx)
    den = jnp.sum(e, axis=1, keepdims=True)
    inv = pl.reciprocal(den, approx=True)
    inv = inv * (2.0 - den * inv)
    return _dot(e, v) * inv


def _kernel(x_hbm, mem0_ref, wq_hbm, wk_hbm, wv_hbm, wo_hbm, w1_hbm, w2_hbm,
            w3_hbm, w4_hbm, out_hbm, hbuf, xg, wo_t, o1, ocar, m1, w12, sems):
    w_hbm = (wq_hbm, wk_hbm, wv_hbm)
    here = lax.fori_loop(0, 2, lambda i, z: z + (i >> 1), jnp.int32(0))

    def b_copies(raw):
        tile = lambda w, i: w.bitcast(u32).at[:, :, pl.ds(128 * i, 128)]
        for n in range(4):
            slabs = pl.ds(4 * n, 4)
            for i, w in enumerate((w1_hbm, w2_hbm)):
                for c in range(2):
                    yield pltpu.make_async_copy(
                        tile(w, 2 * n + c),
                        raw.at[slabs, pl.ds(128 * (NC + 2 * i + c), 128)],
                        sems.at[SEM_B])
            for c in range(NC):
                yield pltpu.make_async_copy(
                    tile(w3_hbm, 4 * c + n), raw.at[slabs, pl.ds(128 * c, 128)],
                    sems.at[SEM_B])

    def b_operands(raw, dst, r1, p1):
        for p0, v in enumerate(_twice(_rhs, lambda k, n: _unpack(raw(k, n)).astype(f32), p1)):
            if p1 in (1, 4) and p0 in (1, 4):
                k = 2 * (p1 // 4) + p0 // 4
                dst.bitcast(u32)[7 * p1 + p0, pl.ds(r1, 8), :] = raw(k, k)
            else:
                dst[7 * p1 + p0, pl.ds(_mult(2 * r1, 16), 16), :] = v.astype(bf16)

    def rows_of(r0, n):
        return pl.ds(pl.multiple_of(r0 + here, 8), n)

    def put(rows, x):
        for c in range(8):
            xg[c, rows, :] = x[:, DH * c:DH * (c + 1)]

    def wo_tile(p, a):
        return _cols(*[_get(wo_t, p, a, c) for c in range(4)])

    def seg_quads(s):
        r0 = HALO + s * SEG
        return [jnp.concatenate(
            [xg[4 * (q & 1) + c, pl.ds(_mult(r0 + (q >> 1) * HS, 8), HS), :]
             for c in range(4)], axis=1) for q in range(4)]

    def heads_of(c_mem, m):
        return [_rows(c_mem[n], _res(n, m.__getitem__), _res(2 + n, m.__getitem__))
                for n in range(2)]

    def wo_pass(phase, a, o, prev, o1_slot):
        whole, part = GROUPS[(phase + 1) % 3], GROUPS[(phase + 2) % 3]
        quad = lambda q: o[q & 1][MEM + (q >> 1) * HS:MEM + (q >> 1) * HS + HS]
        x = [_lhs(p, quad) for p in range(7)]
        o1[o1_slot, a] = x[0].astype(bf16)
        ocar[a] = _rows(*[x[p] for p in GROUPS[phase]], *[x[p][8:] for p in part])
        res = {}
        for k in range(2):
            for p, riders in ((whole[k], (prev[SEG + 8 * k:SEG + 8 * k + 8], x[whole[k]])),
                              (part[k], (x[part[k]][:8], prev[HS * k:HS * k + HS]))):
                lhs = _rows(_row_lhs(p, o[0][:MEM], o[1][:MEM]), *riders)
                res[p] = _dot(lhs.astype(bf16), wo_tile(p, a))
        return res

    def add_h(s, terms):
        for q in range(4):
            for z in range(2):
                mine = [(sign, v) for p, zz, v in terms if zz == z
                        for qq, sign in TARGETS[p] if qq == q]
                if mine:
                    at = (pl.ds(_mult(PAD + s * SEG + (q >> 1) * HS + 8 * z, 8), 8),
                          pl.ds((q & 1) * HD, HD))
                    acc = hbuf[at]
                    for sign, v in mine:
                        acc = acc + v if sign > 0 else acc - v
                    hbuf[at] = acc

    def wo_finish(phase, s, tot, first=False):
        gw, gp = (phase + 1) % 3, (phase + 2) % 3
        whole, part = GROUPS[gw], GROUPS[gp]
        mem = _row_res({g: tot[GROUPS[g][0]][:MEM] + tot[GROUPS[g][1]][:MEM]
                        for g in (gw, gp)})
        if not first:
            add_h(s - 1, [(p, 1, tot[p][8:16]) for p in whole]
                  + [(p, z, tot[p][16 + 8 * z:24 + 8 * z]) for p in part for z in range(2)])
        add_h(s, [(p, 0, tot[p][8:16]) for p in part]
              + [(p, z, tot[p][16 + 8 * z:24 + 8 * z]) for p in whole for z in range(2)])
        return mem

    def wo_m1(slot, pairs):
        lhs = jnp.concatenate(
            [_rows(*[_get(o1, slot + k, a) for k in range(3)]) for a in pairs], axis=1)
        return _dot(lhs, _rows(*[wo_tile(0, a) for a in pairs]))

    def add_m1(s, r):
        for k in range(3):
            add_h(jnp.maximum(s + k, 0),
                  [(0, z, r[HS * k + 8 * z:HS * k + 8 * z + 8]) for z in range(2)])

    def mixer_norm(r0, keep=None):
        return _ln_tasks(lambda: hbuf[rows_of(PAD + r0, HS), :],
                         functools.partial(put, rows_of(HALO + r0, HS)), True, keep)

    def prologue(wt, qcar, stg, words, lhs1, lhs0, qkv0):
        def row_copy(src, i, n, sem):
            rows = pl.ds(_mult(i * n, n), n)
            return pltpu.make_async_copy(src.bitcast(u32).at[rows], words.at[rows],
                                         sems.at[sem + i])

        x_copy = lambda i: row_copy(x_hbm, i, S // 8, SEM_X)
        wo_copy = lambda g: row_copy(wo_hbm, g, 512, SEM_WO)

        def start_chunk(g, m):
            src = w_hbm[m].bitcast(u32)
            dst = stg.reshape(3 * HD, 8, DH)
            for par in range(2):
                pltpu.make_async_copy(
                    src.at[:, pl.ds(_mult(16 * par + 4 * g, 4), 4), :],
                    dst.at[pl.ds(HD * m, HD), pl.ds(4 * par, 4), :],
                    sems.at[SEM_W + 3 * g + m]).start()

        def wait_chunk(g, m):
            part = stg.at[pl.ds(_mult(4 * D * m, 4 * D), 4 * D)]
            pltpu.make_async_copy(part, part, sems.at[SEM_W + 3 * g + m]).wait()

        def operands(g, m, pair, i):
            w = [stg[pl.ds(4 * (D * m + HD * k + 16 * i) + pair, 16, stride=4), :]
                 for k in range(2)]
            quad = [pltpu.bitcast(w[q >> 1] & jnp.uint32(0xFFFF0000) if q & 1
                                  else w[q >> 1] << 16, f32) for q in range(4)]
            wt[3 * NP + m, pair, pl.ds(16 * i, 16), :] = _rhs(0, quad.__getitem__).astype(bf16)
            for p in range(1, 7):
                wt[NP * m + 4 * g + pair, p - 1, pl.ds(16 * i, 16), :] = _rhs(
                    p, quad.__getitem__).astype(bf16)

        def wo_operands(g, pair, i):
            c, r0 = i & 3, 8 * (i >> 2)
            w = [words[rows_of(DH * (4 * g + pair) + DH // 2 * (q >> 1) + r0, 8),
                       pl.ds(HD * (q & 1) + DH * c, DH)] for q in range(4)]
            quad = [_unpack(v).astype(f32) for v in w]
            for p in range(7):
                v = _rhs(p, quad.__getitem__).astype(bf16)
                wo_t[p, 4 * g + pair, c, pl.ds(2 * r0, 16), :] = v

        start_chunk(0, 0)
        for i in range(4):
            x_copy(i).start()
        start_chunk(0, 1)
        start_chunk(0, 2)
        for r0 in (0, HALO + S):
            put(pl.ds(r0, HALO), jnp.zeros((HALO, D), f32))
        for k in range(2):
            o1[k] = jnp.zeros((NP, HS, DH), bf16)
        wait_chunk(0, 0)

        @pl.loop(0, 4)
        def _(pair):
            for i in range(HD // 16):
                operands(0, 0, pair, i)

        @pl.loop(0, 4)
        def _(i):
            x_copy(i).wait()

            @pl.loop(0, 4)
            def _(k):
                r0 = pl.multiple_of(i * (S // 4) + k * 128, 128)
                xv = _unpack(words[pl.ds(pl.multiple_of(r0 // 2, 64), 64), :]).astype(f32)
                hbuf[pl.ds(PAD + r0, 128), :] = xv
                xn = _ln(xv)
                put(pl.ds(HALO + r0, 128), xn)
                v = _rows(*[xn[z:z + HS, :HD] + xn[z + HS:z + SEG, HD:]
                            for z in range(0, 128, SEG)])
                for c in range(4):
                    lhs1[c, pl.ds(pl.multiple_of(r0 // 2, 64), 64), :] = (
                        v[:, DH * c:DH * (c + 1)].astype(bf16))

        mem = mem0_ref[...].astype(f32)
        cur, nxt = seg_quads(0), seg_quads(1)
        for p in range(1, 7):
            x0, x1 = _lhs(p, cur.__getitem__), _lhs(p, nxt.__getitem__)
            v = (_rows(x0, x1) if p in GROUPS[1]
                 else _rows(_row_lhs(p, mem[:, :HD], mem[:, HD:]), x1[:8], x0))
            for c in range(4):
                lhs0[p - 1, c] = v[:, DH * c:DH * (c + 1)].astype(bf16)

        def first(g, m, pair, i):
            n = S // 2 // M1_CUT
            lhs = _cols(*[_get(lhs1, c, rows=(n * i, n)) for c in range(4)])
            r = pltpu.bitcast(_dot(lhs, _get(wt, 3 * NP + m + here, pair)), u32)
            m1.bitcast(u32)[NP * m + 4 * g + pair, pl.ds(n * i, n), :] = r
            return r

        def project(g, m, pair):
            a = 4 * g + pair
            r = {p: _dot(_cols(*[_get(lhs0, p - 1, c) for c in range(4)]),
                         _get(wt, NP * m + a, p - 1))
                 for p in range(1, 7)}
            prod = {p: r[p][:HS] if p in GROUPS[1] else r[p][HS:] for p in r}
            prod[0] = pltpu.bitcast(m1.bitcast(u32)[NP * m + a, pl.ds(0, HS), :], f32)
            qcar[m, a] = _rows(*[r[p][HS:] for p in GROUPS[1]],
                               *[r[p][8:16] for p in GROUPS[2]])
            c_mem = _row_res({k: r[GROUPS[k][0]][:MEM] + r[GROUPS[k][1]][:MEM]
                              for k in (0, 2)})
            for n, v in enumerate(heads_of(c_mem, prod)):
                qkv0[m, a, n] = v

        def wo_tasks(g):
            return _held(words.at[pl.ds(H * DH // 2, 8), pl.ds(0, DH)],
                         _tasks(functools.partial(wo_operands, g), range(4), range(32)))

        def dots(g, m):
            return _tasks(functools.partial(first, g, m), range(4), range(M1_CUT))

        @pl.loop(0, 11)
        def _(c):
            g, g2 = lax.div(c, 3), lax.div(c + 1, 3)
            m, m2 = c - 3 * g, c + 1 - 3 * g2
            for k in range(3):
                pl.when((m == k) & (g < 3))(functools.partial(start_chunk, g + 1, k))
            pl.when(c == 9)(lambda: _start([wo_copy(k) for k in range(4)]))
            wait_chunk(g2, m2)
            _interleave(_tasks(functools.partial(operands, g2, m2), range(4), range(HD // 16)),
                        dots(g, m))
            for pair in range(4):
                project(g, m, pair)

        for k in range(2):
            wo_copy(k).wait()
            _overlap(_share(dots(3, 2), k, 2), wo_tasks(k), 2)

        scores, outs, tot = {}, {}, {}
        none = jnp.zeros((3 * HS, DH), f32)

        def step0(t):
            if t < NP:
                scores[t] = [_scores(qkv0[0, t, n], qkv0[1, t, n]) for n in range(2)]
            if 0 <= t - 2 < NP:
                outs[t - 2] = [_attend(scores[t - 2][n], qkv0[2, t - 2, n]) for n in range(2)]
            if 0 <= t - 4 < NP:
                for p, r in wo_pass(0, t - 4, outs[t - 4], none, 2).items():
                    tot[p] = tot[p] + r if p in tot else r
                return r
            project(3, 2, t)
            return qkv0[0, t, 0]

        for k, slots in ((2, range(12)), (3, range(12, 16))):
            wo_copy(k).wait()
            _overlap(_tasks(step0, slots), wo_tasks(k), 1)
        _interleave(_tasks(step0, range(16, 20)))
        return wo_finish(0, 0, tot, first=True)

    def step(wt, qcar, s, phase, cur, nxt, first, mem, o1_slot, fillers, chores):
        gw, gp = (phase + 1) % 3, (phase + 2) % 3
        ahead, now = GROUPS[gw], GROUPS[gp]
        lhs = {}
        for p in ahead + now:
            x0, x1 = _lhs(p, cur.__getitem__), _lhs(p, nxt.__getitem__)
            riders = (x0[8:], x1) if p in ahead else (x1[:8], x0)
            lhs[p] = _rows(_row_lhs(p, *mem), *riders).astype(bf16)
        heads, scores, outs, tot = {}, {}, {}, {}

        def qkv(a):
            heads[a] = []
            for m in range(3):
                r = {p: _dot(lhs[p], _get(wt, NP * m + a, p - 1)) for p in lhs}
                _release(r[now[1]], _share(chores, 3 * a + m, 3 * NP - CH0))
                old = qcar[m, a]
                prod = {0: pltpu.bitcast(first(NP * m + a), f32)}
                for k in range(2):
                    prod[GROUPS[phase][k]] = old[HS * k:HS * k + HS]
                    prod[ahead[k]] = _rows(old[SEG + 8 * k:SEG + 8 * k + 8],
                                           r[ahead[k]][8:16])
                    prod[now[k]] = r[now[k]][HS:]
                qcar[m, a] = _rows(*[r[p][HS:] for p in ahead], *[r[p][8:16] for p in now])
                c_mem = _row_res({g: r[GROUPS[g][0]][:MEM] + r[GROUPS[g][1]][:MEM]
                                  for g in (gw, gp)})
                heads[a].append(heads_of(c_mem, prod))

        for t in range(NP + LAG_WO):
            a = t - LAG_QK
            if 0 <= a < NP:
                scores[a] = [_scores(heads[a][0][n], heads[a][1][n]) for n in range(2)]
            a = t - LAG_PV
            if 0 <= a < NP:
                outs[a] = [_attend(scores[a][n], heads[a][2][n]) for n in range(2)]
            if t < NP:
                qkv(t)
            if t == FILL_AT:
                fillers[0]()
            a = t - LAG_WO
            if 0 <= a < NP:
                for p, r in wo_pass(phase, a, outs[a], ocar[a], o1_slot).items():
                    tot[p] = tot[p] + r if p in tot else r
        fillers[1]()
        return wo_finish(phase, s, tot)

    def recurrence(wt, qcar, mem, raw, fin):
        _start(b_copies(raw))
        spare = 128 * (NC + 4)
        raw[pl.ds(0, 16), pl.ds(spare, 8), :] = jnp.zeros((16, 8, DH), u32)

        def chores(i):
            def convert(dst, base, per, groups):
                tasks = []
                for k in range(per):
                    r = pl.multiple_of(8 * jnp.clip(per * (i - 2) + k, 0, groups - 1), 8)
                    r0 = pl.multiple_of(jnp.where(i > 1, base + r, spare), 8)
                    tasks += _tasks(functools.partial(
                        b_operands, lambda k, n, r0=r0: raw[4 * n + k, pl.ds(r0, 8), :],
                        dst, r), range(7))
                return _held(raw.at[16, pl.ds(0, 8)], tasks)
            rest = convert(w12, 128 * NC, 4, 64)
            norm = _abreast(
                [mixer_norm(jnp.maximum(3 * i - 5 + (k >> 1), 0) * SEG + (k & 1) * HS,
                            fin.at[rows_of(HS * k, HS)])
                 for k in range(6)], 6)
            in_h = hbuf.at[pl.ds(0, 8), pl.ds(0, DH)]
            norm = (_held(in_h, norm[:12]), _held(in_h, norm[12:36]),
                    _held(fin.at[pl.ds(3 * SEG, 8), pl.ds(0, DH)], norm[36:]))

            def due():
                m1.bitcast(u32)[3 * NP + here, pl.ds(S // 2 - 8, 8), :] = pltpu.bitcast(
                    xg[here, pl.ds(0, 8), :], u32)
            norm[2].append((norm[2][0][0], due))
            return [_merge(t, n)
                    for t, n in zip((_share(rest, 0, 2), _share(rest, 1, 2),
                                     convert(m1, 0, 6, 16 * NC)), norm)]

        def steps(i, mem):
            pl.when(i == 2)(lambda: _wait(b_copies(raw)))
            src = 3 * (i & 1)
            acc = []

            def filler(n):
                if CUTS[n] < CUTS[n + 1]:
                    acc.append(wo_m1(src, range(CUTS[n], CUTS[n + 1])))
                    if CUTS[n + 1] == NP:
                        add_m1(3 * i - 2, functools.reduce(lambda u, v: u + v, acc))

            todo = [t if CH >> k & 1 else [] for k, t in enumerate(chores(i))]
            nxt = seg_quads(3 * i + 1)
            for k in range(3):
                fillers = _tasks(filler, (2 * k, 2 * k + 1))
                rows = pl.ds(pl.multiple_of((3 * i + 1 + k) * HS, HS), HS)
                first = lambda j: m1.bitcast(u32)[j, rows, :]
                if k == 2:
                    early = {j: first(j) for j in range(3 * NP) if j % NP < DUE}
                    first = lambda j, late=first: early[j] if j in early else late(j)
                cur, nxt = nxt, seg_quads(jnp.minimum(3 * i + 2 + k, NSEG - 1))
                mem = step(wt, qcar, 3 * i + 1 + k, (1 + k) % 3, cur, nxt, first, mem,
                           3 - src + k, fillers, todo[k])
            return mem

        if not SKIP & 2:
            lax.fori_loop(0, NSEG // 3, steps, mem)
        else:
            _wait(b_copies(raw))

    def block_a(wt, qcar):
        if SKIP & 1:
            mem = (mem0_ref[:, :HD].astype(f32), mem0_ref[:, HD:].astype(f32))
        else:
            mem = pl.run_scoped(
                functools.partial(prologue, wt, qcar),
                pltpu.VMEM((12 * D, DH), u32),
                pltpu.VMEM((H * DH // 2 + 8, D), u32),
                pltpu.VMEM((4, S // 2, DH), bf16),
                pltpu.VMEM((6, 4, SEG, DH), bf16),
                pltpu.VMEM((3, NP, 2, L, DH), f32))

        pl.run_scoped(functools.partial(recurrence, wt, qcar, mem),
                      pltpu.VMEM((17, 128 * (NC + 4) + 8, DH), u32),
                      pltpu.VMEM((3 * SEG + 8, D), f32))

    pl.run_scoped(block_a, pltpu.VMEM((3 * NP + 3, 6, HD, DH), bf16),
                  pltpu.VMEM((3, NP, 3 * HS, DH), f32))

    def block_b(w4t, x1b, yn, ya, *pu):
        in_h = hbuf.at[pl.ds(0, 8), pl.ds(0, DH)]
        in_y = yn.at[pl.ds(RB, 8), pl.ds(0, DH)]
        pu = [pu[(0, 1, 2, 0, 1, 2, 1)[c]] for c in range(NC)]
        def wo_last():
            phase = NSEG % 3
            tot = {}

            def task(a0, p, r0=0, n=0):
                pairs = range(a0, a0 + 2)
                if p == 0:
                    r = wo_m1(3 * (NSEG // 3 & 1), pairs)
                else:
                    lhs = _cols(*[ocar[a, pl.ds(r0, n), :] for a in pairs])
                    r = _dot(lhs.astype(bf16), _rows(*[wo_tile(p, a) for a in pairs]))
                tot[p] = tot[p] + r if a0 else r
                if a0 == NP - 2 and p == 0:
                    add_m1(NSEG - 3, tot[p])
                elif a0 == NP - 2:
                    add_h(NSEG - 1, [(p, 1, tot[p][-8:])] + [(p, 0, tot[p][:8])] * (n > 8))
                return r

            todo = [(0,)] + [t for k in range(2) for t in (
                (GROUPS[(phase + 2) % 3][k], HS * k, HS),
                (GROUPS[(phase + 1) % 3][k], SEG + 8 * k, 8))]
            return [functools.partial(task, a0, *t) for t in todo for a0 in range(0, NP, 2)]

        def a_operands(load, dst):
            def task(g, p1):
                r0, c = 16 * (g >> 1), g & 1
                for p0, v in enumerate(_twice(
                        _lhs, lambda i, k: load(i * R + r0, 2 * k + c), p1)):
                    dst[7 * p1 + p0, c, pl.ds(r0, 16), :] = v.astype(bf16)
            return _tasks(task, range(R // 8), range(7))

        def products(src, w, r0, dst):
            m = {}

            def task(p1, p0):
                p = 7 * p1 + p0
                m[p0] = _dot(_cols(*[_get(src, p + here, k) for k in range(2)]),
                             _get(w, p, rows=(r0, C4)))
                if p0 >= 3:
                    j = (2, 1, 3, 0)[p0 - 3]
                    dst[p1, j] = _res(j, m.__getitem__)
                return m[p0]
            return _tasks(task, range(7), range(7))

        def mlp_in(b):
            def residual(r0, y):
                x1 = y + x1b[rows_of(b * RB + r0, 16), :]
                yn[pl.ds(r0, 16), :] = x1
                put(rows_of(b * RB + r0, 16), hbuf[rows_of(PAD + b * RB + r0, 16), :] + x1)

            def store(r0, y):
                yn[pl.ds(r0, 16), :] = y
                return y

            chains = [
                _held(in_h, _ln_tasks(lambda r0=r0: hbuf[rows_of(PAD + b * RB + r0, 16), :],
                                      functools.partial(residual, r0)))
                + _held(in_y, _ln_tasks(lambda r0=r0: yn[rows_of(r0, 16), :],
                                        functools.partial(store, r0)))
                for r0 in range(0, RB, 16)]
            return _abreast(chains, AB) + _held(in_y, a_operands(
                lambda r0, c: yn[rows_of(r0, 16), pl.ds(DH * c, DH)], ya))

        def ups(c):
            return products(ya, m1, C4 * c, pu[c])

        def mixer(raw, *bufs):
            sa, sp = bufs[:2], bufs[2:]
            in_g = xg.at[0, pl.ds(S + 2 * HALO, 8)]
            w4_copies = [pltpu.make_async_copy(
                w4_hbm.bitcast(u32).at[pl.ds(c, n), :, :, pl.ds(DH * i, DH)],
                raw.at[i, pl.ds(c, n)], sems.at[SEM_B + s])
                for c, n, s in ((0, 2, 1), (2, NC - 2, 3)) for i in range(8)]
            _start(w4_copies)

            def pre(n, w, b):
                shift = lambda c: w * (-1, 1, -2, 2)[c >> 1]
                return _held(in_g, a_operands(lambda r0, c: xg[c + here, pl.ds(
                    HALO + b * RB + r0 + shift(c), 16), :], sa[n & 1]))

            def post(n, w, b):
                def task(g, j):
                    c = g & 1
                    m = [sp[n & 1][c + here, p1, j, pl.ds(8 * (g >> 1), 8), :]
                         for p1 in range(7)]
                    for q in range(4):
                        i, k = _pos(q, j)
                        r0 = _mult(b * RB + i * R + 8 * (g >> 1), 8)
                        v = _res(q, m.__getitem__)
                        if w == 0:
                            xg[2 * k + c, pl.ds(HALO + r0, 8), :] = _gelu2(v)
                        else:
                            x1b[pl.ds(r0, 8), pl.ds(DH * (2 * k + c), DH)] = 0.5 * v
                return _held(sp[n & 1].at[0, 7, 0, pl.ds(0, 8)],
                             _tasks(task, range(R // 4), range(4)))

            def unit(n, w, *side):
                dots = [t for c in range(2) for t in products(
                    sa[n & 1], w12, C4 * (2 * w + c), sp[n & 1].at[c])]
                _overlap(dots, _merge(*side), MX_LAG)

            def w4_work(k, n):
                def task(i, p1):
                    g = k + i
                    b_operands(lambda q, c: raw[2 * c + ((g >> 3) & 1) + here, g >> 4, q,
                                                pl.ds(_mult(8 * (g & 7), 8), 8), :],
                               w4t, _mult(8 * g, 8), p1)
                return _held(raw.at[8, 0, 0, pl.ds(0, 8)], _tasks(task, range(n), range(7)))

            if not SKIP & 4:
                norms = lambda s: _held(in_h, _abreast(
                    [mixer_norm(s * SEG + k * HS) for k in range(6)], 3))
                _overlap(wo_last(), _merge(pre(0, 0, 0), norms(NSEG - 6)), MX_LAG)
                unit(0, 0, pre(1, 0, 1), norms(NSEG - 3))
                _wait(w4_copies[:8])

                @pl.loop(0, 3)
                def _(i):
                    pl.when(i == 2)(lambda: _wait(w4_copies[8:]))
                    for n in range(2):
                        b = 2 * i + 1 + n
                        unit(n + 1, 0, pre(n, 0, b + 1), post(n, 0, b - 1),
                             w4_work(G1 * (b - 1), G1))

                unit(1, 0, pre(0, 1, 0), post(0, 0, 6), w4_work(6 * G1, G1))
                unit(0, 1, pre(1, 1, 1), post(1, 0, 7), w4_work(7 * G1, G1))

                @pl.loop(0, 2)
                def _(i):
                    for n in range(2):
                        b = 2 * i + 1 + n
                        unit(n + 1, 1, pre(n, 1, b + 1), post(n, 1, b - 1),
                             w4_work(8 * G1 + G2 * (b - 1), G2))

                done = 8 * G1 + 4 * G2
                rest = w4_work(done, 16 * NC - done)
                ahead = mlp_in(0)
                for b in range(5, NB):
                    unit(b, 1, pre(b + 1, 1, b + 1) if b + 1 < NB else _share(rest, 2, 5),
                         post(b - 1, 1, b - 1), _share(ahead, b - 5, 3),
                         _share(rest, (0, 1, 3)[b - 5], 5))
                _overlap(ups(0), _merge(post(1, 1, 7), _share(rest, 4, 5)),
                         MX_LAG)
            else:
                _wait(w4_copies)

        def mlp(ta0, ta1, pd, ob):
            ta = [ta0.at[c] for c in range(NC - 1)] + [ta1]

            def mid(c, g, j):
                r = pl.ds(8 * g, 8)
                m = [pu[c][p1 + here, j, r, :] for p1 in range(7)]
                y = [_gelu2(_res(q, m.__getitem__)) for q in range(4)]
                for p1 in range(7):
                    v = _lhs(p1, y.__getitem__)
                    ta[c][p1, j, r, :] = v
                return v

            def down(b, m, p, c):
                p1, p0 = divmod(p, 7)
                lhs = _lhs(p0, lambda j: ta[c][p1 + here, j]).astype(bf16)
                tot = _dot(lhs, jnp.concatenate(
                    [_get(w4t, p, rows=(C4 * c + 128 * k, 128)) for k in range(2)],
                    axis=1))
                m[p] = m[p] + tot if c else tot
                if c == NC - 1 and p0 >= 3:
                    j = (2, 1, 3, 0)[p0 - 3]
                    v = _res(j, lambda k: m[7 * p1 + k])
                    if p1 < 6:
                        pd[p1, j] = v
                    if p1 >= 3:
                        q = (2, 1, 3, 0)[p1 - 3]
                        i, n = _pos(q, j)
                        r0, cols = _mult(b * RB + i * R, R), pl.ds(n * C4, C4)
                        v = _res(q, lambda k: v if k == p1 else pd[k + here, j])
                        ob[pl.ds(r0, R), cols] = (
                            _cols(*[xg[2 * n + k, pl.ds(r0, R), :] for k in range(2)]) + 0.5 * v).astype(bf16)
                return tot

            def out_copy(b):
                rows = pl.ds(_mult(b * RB, RB), RB)
                return pltpu.make_async_copy(ob.at[rows], out_hbm.at[rows],
                                             sems.at[SEM_OUT + b])

            @pl.loop(0, NB)
            def _(b):
                if SKIP & 8:
                    ob[pl.ds(0, 16), pl.ds(0, DH)] = w4t[b, pl.ds(0, 16), :] + ya[b, 0, pl.ds(0, 16), :] + (pu[0][b, 0, pl.ds(0, 16), :] + x1b[rows_of(b * 8, 16), pl.ds(0, DH)] + xg[b, pl.ds(0, 16), :]).astype(bf16) + wo_t[b, 0, 0, pl.ds(0, 16), :] + w12[b, pl.ds(0, 16), :]
                    out_copy(b).start()
                    return
                mids = lambda c: _held(pu[c].at[7, 0, pl.ds(0, 8)], _tasks(
                    functools.partial(mid, c), range(R // 8), range(4)))
                task = functools.partial(down, b, {})
                early = _tasks(task, range(EARLY), range(NC - 1))
                for c in range(NC):
                    _overlap(ups(c + 1) if c + 1 < NC else early, mids(c), UP_LAG)

                _overlap(_tasks(task, range(EARLY), [NC - 1])
                         + _tasks(task, range(EARLY, 49), range(NC)),
                         mlp_in(jnp.minimum(b + 1, NB - 1)), DN_LAG)
                _interleave(ups(0)[:OUT_AT])
                out_copy(b).start()
                _interleave(ups(0)[OUT_AT:])

            for b in range(NB):
                out_copy(b).wait()

        pl.run_scoped(mixer, pltpu.VMEM((9, NC, 4, 64, DH), u32),
                      *[pltpu.VMEM((49, 2, R, DH), bf16)] * 2,
                      *[pltpu.VMEM((2, 8, 4, R, DH), f32)] * 2)
        pl.run_scoped(mlp, pltpu.VMEM((NC - 1, 7, 4, R, DH), f32),
                      pltpu.VMEM((7, 4, R, DH), f32),
                      pltpu.VMEM((6, 4, R, C4), f32), pltpu.VMEM((S, D), bf16))

    pl.run_scoped(
        block_b,
        pltpu.VMEM((49, C4 * NC, DH), bf16),
        pltpu.VMEM((S, D), f32),
        pltpu.VMEM((RB + 8, D), f32),
        pltpu.VMEM((49, 2, R, DH), bf16),
        *[pltpu.VMEM((8, 4, R, 128), f32)] * 3)


@jax.jit
def pallas_sequential_preLN__memory_aug_recurrent_mem_tr__mixer_s_mlp__prompt_kernel(
    A_x: jax.Array,
    A_mem0: jax.Array,
    A_Wq: jax.Array,
    A_Wk: jax.Array,
    A_Wv: jax.Array,
    A_Wo: jax.Array,
    A_seg_len: jax.Array,
    B_x: jax.Array,
    B_w1: jax.Array,
    B_w2: jax.Array,
    B_w3: jax.Array,
    B_w4: jax.Array,
):
    del A_seg_len, B_x
    hbm = pl.BlockSpec(memory_space=pl.ANY)
    vmem = pl.BlockSpec(memory_space=pltpu.VMEM)
    scratch = [
        pltpu.VMEM((PAD + S, D), f32),
        pltpu.VMEM((8, S + 3 * HALO, DH), f32),
        pltpu.VMEM((7, NP, 4, DH, DH), bf16),
        pltpu.VMEM((6, NP, HS, DH), bf16),
        pltpu.VMEM((NP, 3 * HS, DH), f32),
        pltpu.VMEM((49, S, DH), bf16),
        pltpu.VMEM((49, D, DH), bf16),
        pltpu.SemaphoreType.DMA((NSEM,)),
    ]
    out = pl.pallas_call(
        _kernel,
        out_shape=jax.ShapeDtypeStruct((S, D), A_x.dtype),
        in_specs=[hbm, vmem] + [hbm] * 8,
        out_specs=hbm,
        scratch_shapes=scratch,
        compiler_params=pltpu.CompilerParams(vmem_limit_bytes=127 * 1024 * 1024),
    )(A_x.reshape(S, D), A_mem0.reshape(MEM, D),
      A_Wq.reshape(D // 2, 2 * H, DH), A_Wk.reshape(D // 2, 2 * H, DH),
      A_Wv.reshape(D // 2, 2 * H, DH),
      A_Wo.reshape(H * DH, D), B_w1.reshape(4, C4, D), B_w2.reshape(4, C4, D),
      B_w3.reshape(4, C4, F), B_w4.reshape(NC, 4, FC // 4, D))
    return out.reshape(A_x.shape)
```

```python
import functools

import jax
import jax.numpy as jnp
from jax import lax
import jax.experimental.pallas as pl
import jax.experimental.pallas.tpu as pltpu

S = 2048
D = 1024
H = 32
DH = 128
MEM = 8
SEG = 32
F = 3584
NSEG = S // SEG
L = MEM + SEG
HS = SEG // 2
NP = H // 2
HD = D // 2
PAD = 8
C4 = D // 4
HALO = 8
R = 64
RB = 4 * R
NB = S // RB
FC = 512
NC = F // FC
EPS = 1e-5
NEG = -1000000000.0

LAG_QK = 2
LAG_PV = 4
LAG_WO = 6
FILL_AT = 18
CUTS = (0, 1, 3, 8, 10, 14, 16, 16)
CH0 = 20
DUE = 15
M1_CUT = 16
G1 = 7
G2 = 12
A0 = 32
AH = 96
EARLY = 11
MX_LAG = 8
UP_LAG = 10
DN_LAG = 20

GROUPS = ((1, 3), (2, 4), (5, 6))
TARGETS = (((0, 1), (3, 1)), ((2, 1), (3, -1)), ((1, 1), (3, 1)), ((0, 1), (2, 1)),
           ((0, -1), (1, 1)), ((3, 1),), ((0, 1),))

bf16 = jnp.bfloat16
f32 = jnp.float32
u32 = jnp.uint32

SEM_X, SEM_W, SEM_WO, SEM_B, SEM_OUT = 0, 4, 16, 20, 24
NSEM = SEM_OUT + NB


def _mult(i, n):
    return i if isinstance(i, int) else pl.multiple_of(i, n)


def _ln(x):
    m = jnp.mean(x, axis=-1, keepdims=True)
    d = x - m
    v = jnp.mean(d * d, axis=-1, keepdims=True)
    return d * lax.rsqrt(v + EPS)


def _gelu2(x):
    c = 0.7978845608028654
    return x + x * jnp.tanh(x * (c + (c * 0.044715) * (x * x)))


def _get(ref, *idx, rows=None):
    rows = slice(None) if rows is None else pl.ds(rows[0] // 2, rows[1] // 2)
    return _unpack(ref.bitcast(u32)[idx + (rows, slice(None))])


def _cols(*xs):
    return jnp.concatenate(xs, axis=1)


def _unpack(x):
    return pltpu.bitcast(x, bf16)


def _dot(a, b):
    return jnp.dot(a, b, preferred_element_type=f32)


def _rows(*xs):
    return jnp.concatenate(xs, axis=0)


def _lhs(p, a):
    return (lambda: a(0) + a(3), lambda: a(2) + a(3), lambda: a(0), lambda: a(3),
            lambda: a(0) + a(1), lambda: a(2) - a(0), lambda: a(1) - a(3))[p]()


def _rhs(p, b):
    return (lambda: b(0) + b(3), lambda: b(0), lambda: b(1) - b(3), lambda: b(2) - b(0),
            lambda: b(3), lambda: b(0) + b(1), lambda: b(2) + b(3))[p]()


def _res(q, m):
    return (lambda: m(0) + m(3) - m(4) + m(6), lambda: m(2) + m(4),
            lambda: m(1) + m(3), lambda: m(0) - m(1) + m(2) + m(5))[q]()


def _pos(q, j):
    return 2 * (q >> 1) + (j >> 1), 2 * (q & 1) + (j & 1)


def _twice(side, blk, p1):
    outer = [side(p1, lambda q: blk(*_pos(q, j))) for j in range(4)]
    return [side(p0, outer.__getitem__) for p0 in range(7)]


def _ln_tasks(load, store, twice=False, keep=None):
    st = {}

    def fold(x):
        return functools.reduce(
            lambda u, v: u + v, [x[:, c:c + DH] for c in range(0, D, DH)])

    def part():
        st["s"] = fold(load())

    def mean():
        st["m"] = jnp.sum(st["s"], axis=-1, keepdims=True) * (1.0 / D)

    def square():
        d = load() - st["m"]
        st["s"] = fold(d * d)
        if keep:
            keep[...] = d

    def var():
        st["v"] = jnp.sum(st["s"], axis=-1, keepdims=True) * (1.0 / D)

    def scale():
        st["r"] = lax.rsqrt(st["v"] + EPS)

    def again():
        st["r"] = st["r"] * lax.rsqrt(st["v"] * st["r"] * st["r"] + EPS)

    def apply():
        store((keep[...] if keep else load() - st["m"]) * st["r"])

    if twice:
        return [part, mean, square, var, scale, again, apply]
    return [lambda: (part(), mean()), lambda: (square(), var(), scale()), apply]


def _abreast(chains, n):
    return [t for i in range(0, len(chains), n) for ts in zip(*chains[i:i + n]) for t in ts]


def _row_lhs(p, a1, a2):
    return a1 + a2 if p in (1, 4) else a1 if p in (2, 5) else a2


def _row_res(t):
    if 0 not in t:
        return t[2] - t[1], t[1]
    if 1 not in t:
        return t[0], t[2] - t[0]
    return t[0], t[1]


def _merge(*lists):
    order = sorted(((i + 0.5) / len(l), n, i)
                   for n, l in enumerate(lists) for i in range(len(l)))
    return [lists[n][i] for _, n, i in order]


def _interleave(*lists):
    for task in _merge(*lists):
        task()


def _held(spare, tasks):
    return [(spare, task) for task in tasks]


def _overlap(dots, side, lag):
    for i, dot in enumerate(dots):
        _release(dot(), _share(side, i, len(dots) - lag))


def _release(result, mine):
    for spare in {id(spare): spare for spare, _ in mine}.values():
        spare[...] = pltpu.bitcast(result[-8:, -DH:], spare.dtype)
    for _, task in mine:
        task()


def _share(tasks, k, n):
    return tasks[len(tasks) * k // n:len(tasks) * (k + 1) // n] if k >= 0 else []


def _tasks(fn, *ranges):
    if len(ranges) == 2:
        return [functools.partial(fn, i, j) for i in ranges[0] for j in ranges[1]]
    return [functools.partial(fn, i) for i in ranges[0]]


def _start(copies):
    for c in copies:
        c.start()


def _wait(copies):
    for c in copies:
        c.wait()


def _scores(q, k):
    return lax.dot_general(q, k, (((1,), (1,)), ((), ())), preferred_element_type=f32)


def _attend(sc, v):
    ri = lax.broadcasted_iota(jnp.int32, (L, L), 0)
    ci = lax.broadcasted_iota(jnp.int32, (L, L), 1)
    sc = jnp.where((ri < MEM) | (ri >= ci), sc * (DH ** -0.5), NEG)
    mx = jnp.max(sc, axis=1, keepdims=True)
    e = jnp.exp(sc - mx)
    den = jnp.sum(e, axis=1, keepdims=True)
    inv = pl.reciprocal(den, approx=True)
    inv = inv * (2.0 - den * inv)
    return _dot(e, v) * inv


def _kernel(x_hbm, mem0_ref, wq_hbm, wk_hbm, wv_hbm, wo_hbm, w1_hbm, w2_hbm,
            w3_hbm, w4_hbm, out_hbm, hbuf, xg, wo_t, o1, ocar, m1, w12, sems):
    w_hbm = (wq_hbm, wk_hbm, wv_hbm)
    here = lax.fori_loop(0, 2, lambda i, z: z + (i >> 1), jnp.int32(0))

    def b_copies(raw):
        tile = lambda w, i: w.bitcast(u32).at[:, :, pl.ds(128 * i, 128)]
        for n in range(4):
            slabs = pl.ds(4 * n, 4)
            for i, w in enumerate((w1_hbm, w2_hbm)):
                for c in range(2):
                    yield pltpu.make_async_copy(
                        tile(w, 2 * n + c),
                        raw.at[slabs, pl.ds(128 * (NC + 2 * i + c), 128)],
                        sems.at[SEM_B])
            for c in range(NC):
                yield pltpu.make_async_copy(
                    tile(w3_hbm, 4 * c + n), raw.at[slabs, pl.ds(128 * c, 128)],
                    sems.at[SEM_B])

    def b_operands(raw, dst, r1, p1):
        for p0, v in enumerate(_twice(_rhs, lambda k, n: _unpack(raw(k, n)).astype(f32), p1)):
            if p1 in (1, 4) and p0 in (1, 4):
                k = 2 * (p1 // 4) + p0 // 4
                dst.bitcast(u32)[7 * p1 + p0, pl.ds(r1, 8), :] = raw(k, k)
            else:
                dst[7 * p1 + p0, pl.ds(_mult(2 * r1, 16), 16), :] = v.astype(bf16)

    def rows_of(r0, n):
        return pl.ds(pl.multiple_of(r0 + here, 8), n)

    def put(rows, x):
        for c in range(8):
            xg[c, rows, :] = x[:, DH * c:DH * (c + 1)]

    def wo_tile(p, a):
        return _cols(*[_get(wo_t, p, a, c) for c in range(4)])

    def seg_quads(s):
        r0 = HALO + s * SEG
        return [jnp.concatenate(
            [xg[4 * (q & 1) + c, pl.ds(_mult(r0 + (q >> 1) * HS, 8), HS), :]
             for c in range(4)], axis=1) for q in range(4)]

    def heads_of(c_mem, m):
        return [_rows(c_mem[n], _res(n, m.__getitem__), _res(2 + n, m.__getitem__))
                for n in range(2)]

    def wo_pass(phase, a, o, prev, o1_slot):
        whole, part = GROUPS[(phase + 1) % 3], GROUPS[(phase + 2) % 3]
        quad = lambda q: o[q & 1][MEM + (q >> 1) * HS:MEM + (q >> 1) * HS + HS]
        x = [_lhs(p, quad) for p in range(7)]
        o1[o1_slot, a] = x[0].astype(bf16)
        ocar[a] = _rows(*[x[p] for p in GROUPS[phase]], *[x[p][8:] for p in part])
        res = {}
        for k in range(2):
            for p, riders in ((whole[k], (prev[SEG + 8 * k:SEG + 8 * k + 8], x[whole[k]])),
                              (part[k], (x[part[k]][:8], prev[HS * k:HS * k + HS]))):
                lhs = _rows(_row_lhs(p, o[0][:MEM], o[1][:MEM]), *riders)
                res[p] = _dot(lhs.astype(bf16), wo_tile(p, a))
        return res

    def add_h(s, terms):
        for q in range(4):
            for z in range(2):
                mine = [(sign, v) for p, zz, v in terms if zz == z
                        for qq, sign in TARGETS[p] if qq == q]
                if mine:
                    at = (pl.ds(_mult(PAD + s * SEG + (q >> 1) * HS + 8 * z, 8), 8),
                          pl.ds((q & 1) * HD, HD))
                    acc = hbuf[at]
                    for sign, v in mine:
                        acc = acc + v if sign > 0 else acc - v
                    hbuf[at] = acc

    def wo_finish(phase, s, tot, first=False):
        gw, gp = (phase + 1) % 3, (phase + 2) % 3
        whole, part = GROUPS[gw], GROUPS[gp]
        mem = _row_res({g: tot[GROUPS[g][0]][:MEM] + tot[GROUPS[g][1]][:MEM]
                        for g in (gw, gp)})
        if not first:
            add_h(s - 1, [(p, 1, tot[p][8:16]) for p in whole]
                  + [(p, z, tot[p][16 + 8 * z:24 + 8 * z]) for p in part for z in range(2)])
        add_h(s, [(p, 0, tot[p][8:16]) for p in part]
              + [(p, z, tot[p][16 + 8 * z:24 + 8 * z]) for p in whole for z in range(2)])
        return mem

    def wo_m1(slot, pairs):
        lhs = jnp.concatenate(
            [_rows(*[_get(o1, slot + k, a) for k in range(3)]) for a in pairs], axis=1)
        return _dot(lhs, _rows(*[wo_tile(0, a) for a in pairs]))

    def add_m1(s, r):
        for k in range(3):
            add_h(jnp.maximum(s + k, 0),
                  [(0, z, r[HS * k + 8 * z:HS * k + 8 * z + 8]) for z in range(2)])

    def mixer_norm(r0, keep=None):
        return _ln_tasks(lambda: hbuf[rows_of(PAD + r0, HS), :],
                         functools.partial(put, rows_of(HALO + r0, HS)), True, keep)

    def prologue(wt, qcar, stg, words, lhs1, lhs0, qkv0):
        def row_copy(src, i, n, sem):
            rows = pl.ds(_mult(i * n, n), n)
            return pltpu.make_async_copy(src.bitcast(u32).at[rows], words.at[rows],
                                         sems.at[sem + i])

        x_copy = lambda i: row_copy(x_hbm, i, S // 8, SEM_X)
        wo_copy = lambda g: row_copy(wo_hbm, g, 512, SEM_WO)

        def start_chunk(g, m):
            src = w_hbm[m].bitcast(u32)
            dst = stg.reshape(3 * HD, 8, DH)
            for par in range(2):
                pltpu.make_async_copy(
                    src.at[:, pl.ds(_mult(16 * par + 4 * g, 4), 4), :],
                    dst.at[pl.ds(HD * m, HD), pl.ds(4 * par, 4), :],
                    sems.at[SEM_W + 3 * g + m]).start()

        def wait_chunk(g, m):
            part = stg.at[pl.ds(_mult(4 * D * m, 4 * D), 4 * D)]
            pltpu.make_async_copy(part, part, sems.at[SEM_W + 3 * g + m]).wait()

        def operands(g, m, pair, i):
            w = [stg[pl.ds(4 * (D * m + HD * k + 16 * i) + pair, 16, stride=4), :]
                 for k in range(2)]
            quad = [pltpu.bitcast(w[q >> 1] & jnp.uint32(0xFFFF0000) if q & 1
                                  else w[q >> 1] << 16, f32) for q in range(4)]
            wt[3 * NP + m, pair, pl.ds(16 * i, 16), :] = _rhs(0, quad.__getitem__).astype(bf16)
            for p in range(1, 7):
                wt[NP * m + 4 * g + pair, p - 1, pl.ds(16 * i, 16), :] = _rhs(
                    p, quad.__getitem__).astype(bf16)

        def wo_operands(g, pair, i):
            c, r0 = i & 3, 8 * (i >> 2)
            w = [words[rows_of(DH * (4 * g + pair) + DH // 2 * (q >> 1) + r0, 8),
                       pl.ds(HD * (q & 1) + DH * c, DH)] for q in range(4)]
            quad = [_unpack(v).astype(f32) for v in w]
            for p in range(7):
                v = _rhs(p, quad.__getitem__).astype(bf16)
                wo_t[p, 4 * g + pair, c, pl.ds(2 * r0, 16), :] = v

        for i in range(4):
            if i == 3:
                start_chunk(0, 0)
            x_copy(i).start()
        start_chunk(0, 1)
        start_chunk(0, 2)
        for r0 in (0, HALO + S):
            put(pl.ds(r0, HALO), jnp.zeros((HALO, D), f32))
        for k in range(2):
            o1[k] = jnp.zeros((NP, HS, DH), bf16)
        @pl.loop(0, 4)
        def _(i):
            x_copy(i).wait()

            @pl.loop(0, 4, unroll=4)
            def _(k):
                r0 = pl.multiple_of(i * (S // 4) + k * 128, 128)
                xv = _unpack(words[pl.ds(pl.multiple_of(r0 // 2, 64), 64), :]).astype(f32)
                hbuf[pl.ds(PAD + r0, 128), :] = xv
                xn = _ln(xv)
                put(pl.ds(HALO + r0, 128), xn)
                v = _rows(*[xn[z:z + HS, :HD] + xn[z + HS:z + SEG, HD:]
                            for z in range(0, 128, SEG)])
                for c in range(4):
                    lhs1[c, pl.ds(pl.multiple_of(r0 // 2, 64), 64), :] = (
                        v[:, DH * c:DH * (c + 1)].astype(bf16))

        wait_chunk(0, 0)

        @pl.loop(0, 4)
        def _(pair):
            for i in range(HD // 16):
                operands(0, 0, pair, i)

        mem = mem0_ref[...].astype(f32)
        cur, nxt = seg_quads(0), seg_quads(1)
        for p in range(1, 7):
            x0, x1 = _lhs(p, cur.__getitem__), _lhs(p, nxt.__getitem__)
            v = (_rows(x0, x1) if p in GROUPS[1]
                 else _rows(_row_lhs(p, mem[:, :HD], mem[:, HD:]), x1[:8], x0))
            for c in range(4):
                lhs0[p - 1, c] = v[:, DH * c:DH * (c + 1)].astype(bf16)

        def first(g, m, pair, i):
            n = S // 2 // M1_CUT
            lhs = _cols(*[_get(lhs1, c, rows=(n * i, n)) for c in range(4)])
            r = pltpu.bitcast(_dot(lhs, _get(wt, 3 * NP + m + here, pair)), u32)
            m1.bitcast(u32)[NP * m + 4 * g + pair, pl.ds(n * i, n), :] = r
            return r

        def project(g, m, pair):
            a = 4 * g + pair
            r = {p: _dot(_cols(*[_get(lhs0, p - 1, c) for c in range(4)]),
                         _get(wt, NP * m + a, p - 1))
                 for p in range(1, 7)}
            prod = {p: r[p][:HS] if p in GROUPS[1] else r[p][HS:] for p in r}
            prod[0] = pltpu.bitcast(m1.bitcast(u32)[NP * m + a, pl.ds(0, HS), :], f32)
            qcar[m, a] = _rows(*[r[p][HS:] for p in GROUPS[1]],
                               *[r[p][8:16] for p in GROUPS[2]])
            c_mem = _row_res({k: r[GROUPS[k][0]][:MEM] + r[GROUPS[k][1]][:MEM]
                              for k in (0, 2)})
            for n, v in enumerate(heads_of(c_mem, prod)):
                qkv0[m, a, n] = v

        def wo_tasks(g):
            return _held(words.at[pl.ds(H * DH // 2, 8), pl.ds(0, DH)],
                         _tasks(functools.partial(wo_operands, g), range(4), range(32)))

        def dots(g, m):
            return _tasks(functools.partial(first, g, m), range(4), range(M1_CUT))

        @pl.loop(0, 11)
        def _(c):
            g, g2 = lax.div(c, 3), lax.div(c + 1, 3)
            m, m2 = c - 3 * g, c + 1 - 3 * g2
            for k in range(3):
                pl.when((m == k) & (g < 3))(functools.partial(start_chunk, g + 1, k))
            pl.when(c == 9)(lambda: _start([wo_copy(k) for k in range(4)]))
            wait_chunk(g2, m2)
            _interleave(_tasks(functools.partial(operands, g2, m2), range(4), range(HD // 16)),
                        dots(g, m))
            for pair in range(4):
                project(g, m, pair)

        for k in range(2):
            wo_copy(k).wait()
            _overlap(_share(dots(3, 2), k, 2), wo_tasks(k), 2)

        scores, outs, tot = {}, {}, {}
        none = jnp.zeros((3 * HS, DH), f32)

        def step0(t):
            if t < NP:
                scores[t] = [_scores(qkv0[0, t, n], qkv0[1, t, n]) for n in range(2)]
            if 0 <= t - 2 < NP:
                outs[t - 2] = [_attend(scores[t - 2][n], qkv0[2, t - 2, n]) for n in range(2)]
            if 0 <= t - 4 < NP:
                for p, r in wo_pass(0, t - 4, outs[t - 4], none, 2).items():
                    tot[p] = tot[p] + r if p in tot else r
                return r
            project(3, 2, t)
            return qkv0[0, t, 0]

        for k, slots in ((2, range(12)), (3, range(12, 16))):
            wo_copy(k).wait()
            _overlap(_tasks(step0, slots), wo_tasks(k), 1)
        _interleave(_tasks(step0, range(16, 20)))
        return wo_finish(0, 0, tot, first=True)

    def step(wt, qcar, s, phase, cur, nxt, first, mem, o1_slot, fillers, chores):
        gw, gp = (phase + 1) % 3, (phase + 2) % 3
        ahead, now = GROUPS[gw], GROUPS[gp]
        lhs = {}
        for p in ahead + now:
            x0, x1 = _lhs(p, cur.__getitem__), _lhs(p, nxt.__getitem__)
            riders = (x0[8:], x1) if p in ahead else (x1[:8], x0)
            lhs[p] = _rows(_row_lhs(p, *mem), *riders).astype(bf16)
        heads, scores, outs, tot = {}, {}, {}, {}

        def qkv(a):
            heads[a] = []
            for m in range(3):
                r = {p: _dot(lhs[p], _get(wt, NP * m + a, p - 1)) for p in lhs}
                _release(r[now[1]], _share(chores, 3 * a + m, 3 * NP - CH0))
                old = qcar[m, a]
                prod = {0: pltpu.bitcast(first(NP * m + a), f32)}
                for k in range(2):
                    prod[GROUPS[phase][k]] = old[HS * k:HS * k + HS]
                    prod[ahead[k]] = _rows(old[SEG + 8 * k:SEG + 8 * k + 8],
                                           r[ahead[k]][8:16])
                    prod[now[k]] = r[now[k]][HS:]
                qcar[m, a] = _rows(*[r[p][HS:] for p in ahead], *[r[p][8:16] for p in now])
                c_mem = _row_res({g: r[GROUPS[g][0]][:MEM] + r[GROUPS[g][1]][:MEM]
                                  for g in (gw, gp)})
                heads[a].append(heads_of(c_mem, prod))

        for t in range(NP + LAG_WO):
            a = t - LAG_QK
            if 0 <= a < NP:
                scores[a] = [_scores(heads[a][0][n], heads[a][1][n]) for n in range(2)]
            a = t - LAG_PV
            if 0 <= a < NP:
                outs[a] = [_attend(scores[a][n], heads[a][2][n]) for n in range(2)]
            if t < NP:
                qkv(t)
            if t == FILL_AT:
                fillers[0]()
            a = t - LAG_WO
            if 0 <= a < NP:
                for p, r in wo_pass(phase, a, outs[a], ocar[a], o1_slot).items():
                    tot[p] = tot[p] + r if p in tot else r
        fillers[1]()
        return wo_finish(phase, s, tot)

    def recurrence(wt, qcar, mem, raw, fin):
        _start(b_copies(raw))
        spare = 128 * (NC + 4)
        raw[pl.ds(0, 16), pl.ds(spare, 8), :] = jnp.zeros((16, 8, DH), u32)

        def chores(i):
            def convert(dst, base, per, groups):
                tasks = []
                for k in range(per):
                    r = pl.multiple_of(8 * jnp.clip(per * (i - 2) + k, 0, groups - 1), 8)
                    r0 = pl.multiple_of(jnp.where(i > 1, base + r, spare), 8)
                    tasks += _tasks(functools.partial(
                        b_operands, lambda k, n, r0=r0: raw[4 * n + k, pl.ds(r0, 8), :],
                        dst, r), range(7))
                return _held(raw.at[16, pl.ds(0, 8)], tasks)
            rest = convert(w12, 128 * NC, 4, 64)
            norm = _abreast(
                [mixer_norm(jnp.maximum(3 * i - 5 + (k >> 1), 0) * SEG + (k & 1) * HS,
                            fin.at[rows_of(HS * k, HS)])
                 for k in range(6)], 6)
            in_h = hbuf.at[pl.ds(0, 8), pl.ds(0, DH)]
            norm = (_held(in_h, norm[:12]), _held(in_h, norm[12:36]),
                    _held(fin.at[pl.ds(3 * SEG, 8), pl.ds(0, DH)], norm[36:]))

            def due():
                m1.bitcast(u32)[3 * NP + here, pl.ds(S // 2 - 8, 8), :] = pltpu.bitcast(
                    xg[here, pl.ds(0, 8), :], u32)
            norm[2].append((norm[2][0][0], due))
            return [_merge(t, n)
                    for t, n in zip((_share(rest, 0, 2), _share(rest, 1, 2),
                                     convert(m1, 0, 6, 16 * NC)), norm)]

        def steps(i, mem):
            pl.when(i == 2)(lambda: _wait(b_copies(raw)))
            src = 3 * (i & 1)
            acc = []

            def filler(n):
                if CUTS[n] < CUTS[n + 1]:
                    acc.append(wo_m1(src, range(CUTS[n], CUTS[n + 1])))
                    if CUTS[n + 1] == NP:
                        add_m1(3 * i - 2, functools.reduce(lambda u, v: u + v, acc))

            todo = chores(i)
            filler(0)
            nxt = seg_quads(3 * i + 1)
            for k in range(3):
                fillers = _tasks(filler, (2 * k + 1, 2 * k + 2))
                rows = pl.ds(pl.multiple_of((3 * i + 1 + k) * HS, HS), HS)
                first = lambda j: m1.bitcast(u32)[j, rows, :]
                if k == 2:
                    early = {j: first(j) for j in range(3 * NP) if j % NP < DUE}
                    first = lambda j, late=first: early[j] if j in early else late(j)
                cur, nxt = nxt, seg_quads(jnp.minimum(3 * i + 2 + k, NSEG - 1))
                mem = step(wt, qcar, 3 * i + 1 + k, (1 + k) % 3, cur, nxt, first, mem,
                           3 - src + k, fillers, todo[k])
            return mem

        lax.fori_loop(0, NSEG // 3, steps, mem)

    def block_a(wt, qcar):
        mem = pl.run_scoped(
            functools.partial(prologue, wt, qcar),
            pltpu.VMEM((12 * D, DH), u32),
            pltpu.VMEM((H * DH // 2 + 8, D), u32),
            pltpu.VMEM((4, S // 2, DH), bf16),
            pltpu.VMEM((6, 4, SEG, DH), bf16),
            pltpu.VMEM((3, NP, 2, L, DH), f32))

        pl.run_scoped(functools.partial(recurrence, wt, qcar, mem),
                      pltpu.VMEM((17, 128 * (NC + 4) + 8, DH), u32),
                      pltpu.VMEM((3 * SEG + 8, D), f32))

    pl.run_scoped(block_a, pltpu.VMEM((3 * NP + 3, 6, HD, DH), bf16),
                  pltpu.VMEM((3, NP, 3 * HS, DH), f32))

    def block_b(w4t, x1b, yn, ya, *pu):
        in_h = hbuf.at[pl.ds(0, 8), pl.ds(0, DH)]
        in_y = yn.at[pl.ds(RB, 8), pl.ds(0, DH)]
        pu = [pu[c % 3] for c in range(NC)]
        def wo_last():
            phase = NSEG % 3
            tot = {}

            def task(a0, p, r0=0, n=0):
                pairs = range(a0, a0 + 2)
                if p == 0:
                    r = wo_m1(3 * (NSEG // 3 & 1), pairs)
                else:
                    lhs = _cols(*[ocar[a, pl.ds(r0, n), :] for a in pairs])
                    r = _dot(lhs.astype(bf16), _rows(*[wo_tile(p, a) for a in pairs]))
                tot[p] = tot[p] + r if a0 else r
                if a0 == NP - 2 and p == 0:
                    add_m1(NSEG - 3, tot[p])
                elif a0 == NP - 2:
                    add_h(NSEG - 1, [(p, 1, tot[p][-8:])] + [(p, 0, tot[p][:8])] * (n > 8))
                return r

            todo = [(0,)] + [t for k in range(2) for t in (
                (GROUPS[(phase + 2) % 3][k], HS * k, HS),
                (GROUPS[(phase + 1) % 3][k], SEG + 8 * k, 8))]
            return [functools.partial(task, a0, *t) for t in todo for a0 in range(0, NP, 2)]

        def a_operands(load, dst):
            def task(g, p1):
                r0, c = 16 * (g >> 1), g & 1
                for p0, v in enumerate(_twice(
                        _lhs, lambda i, k: load(i * R + r0, 2 * k + c), p1)):
                    dst[7 * p1 + p0, c, pl.ds(r0, 16), :] = v.astype(bf16)
            return _tasks(task, range(R // 8), range(7))

        def products(src, w, r0, dst):
            m = {}

            def task(p1, p0):
                p = 7 * p1 + p0
                m[p0] = _dot(_cols(*[_get(src, p + here, k) for k in range(2)]),
                             _get(w, p, rows=(r0, C4)))
                if p0 >= 3:
                    j = (2, 1, 3, 0)[p0 - 3]
                    dst[p1, j] = _res(j, m.__getitem__)
                return m[p0]
            return _tasks(task, range(7), range(7))

        def mlp_in(b):
            def residual(r0, y):
                x1 = y + x1b[rows_of(b * RB + r0, 16), :]
                yn[pl.ds(r0, 16), :] = x1
                put(rows_of(b * RB + r0, 16), hbuf[rows_of(PAD + b * RB + r0, 16), :] + x1)

            def store(r0, y):
                yn[pl.ds(r0, 16), :] = y
                return y

            return _held(in_h, _abreast([
                _ln_tasks(lambda r0=r0: hbuf[rows_of(PAD + b * RB + r0, 16), :],
                          functools.partial(residual, r0)) for r0 in range(0, RB, 16)], RB // 16)
            ) + _held(in_y, _abreast([
                _ln_tasks(lambda r0=r0: yn[rows_of(r0, 16), :],
                          functools.partial(store, r0)) for r0 in range(0, RB, 16)], RB // 16)
                + a_operands(
                lambda r0, c: yn[rows_of(r0, 16), pl.ds(DH * c, DH)], ya))

        def ups(c):
            return products(ya, m1, C4 * c, pu[c])

        def mixer(raw, *bufs):
            sa, sp = bufs[:2], (bufs[2:4], bufs[4:])
            in_g = xg.at[0, pl.ds(S + 2 * HALO, 8)]
            w4_copies = [pltpu.make_async_copy(
                w4_hbm.bitcast(u32).at[pl.ds(c, n)], raw.at[pl.ds(c, n)], sems.at[SEM_B + s])
                for c, n, s in ((0, 2, 1), (2, NC - 2, 2))]
            _start(w4_copies)

            def pre(n, w, b):
                shift = lambda c: w * (-1, 1, -2, 2)[c >> 1]
                return _held(in_g, a_operands(lambda r0, c: xg[c + here, pl.ds(
                    HALO + b * RB + r0 + shift(c), 16), :], sa[n & 1]))

            def post(n, w, b):
                def task(g, j):
                    c, g = divmod(g, R // 8)
                    m = [sp[n & 1][c][p1 + here, j, pl.ds(8 * g, 8), :]
                         for p1 in range(7)]
                    for q in range(4):
                        i, k = _pos(q, j)
                        r0 = _mult(b * RB + i * R + 8 * g, 8)
                        v = _res(q, m.__getitem__)
                        if w == 0:
                            xg[2 * k + c, pl.ds(HALO + r0, 8), :] = _gelu2(v)
                        else:
                            x1b[pl.ds(r0, 8), pl.ds(DH * (2 * k + c), DH)] = 0.5 * v
                return [t for c in range(2) for t in _held(
                    sp[n & 1][c].at[7, 0, pl.ds(0, 8)],
                    _tasks(task, range(R // 8 * c, R // 8 * (c + 1)), range(4)))]

            def unit(n, w, *side):
                dots = [t for c in range(2) for t in products(
                    sa[n & 1], w12, C4 * (2 * w + c), sp[n & 1][c])]
                _overlap(dots, _merge(*side), MX_LAG)

            def w4_work(k, n, half=0):
                def task(i, p1):
                    g, c = half + (i >> 1), i & 1
                    r0 = _mult(8 * (g & 7), 8)
                    b_operands(lambda q, j: raw[(g >> 3) + here, q, pl.ds(r0, 8),
                                                pl.ds(DH * (2 * j + c), DH)],
                               w4t, _mult(DH * (g >> 3) + 64 * c + r0, 8), p1)
                return _held(raw.at[NC, 0, pl.ds(0, 8), pl.ds(0, DH)],
                             _tasks(task, range(k, k + n), range(7)))

            norms = lambda s: _held(in_h, _abreast(
                [mixer_norm(s * SEG + k * HS) for k in range(6)], 3))
            _overlap(wo_last(), _merge(pre(0, 0, 0), norms(NSEG - 6)), MX_LAG)
            unit(0, 0, pre(1, 0, 1), norms(NSEG - 3))
            _wait(w4_copies[:1])

            @pl.loop(0, 3)
            def _(i):
                pl.when(i == 2)(lambda: _wait(w4_copies[1:]))
                for n in range(2):
                    b = 2 * i + 1 + n
                    unit(n + 1, 0, pre(n, 0, b + 1), post(n, 0, b - 1),
                         w4_work(G1 * n, G1, G1 * i))

            unit(1, 0, pre(0, 1, 0), post(0, 0, 6), w4_work(6 * G1, G1))
            unit(0, 1, pre(1, 1, 1), post(1, 0, 7), w4_work(7 * G1, G1))

            @pl.loop(0, 2)
            def _(i):
                for n in range(2):
                    b = 2 * i + 1 + n
                    unit(n + 1, 1, pre(n, 1, b + 1), post(n, 1, b - 1),
                         w4_work(8 * G1 + G2 * n, G2, G2 * i))

            done = 8 * G1 + 4 * G2
            rest = w4_work(done, 16 * NC - done)
            ahead = mlp_in(0)
            for b in range(5, NB):
                unit(b, 1, pre(b + 1, 1, b + 1) if b + 1 < NB else _share(rest, 2, 4),
                     post(b - 1, 1, b - 1), _share(ahead, b - 5, 3),
                     _share(rest, (0, 1, 3)[b - 5], 4))
            for _, task in post(1, 1, NB - 1):
                task()

        def mlp(ta0, ta1, pd, ob):
            ta = [ta0.at[c] for c in range(NC - 1)] + [ta1]

            def mid(c, g, j):
                r = pl.ds(8 * g, 8)
                m = [pu[c][p1 + here, j, r, :] for p1 in range(7)]
                y = [_gelu2(_res(q, m.__getitem__)) for q in range(4)]
                for p1 in range(7):
                    v = _lhs(p1, y.__getitem__)
                    ta[c][p1, j, r, :] = v
                return v

            def down(b, m, p, c):
                p1, p0 = divmod(p, 7)
                lhs = _lhs(p0, lambda j: ta[c][p1 + here, j]).astype(bf16)
                tot = _dot(lhs, jnp.concatenate(
                    [_get(w4t, p, rows=(C4 * c + 128 * k, 128)) for k in range(2)],
                    axis=1))
                m[p] = m[p] + tot if c else tot
                if c == NC - 1 and p0 >= 3:
                    j = (2, 1, 3, 0)[p0 - 3]
                    v = _res(j, lambda k: m[7 * p1 + k])
                    if p1 < 6:
                        pd[p1, j] = v
                    if p1 >= 3:
                        q = (2, 1, 3, 0)[p1 - 3]
                        i, n = _pos(q, j)
                        r0, cols = _mult(b * RB + i * R, R), pl.ds(n * C4, C4)
                        v = _res(q, lambda k: v if k == p1 else pd[k + here, j])
                        ob[pl.ds(r0, R), cols] = (
                            _cols(*[xg[2 * n + k, pl.ds(r0, R), :] for k in range(2)]) + 0.5 * v).astype(bf16)
                return tot

            def out_copy(b):
                rows = pl.ds(_mult(b * RB, RB), RB)
                return pltpu.make_async_copy(ob.at[rows], out_hbm.at[rows],
                                             sems.at[SEM_OUT + b])

            @pl.loop(0, NB)
            def _(b):
                mids = lambda c: _held(pu[c].at[7, 0, pl.ds(0, 8)], _tasks(
                    functools.partial(mid, c), range(R // 8), range(4)))
                task = functools.partial(down, b, {})
                early = _tasks(task, range(EARLY), range(NC - 1))
                ahead = mlp_in(jnp.minimum(b + 1, NB - 1))
                _overlap(ups(0), ahead[:A0], 0)
                for c in range(NC):
                    _overlap(ups(c + 1) if c + 1 < NC else early,
                             _merge(mids(c), _share(ahead[A0:AH], c, NC - 1)), UP_LAG)

                _overlap(_tasks(task, range(EARLY), [NC - 1])
                         + _tasks(task, range(EARLY, 49), range(NC)),
                         ahead[AH:], DN_LAG)
                out_copy(b).start()

            for b in range(NB):
                out_copy(b).wait()

        pl.run_scoped(mixer, pltpu.VMEM((NC + 1, 4, 64, D), u32),
                      *[pltpu.VMEM((49, 2, R, DH), bf16)] * 2,
                      *[pltpu.VMEM((8, 4, R, DH), f32)] * 4)
        pl.run_scoped(mlp, pltpu.VMEM((NC - 1, 7, 4, R, DH), f32),
                      pltpu.VMEM((7, 4, R, DH), f32),
                      pltpu.VMEM((6, 4, R, C4), f32), pltpu.VMEM((S, D), bf16))

    pl.run_scoped(
        block_b,
        pltpu.VMEM((49, C4 * NC, DH), bf16),
        pltpu.VMEM((S, D), f32),
        pltpu.VMEM((RB + 8, D), f32),
        pltpu.VMEM((49, 2, R, DH), bf16),
        *[pltpu.VMEM((8, 4, R, 128), f32)] * 3)


@jax.jit
def pallas_sequential_preLN__memory_aug_recurrent_mem_tr__mixer_s_mlp__prompt_kernel(
    A_x: jax.Array,
    A_mem0: jax.Array,
    A_Wq: jax.Array,
    A_Wk: jax.Array,
    A_Wv: jax.Array,
    A_Wo: jax.Array,
    A_seg_len: jax.Array,
    B_x: jax.Array,
    B_w1: jax.Array,
    B_w2: jax.Array,
    B_w3: jax.Array,
    B_w4: jax.Array,
):
    del A_seg_len, B_x
    hbm = pl.BlockSpec(memory_space=pl.ANY)
    vmem = pl.BlockSpec(memory_space=pltpu.VMEM)
    scratch = [
        pltpu.VMEM((PAD + S, D), f32),
        pltpu.VMEM((8, S + 3 * HALO, DH), f32),
        pltpu.VMEM((7, NP, 4, DH, DH), bf16),
        pltpu.VMEM((6, NP, HS, DH), bf16),
        pltpu.VMEM((NP, 3 * HS, DH), f32),
        pltpu.VMEM((49, S, DH), bf16),
        pltpu.VMEM((49, D, DH), bf16),
        pltpu.SemaphoreType.DMA((NSEM,)),
    ]
    out = pl.pallas_call(
        _kernel,
        out_shape=jax.ShapeDtypeStruct((S, D), A_x.dtype),
        in_specs=[hbm, vmem] + [hbm] * 8,
        out_specs=hbm,
        scratch_shapes=scratch,
        compiler_params=pltpu.CompilerParams(vmem_limit_bytes=127 * 1024 * 1024),
    )(A_x.reshape(S, D), A_mem0.reshape(MEM, D),
      A_Wq.reshape(D // 2, 2 * H, DH), A_Wk.reshape(D // 2, 2 * H, DH),
      A_Wv.reshape(D // 2, 2 * H, DH),
      A_Wo.reshape(H * DH, D), B_w1.reshape(4, C4, D), B_w2.reshape(4, C4, D),
      B_w3.reshape(4, C4, F), B_w4.reshape(NC, 4, FC // 4, D))
    return out.reshape(A_x.shape)
```

```python
import functools

import jax
import jax.numpy as jnp
from jax import lax
import jax.experimental.pallas as pl
import jax.experimental.pallas.tpu as pltpu

S = 2048
D = 1024
H = 32
DH = 128
MEM = 8
SEG = 32
F = 3584
NSEG = S // SEG
L = MEM + SEG
HS = SEG // 2
NP = H // 2
HD = D // 2
PAD = 8
C4 = D // 4
HALO = 8
R = 64
RB = 4 * R
NB = S // RB
FC = 512
NC = F // FC
EPS = 1e-5
NEG = -1000000000.0

LAG_QK = 2
LAG_PV = 4
LAG_WO = 6
FILL_AT = 19
CUTS = (0, 1, 3, 8, 10, 14, 16, 16)
CH0 = 20
DUE = 15
M1_CUT = 16
G1 = 8
G2 = 11
A0 = 32
AH = 96
EARLY = 11
MX_LAG = 5
UP_LAG = 10
DN_LAG = 20

GROUPS = ((1, 3), (2, 4), (5, 6))
TARGETS = (((0, 1), (3, 1)), ((2, 1), (3, -1)), ((1, 1), (3, 1)), ((0, 1), (2, 1)),
           ((0, -1), (1, 1)), ((3, 1),), ((0, 1),))

bf16 = jnp.bfloat16
f32 = jnp.float32
u32 = jnp.uint32

SEM_X, SEM_W, SEM_WO, SEM_B, SEM_OUT = 0, 4, 16, 20, 24
NSEM = SEM_OUT + NB


def _mult(i, n):
    return i if isinstance(i, int) else pl.multiple_of(i, n)


def _ln(x):
    m = jnp.mean(x, axis=-1, keepdims=True)
    d = x - m
    v = jnp.mean(d * d, axis=-1, keepdims=True)
    return d * lax.rsqrt(v + EPS)


def _gelu2(x):
    c = 0.7978845608028654
    return x + x * jnp.tanh(x * (c + (c * 0.044715) * (x * x)))


def _get(ref, *idx, rows=None):
    rows = slice(None) if rows is None else pl.ds(rows[0] // 2, rows[1] // 2)
    return _unpack(ref.bitcast(u32)[idx + (rows, slice(None))])


def _cols(*xs):
    return jnp.concatenate(xs, axis=1)


def _unpack(x):
    return pltpu.bitcast(x, bf16)


def _dot(a, b):
    return jnp.dot(a, b, preferred_element_type=f32)


def _rows(*xs):
    return jnp.concatenate(xs, axis=0)


def _lhs(p, a):
    return (lambda: a(0) + a(3), lambda: a(2) + a(3), lambda: a(0), lambda: a(3),
            lambda: a(0) + a(1), lambda: a(2) - a(0), lambda: a(1) - a(3))[p]()


def _rhs(p, b):
    return (lambda: b(0) + b(3), lambda: b(0), lambda: b(1) - b(3), lambda: b(2) - b(0),
            lambda: b(3), lambda: b(0) + b(1), lambda: b(2) + b(3))[p]()


def _res(q, m):
    return (lambda: m(0) + m(3) - m(4) + m(6), lambda: m(2) + m(4),
            lambda: m(1) + m(3), lambda: m(0) - m(1) + m(2) + m(5))[q]()


def _pos(q, j):
    return 2 * (q >> 1) + (j >> 1), 2 * (q & 1) + (j & 1)


def _twice(side, blk, p1):
    outer = [side(p1, lambda q: blk(*_pos(q, j))) for j in range(4)]
    return [side(p0, outer.__getitem__) for p0 in range(7)]


def _ln_tasks(load, store, twice=False, keep=None):
    st = {}

    def fold(x):
        return functools.reduce(
            lambda u, v: u + v, [x[:, c:c + DH] for c in range(0, D, DH)])

    def part():
        st["s"] = fold(load())

    def mean():
        st["m"] = jnp.sum(st["s"], axis=-1, keepdims=True) * (1.0 / D)

    def square():
        d = load() - st["m"]
        st["s"] = fold(d * d)
        if keep:
            keep[...] = d

    def var():
        st["v"] = jnp.sum(st["s"], axis=-1, keepdims=True) * (1.0 / D)

    def scale():
        st["r"] = lax.rsqrt(st["v"] + EPS)

    def again():
        st["r"] = st["r"] * lax.rsqrt(st["v"] * st["r"] * st["r"] + EPS)

    def apply():
        store((keep[...] if keep else load() - st["m"]) * st["r"])

    if twice:
        return [part, mean, square, var, scale, again, apply]
    return [lambda: (part(), mean()), lambda: (square(), var(), scale()), apply]


def _abreast(chains, n):
    return [t for i in range(0, len(chains), n) for ts in zip(*chains[i:i + n]) for t in ts]


def _row_lhs(p, a1, a2):
    return a1 + a2 if p in (1, 4) else a1 if p in (2, 5) else a2


def _row_res(t):
    if 0 not in t:
        return t[2] - t[1], t[1]
    if 1 not in t:
        return t[0], t[2] - t[0]
    return t[0], t[1]


def _merge(*lists):
    order = sorted(((i + 0.5) / len(l), n, i)
                   for n, l in enumerate(lists) for i in range(len(l)))
    return [lists[n][i] for _, n, i in order]


def _interleave(*lists):
    for task in _merge(*lists):
        task()


def _held(spare, tasks):
    return [(spare, task) for task in tasks]


def _overlap(dots, side, lag):
    for i, dot in enumerate(dots):
        _release(dot(), _share(side, i, len(dots) - lag))


def _release(result, mine):
    for spare in {id(spare): spare for spare, _ in mine}.values():
        spare[...] = pltpu.bitcast(result[-8:, -DH:], spare.dtype)
    for _, task in mine:
        task()


def _share(tasks, k, n):
    return tasks[len(tasks) * k // n:len(tasks) * (k + 1) // n] if k >= 0 else []


def _tasks(fn, *ranges):
    if len(ranges) == 2:
        return [functools.partial(fn, i, j) for i in ranges[0] for j in ranges[1]]
    return [functools.partial(fn, i) for i in ranges[0]]


def _start(copies):
    for c in copies:
        c.start()


def _wait(copies):
    for c in copies:
        c.wait()


def _scores(q, k):
    return lax.dot_general(q, k, (((1,), (1,)), ((), ())), preferred_element_type=f32)


def _attend(sc, v):
    ri = lax.broadcasted_iota(jnp.int32, (L, L), 0)
    ci = lax.broadcasted_iota(jnp.int32, (L, L), 1)
    sc = jnp.where((ri < MEM) | (ri >= ci), sc, NEG * DH ** 0.5)
    mx = jnp.max(sc, axis=1, keepdims=True)
    e = jnp.exp2((sc - mx) * (DH ** -0.5 * 1.4426950408889634))
    den = jnp.sum(e, axis=1, keepdims=True)
    inv = pl.reciprocal(den, approx=True)
    inv = inv * (2.0 - den * inv)
    return _dot(e, v) * inv


def _kernel(x_hbm, mem0_hbm, wq_hbm, wk_hbm, wv_hbm, wo_hbm, w1_hbm, w2_hbm,
            w3_hbm, w4_hbm, out_hbm, hbuf, xg, wo_t, o1, ocar, m1, w12, sems):
    w_hbm = (wq_hbm, wk_hbm, wv_hbm)
    here = lax.fori_loop(0, 2, lambda i, z: z + (i >> 1), jnp.int32(0))

    def b_copies(raw):
        tile = lambda w, i: w.bitcast(u32).at[:, :, pl.ds(128 * i, 128)]
        for n in range(4):
            slabs = pl.ds(4 * n, 4)
            for i, w in enumerate((w1_hbm, w2_hbm)):
                for c in range(2):
                    yield pltpu.make_async_copy(
                        tile(w, 2 * n + c),
                        raw.at[slabs, pl.ds(128 * (NC + 2 * i + c), 128)],
                        sems.at[SEM_B])
            for c in range(NC):
                yield pltpu.make_async_copy(
                    tile(w3_hbm, 4 * c + n), raw.at[slabs, pl.ds(128 * c, 128)],
                    sems.at[SEM_B])

    def b_operands(raw, dst, r1, p1):
        for p0, v in enumerate(_twice(_rhs, lambda k, n: _unpack(raw(k, n)).astype(f32), p1)):
            if p1 in (1, 4) and p0 in (1, 4):
                k = 2 * (p1 // 4) + p0 // 4
                dst.bitcast(u32)[7 * p1 + p0, pl.ds(r1, 8), :] = raw(k, k)
            else:
                dst[7 * p1 + p0, pl.ds(_mult(2 * r1, 16), 16), :] = v.astype(bf16)

    def rows_of(r0, n):
        return pl.ds(pl.multiple_of(r0 + here, 8), n)

    def put(rows, x):
        for c in range(8):
            xg[c, rows, :] = x[:, DH * c:DH * (c + 1)]

    def wo_tile(p, a):
        return _cols(*[_get(wo_t, p, a, c) for c in range(4)])

    def seg_quads(s):
        r0 = HALO + s * SEG
        return [jnp.concatenate(
            [xg[4 * (q & 1) + c, pl.ds(_mult(r0 + (q >> 1) * HS, 8), HS), :]
             for c in range(4)], axis=1) for q in range(4)]

    def heads_of(c_mem, m):
        return [_rows(c_mem[n], _res(n, m.__getitem__), _res(2 + n, m.__getitem__))
                for n in range(2)]

    def wo_pass(phase, a, o, prev, o1_slot):
        whole, part = GROUPS[(phase + 1) % 3], GROUPS[(phase + 2) % 3]
        quad = lambda q: o[q & 1][MEM + (q >> 1) * HS:MEM + (q >> 1) * HS + HS]
        x = [_lhs(p, quad) for p in range(7)]
        o1[o1_slot, a] = x[0].astype(bf16)
        ocar[a] = _rows(*[x[p] for p in GROUPS[phase]], *[x[p][8:] for p in part])
        res = {}
        for k in range(2):
            for p, riders in ((whole[k], (prev[SEG + 8 * k:SEG + 8 * k + 8], x[whole[k]])),
                              (part[k], (x[part[k]][:8], prev[HS * k:HS * k + HS]))):
                lhs = _rows(_row_lhs(p, o[0][:MEM], o[1][:MEM]), *riders)
                res[p] = lhs.astype(bf16)
        return res

    def add_h(s, terms):
        for q in range(4):
            for z in range(2):
                mine = [(sign, v) for p, zz, v in terms if zz == z
                        for qq, sign in TARGETS[p] if qq == q]
                if mine:
                    at = (pl.ds(_mult(PAD + s * SEG + (q >> 1) * HS + 8 * z, 8), 8),
                          pl.ds((q & 1) * HD, HD))
                    acc = hbuf[at]
                    for sign, v in mine:
                        acc = acc + v if sign > 0 else acc - v
                    hbuf[at] = acc

    def wo_finish(phase, s, tot, first=False):
        gw, gp = (phase + 1) % 3, (phase + 2) % 3
        whole, part = GROUPS[gw], GROUPS[gp]
        mem = _row_res({g: tot[GROUPS[g][0]][:MEM] + tot[GROUPS[g][1]][:MEM]
                        for g in (gw, gp)})
        if not first:
            add_h(s - 1, [(p, 1, tot[p][8:16]) for p in whole]
                  + [(p, z, tot[p][16 + 8 * z:24 + 8 * z]) for p in part for z in range(2)])
        add_h(s, [(p, 0, tot[p][8:16]) for p in part]
              + [(p, z, tot[p][16 + 8 * z:24 + 8 * z]) for p in whole for z in range(2)])
        return mem

    def wo_m1(slot, pairs):
        lhs = jnp.concatenate(
            [_rows(*[_get(o1, slot + k, a) for k in range(3)]) for a in pairs], axis=1)
        return _dot(lhs, _rows(*[wo_tile(0, a) for a in pairs]))

    def add_m1(s, r):
        for k in range(3):
            add_h(jnp.maximum(s + k, 0),
                  [(0, z, r[HS * k + 8 * z:HS * k + 8 * z + 8]) for z in range(2)])

    def mixer_norm(r0, keep=None):
        return _ln_tasks(lambda: hbuf[rows_of(PAD + r0, HS), :],
                         functools.partial(put, rows_of(HALO + r0, HS)), True, keep)

    def prologue(wt, qcar, stg, words, lhs1, lhs0, qkv0, mem0):
        def row_copy(src, i, n, sem):
            rows = pl.ds(_mult(i * n, n), n)
            return pltpu.make_async_copy(src.bitcast(u32).at[rows], words.at[rows],
                                         sems.at[sem + i])

        x_copy = lambda i: row_copy(x_hbm, i, S // 8, SEM_X)
        wo_copy = lambda g: row_copy(wo_hbm, g, 512, SEM_WO)

        def start_chunk(g, m):
            src = w_hbm[m].bitcast(u32)
            dst = stg.reshape(3 * HD, 8, DH)
            for par in range(2):
                pltpu.make_async_copy(
                    src.at[:, pl.ds(_mult(16 * par + 4 * g, 4), 4), :],
                    dst.at[pl.ds(HD * m, HD), pl.ds(4 * par, 4), :],
                    sems.at[SEM_W + 3 * g + m]).start()

        def wait_chunk(g, m):
            part = stg.at[pl.ds(_mult(4 * D * m, 4 * D), 4 * D)]
            pltpu.make_async_copy(part, part, sems.at[SEM_W + 3 * g + m]).wait()

        def operands(g, m, pair, i):
            w = [stg[pl.ds(4 * (D * m + HD * k + 16 * i) + pair, 16, stride=4), :]
                 for k in range(2)]
            quad = [pltpu.bitcast(w[q >> 1] & jnp.uint32(0xFFFF0000) if q & 1
                                  else w[q >> 1] << 16, f32) for q in range(4)]
            wt[3 * NP + m, pair, pl.ds(_mult(16 * i, 16), 16), :] = _rhs(0, quad.__getitem__).astype(bf16)
            for p in range(1, 7):
                wt[NP * m + 4 * g + pair, p - 1, pl.ds(_mult(16 * i, 16), 16), :] = _rhs(
                    p, quad.__getitem__).astype(bf16)

        def wo_operands(g, pair, i):
            c, r0 = i & 3, 8 * (i >> 2)
            w = [words[rows_of(DH * (4 * g + pair) + DH // 2 * (q >> 1) + r0, 8),
                       pl.ds(HD * (q & 1) + DH * c, DH)] for q in range(4)]
            quad = [_unpack(v).astype(f32) for v in w]
            for p in range(7):
                v = _rhs(p, quad.__getitem__).astype(bf16)
                wo_t[p, 4 * g + pair, c, pl.ds(2 * r0, 16), :] = v

        for i in range(4):
            if i == 3:
                start_chunk(0, 0)
            x_copy(i).start()
        mem_copy = pltpu.make_async_copy(mem0_hbm, mem0, sems.at[SEM_B + 3])
        mem_copy.start()
        start_chunk(0, 1)
        start_chunk(0, 2)
        for r0 in (0, HALO + S):
            put(pl.ds(r0, HALO), jnp.zeros((HALO, D), f32))
        for k in range(2):
            o1[k] = jnp.zeros((NP, HS, DH), bf16)
        @pl.loop(0, 4)
        def _(i):
            x_copy(i).wait()

            @pl.loop(0, 4, unroll=4)
            def _(k):
                r0 = pl.multiple_of(i * (S // 4) + k * 128, 128)
                xv = _unpack(words[pl.ds(pl.multiple_of(r0 // 2, 64), 64), :]).astype(f32)
                hbuf[pl.ds(PAD + r0, 128), :] = xv
                xn = _ln(xv)
                put(pl.ds(HALO + r0, 128), xn)
                v = _rows(*[xn[z:z + HS, :HD] + xn[z + HS:z + SEG, HD:]
                            for z in range(0, 128, SEG)])
                for c in range(4):
                    lhs1[c, pl.ds(pl.multiple_of(r0 // 2, 64), 64), :] = (
                        v[:, DH * c:DH * (c + 1)].astype(bf16))

        wait_chunk(0, 0)

        @pl.loop(0, HD // 16, step=4)
        def _(i):
            for k in range(4):
                for pair in range(4):
                    operands(0, 0, pair, i + k)

        mem_copy.wait()
        mem = mem0[...].astype(f32)
        cur, nxt = seg_quads(0), seg_quads(1)
        for p in range(1, 7):
            x0, x1 = _lhs(p, cur.__getitem__), _lhs(p, nxt.__getitem__)
            v = (_rows(x0, x1) if p in GROUPS[1]
                 else _rows(_row_lhs(p, mem[:, :HD], mem[:, HD:]), x1[:8], x0))
            for c in range(4):
                lhs0[p - 1, c] = v[:, DH * c:DH * (c + 1)].astype(bf16)

        def first(g, m, pair, i):
            n = S // 2 // M1_CUT
            lhs = _cols(*[_get(lhs1, c, rows=(n * i, n)) for c in range(4)])
            r = pltpu.bitcast(_dot(lhs, _get(wt, 3 * NP + m + here, pair)), u32)
            m1.bitcast(u32)[NP * m + 4 * g + pair, pl.ds(n * i, n), :] = r
            return r

        def project(g, m, pair):
            a = 4 * g + pair
            r = {p: _dot(_cols(*[_get(lhs0, p - 1, c) for c in range(4)]),
                         _get(wt, NP * m + a, p - 1))
                 for p in range(1, 7)}
            prod = {p: r[p][:HS] if p in GROUPS[1] else r[p][HS:] for p in r}
            prod[0] = pltpu.bitcast(m1.bitcast(u32)[NP * m + a, pl.ds(0, HS), :], f32)
            qcar[m, a] = _rows(*[r[p][HS:] for p in GROUPS[1]],
                               *[r[p][8:16] for p in GROUPS[2]])
            c_mem = _row_res({k: r[GROUPS[k][0]][:MEM] + r[GROUPS[k][1]][:MEM]
                              for k in (0, 2)})
            for n, v in enumerate(heads_of(c_mem, prod)):
                qkv0[m, a, n] = v

        def wo_tasks(g):
            return _held(words.at[pl.ds(H * DH // 2, 8), pl.ds(0, DH)],
                         _tasks(functools.partial(wo_operands, g), range(4), range(32)))

        @pl.loop(0, 11)
        def _(c):
            g, g2 = lax.div(c, 3), lax.div(c + 1, 3)
            m, m2 = c - 3 * g, c + 1 - 3 * g2
            for k in range(3):
                pl.when((m == k) & (g < 3))(functools.partial(start_chunk, g + 1, k))
            pl.when(c == 9)(lambda: _start([wo_copy(k) for k in range(4)]))
            wait_chunk(g2, m2)
            _interleave(_tasks(functools.partial(operands, g2, m2), range(4), range(HD // 16)),
                        _tasks(functools.partial(first, g, m), range(4), range(M1_CUT)))
            for pair in range(4):
                project(g, m, pair)

        @pl.loop(0, 2)
        def _(k):
            wo_copy(k).wait()
            _overlap(_tasks(lambda j, i: first(3, 2, 2 * k + j, i), range(2), range(M1_CUT)),
                     wo_tasks(k), 2)

        scores, outs, tot = {}, {}, {}
        none = jnp.zeros((3 * HS, DH), f32)

        def step0(t):
            if t < NP:
                scores[t] = [_scores(qkv0[0, t, n], qkv0[1, t, n]) for n in range(2)]
            if 0 <= t - 2 < NP:
                outs[t - 2] = [_attend(scores[t - 2][n], qkv0[2, t - 2, n]) for n in range(2)]
            if 0 <= t - 4 < NP:
                for p, v in wo_pass(0, t - 4, outs[t - 4], none, 2).items():
                    r = _dot(v, wo_tile(p, t - 4))
                    tot[p] = tot[p] + r if p in tot else r
                return r
            project(3, 2, t)
            return qkv0[0, t, 0]

        for k, slots in ((2, range(12)), (3, range(12, 16))):
            wo_copy(k).wait()
            _overlap(_tasks(step0, slots), wo_tasks(k), 1)
        _interleave(_tasks(step0, range(16, 20)))
        return wo_finish(0, 0, tot, first=True)

    def step(wt, qcar, s, phase, cur, nxt, first, mem, o1_slot, fillers, chores):
        gw, gp = (phase + 1) % 3, (phase + 2) % 3
        ahead, now = GROUPS[gw], GROUPS[gp]
        lhs = {}
        for p in ahead + now:
            x0, x1 = _lhs(p, cur.__getitem__), _lhs(p, nxt.__getitem__)
            riders = (x0[8:], x1) if p in ahead else (x1[:8], x0)
            lhs[p] = _rows(_row_lhs(p, *mem), *riders).astype(bf16)
        heads, scores, outs, tot = {}, {}, {}, {}

        def qkv(m, a):
            r = {p: _dot(lhs[p], _get(wt, NP * m + a, p - 1)) for p in lhs}
            _release(r[now[1]], _share(chores, len(heads), 3 * NP - CH0))
            old = qcar[m, a]
            prod = {0: pltpu.bitcast(first(NP * m + a), f32)}
            for k in range(2):
                prod[GROUPS[phase][k]] = old[HS * k:HS * k + HS]
                prod[ahead[k]] = _rows(old[SEG + 8 * k:SEG + 8 * k + 8],
                                       r[ahead[k]][8:16])
                prod[now[k]] = r[now[k]][HS:]
            qcar[m, a] = _rows(*[r[p][HS:] for p in ahead], *[r[p][8:16] for p in now])
            c_mem = _row_res({g: r[GROUPS[g][0]][:MEM] + r[GROUPS[g][1]][:MEM]
                              for g in (gw, gp)})
            heads[m, a] = heads_of(c_mem, prod)

        for t in range(NP + LAG_WO):
            a = t - LAG_QK
            if 0 <= a < NP:
                scores[a] = [_scores(heads[0, a][n], heads[1, a][n]) for n in range(2)]
            a = t - LAG_PV
            if 0 <= a < NP:
                outs[a] = [_attend(scores[a][n], heads[2, a][n]) for n in range(2)]
            if t < NP:
                for m in range(3):
                    qkv(m, t)
            if t == FILL_AT:
                fillers[0]()
            a = t - LAG_WO
            if 0 <= a < NP:
                for p, v in wo_pass(phase, a, outs[a], ocar[a], o1_slot).items():
                    r = _dot(v, wo_tile(p, a))
                    tot[p] = tot[p] + r if p in tot else r
        fillers[1]()
        return wo_finish(phase, s, tot)

    def recurrence(wt, qcar, mem, raw, fin):
        _start(b_copies(raw))
        spare = 128 * (NC + 4)
        raw[pl.ds(0, 16), pl.ds(spare, 8), :] = jnp.zeros((16, 8, DH), u32)

        def chores(i):
            def convert(dst, base, per, groups):
                tasks = []
                for k in range(per):
                    r = pl.multiple_of(8 * jnp.clip(per * (i - 2) + k, 0, groups - 1), 8)
                    r0 = pl.multiple_of(jnp.where(i > 1, base + r, spare), 8)
                    tasks += _tasks(functools.partial(
                        b_operands, lambda k, n, r0=r0: raw[4 * n + k, pl.ds(r0, 8), :],
                        dst, r), range(7))
                return _held(raw.at[16, pl.ds(0, 8)], tasks)
            rest = convert(w12, 128 * NC, 4, 64)
            norm = _abreast(
                [mixer_norm(jnp.maximum(3 * i - 5 + (k >> 1), 0) * SEG + (k & 1) * HS,
                            fin.at[rows_of(HS * k, HS)])
                 for k in range(6)], 6)
            in_h = hbuf.at[pl.ds(0, 8), pl.ds(0, DH)]
            norm = (_held(in_h, norm[:36])
                    + _held(fin.at[pl.ds(3 * SEG, 8), pl.ds(0, DH)], norm[36:]))

            def due():
                m1.bitcast(u32)[3 * NP + here, pl.ds(S // 2 - 8, 8), :] = pltpu.bitcast(
                    xg[here, pl.ds(0, 8), :], u32)
            last = _merge(convert(m1, 0, 6, 16 * NC), norm[36:] + [(norm[-1][0], due)])
            return _merge(rest[:14], norm[:12]), _merge(rest[14:], norm[12:36]), last

        def steps(i, mem):
            pl.when(i == 2)(lambda: _wait(b_copies(raw)))
            src = 3 * (i & 1)
            acc = []

            def filler(n):
                if CUTS[n] < CUTS[n + 1]:
                    acc.append(wo_m1(src, range(CUTS[n], CUTS[n + 1])))
                    if CUTS[n + 1] == NP:
                        add_m1(3 * i - 2, functools.reduce(lambda u, v: u + v, acc))

            todo = chores(i)
            filler(0)
            nxt = seg_quads(3 * i + 1)
            for k in range(3):
                fillers = _tasks(filler, (2 * k + 1, 2 * k + 2))
                rows = pl.ds(pl.multiple_of((3 * i + 1 + k) * HS, HS), HS)
                first = lambda j: m1.bitcast(u32)[j, rows, :]
                if k == 2:
                    early = {j: first(j) for j in range(3 * NP) if j % NP < DUE}
                    first = lambda j, late=first: early[j] if j in early else late(j)
                cur, nxt = nxt, seg_quads(jnp.minimum(3 * i + 2 + k, NSEG - 1))
                mem = step(wt, qcar, 3 * i + 1 + k, (1 + k) % 3, cur, nxt, first, mem,
                           3 - src + k, fillers, todo[k])
            return mem

        lax.fori_loop(0, NSEG // 3, steps, mem)

    def block_a(wt, qcar):
        mem = pl.run_scoped(
            functools.partial(prologue, wt, qcar),
            pltpu.VMEM((12 * D, DH), u32),
            pltpu.VMEM((H * DH // 2 + 8, D), u32),
            pltpu.VMEM((4, S // 2, DH), bf16),
            pltpu.VMEM((6, 4, SEG, DH), bf16),
            pltpu.VMEM((3, NP, 2, L, DH), f32),
            pltpu.VMEM((MEM, D), bf16))

        pl.run_scoped(functools.partial(recurrence, wt, qcar, mem),
                      pltpu.VMEM((17, 128 * (NC + 4) + 8, DH), u32),
                      pltpu.VMEM((3 * SEG + 8, D), f32))

    pl.run_scoped(block_a, pltpu.VMEM((3 * NP + 3, 6, HD, DH), bf16),
                  pltpu.VMEM((3, NP, 3 * HS, DH), f32))

    def block_b(w4t, x1b, yn, ya, *pu):
        in_h = hbuf.at[pl.ds(0, 8), pl.ds(0, DH)]
        in_y = yn.at[pl.ds(RB, 8), pl.ds(0, DH)]
        pu = [pu[c % 3] for c in range(NC)]
        def wo_last():
            phase = NSEG % 3
            tot = {}

            def task(a0, p, r0=0, n=0):
                pairs = range(a0, a0 + 2)
                if p == 0:
                    r = wo_m1(3 * (NSEG // 3 & 1), pairs)
                else:
                    lhs = _cols(*[ocar[a, pl.ds(r0, n), :] for a in pairs])
                    r = _dot(lhs.astype(bf16), _rows(*[wo_tile(p, a) for a in pairs]))
                tot[p] = tot[p] + r if a0 else r
                if a0 == NP - 2 and p == 0:
                    add_m1(NSEG - 3, tot[p])
                elif a0 == NP - 2:
                    add_h(NSEG - 1, [(p, 1, tot[p][-8:])] + [(p, 0, tot[p][:8])] * (n > 8))
                return r

            todo = [(0,)] + [t for k in range(2) for t in (
                (GROUPS[(phase + 2) % 3][k], HS * k, HS),
                (GROUPS[(phase + 1) % 3][k], SEG + 8 * k, 8))]
            return [functools.partial(task, a0, *t) for t in todo for a0 in range(0, NP, 2)]

        def a_operands(load, dst):
            def task(g, p1):
                r0, c = 16 * (g >> 1), g & 1
                for p0, v in enumerate(_twice(
                        _lhs, lambda i, k: load(i * R + r0, 2 * k + c), p1)):
                    dst[7 * p1 + p0, c, pl.ds(r0, 16), :] = v.astype(bf16)
            return _tasks(task, range(R // 8), range(7))

        def products(src, w, r0, dst):
            m = {}

            def task(p1, p0):
                p = 7 * p1 + p0
                m[p0] = _dot(_cols(*[_get(src, p + here, k) for k in range(2)]),
                             _get(w, p, rows=(r0, C4)))
                if p0 >= 3:
                    j = (2, 1, 3, 0)[p0 - 3]
                    dst[p1, j] = _res(j, m.__getitem__)
                return m[p0]
            return _tasks(task, range(7), range(7))

        def mlp_in(b):
            def residual(r0, y):
                x1 = y + x1b[rows_of(b * RB + r0, 16), :]
                yn[pl.ds(r0, 16), :] = x1
                put(rows_of(b * RB + r0, 16), hbuf[rows_of(PAD + b * RB + r0, 16), :] + x1)

            def store(r0, y):
                yn[pl.ds(r0, 16), :] = y
                return y

            return _held(in_h, _abreast([
                _ln_tasks(lambda r0=r0: hbuf[rows_of(PAD + b * RB + r0, 16), :],
                          functools.partial(residual, r0)) for r0 in range(0, RB, 16)], RB // 16)
            ) + _held(in_y, _abreast([
                _ln_tasks(lambda r0=r0: yn[rows_of(r0, 16), :],
                          functools.partial(store, r0)) for r0 in range(0, RB, 16)], RB // 16)
                + a_operands(
                lambda r0, c: yn[rows_of(r0, 16), pl.ds(DH * c, DH)], ya))

        def ups(c):
            return products(ya, m1, C4 * c, pu[c])

        def mixer(raw, *bufs):
            sa, sp = bufs[:2], (bufs[2:4], bufs[4:])
            in_g = xg.at[0, pl.ds(S + 2 * HALO, 8)]
            w4_copies = [pltpu.make_async_copy(
                w4_hbm.bitcast(u32).at[pl.ds(c, n)], raw.at[pl.ds(c, n)], sems.at[SEM_B + s])
                for c, n, s in ((0, 2, 1), (2, NC - 2, 2))]
            _start(w4_copies)

            def pre(n, w, b):
                shift = lambda c: w * (-1, 1, -2, 2)[c >> 1]
                return _held(in_g, a_operands(lambda r0, c: xg[c + here, pl.ds(
                    HALO + b * RB + r0 + shift(c), 16), :], sa[n & 1]))

            def post(n, w, b):
                def task(g, j):
                    c, g = divmod(g, R // 8)
                    m = [sp[n & 1][c][p1 + here, j, pl.ds(8 * g, 8), :]
                         for p1 in range(7)]
                    for q in range(4):
                        i, k = _pos(q, j)
                        r0 = _mult(b * RB + i * R + 8 * g, 8)
                        v = _res(q, m.__getitem__)
                        if w == 0:
                            xg[2 * k + c, pl.ds(HALO + r0, 8), :] = _gelu2(v)
                        else:
                            x1b[pl.ds(r0, 8), pl.ds(DH * (2 * k + c), DH)] = 0.5 * v
                return [t for c in range(2) for t in _held(
                    sp[n & 1][c].at[7, 0, pl.ds(0, 8)],
                    _tasks(task, range(R // 8 * c, R // 8 * (c + 1)), range(4)))]

            def unit(n, w, *side):
                dots = [t for c in range(2) for t in products(
                    sa[n & 1], w12, C4 * (2 * w + c), sp[n & 1][c])]
                _overlap(dots, _merge(*side), MX_LAG)

            def w4_work(k, n, half=0):
                def task(i, p1):
                    g, c = half + (i >> 1), i & 1
                    r0 = _mult(8 * (g & 7), 8)
                    b_operands(lambda q, j: raw[(g >> 3) + here, q, pl.ds(r0, 8),
                                                pl.ds(DH * (2 * j + c), DH)],
                               w4t, _mult(DH * (g >> 3) + 64 * c + r0, 8), p1)
                return _held(raw.at[NC, 0, pl.ds(0, 8), pl.ds(0, DH)],
                             _tasks(task, range(k, k + n), range(7)))

            norms = lambda s: _held(in_h, _abreast(
                [mixer_norm(s * SEG + k * HS) for k in range(6)], 3))
            _overlap(wo_last(), _merge(pre(0, 0, 0), norms(NSEG - 6)), MX_LAG)
            unit(0, 0, pre(1, 0, 1), norms(NSEG - 3))
            _wait(w4_copies[:1])

            @pl.loop(0, 3)
            def _(i):
                pl.when(i == 2)(lambda: _wait(w4_copies[1:]))
                for n in range(2):
                    b = 2 * i + 1 + n
                    unit(n + 1, 0, pre(n, 0, b + 1), post(n, 0, b - 1),
                         w4_work(G1 * n, G1, G1 * i))

            unit(1, 0, pre(0, 1, 0), post(0, 0, 6), w4_work(6 * G1, G1))
            unit(0, 1, pre(1, 1, 1), post(1, 0, 7), w4_work(7 * G1, G1))

            @pl.loop(0, 2)
            def _(i):
                for n in range(2):
                    b = 2 * i + 1 + n
                    unit(n + 1, 1, pre(n, 1, b + 1), post(n, 1, b - 1),
                         w4_work(8 * G1 + G2 * n, G2, G2 * i))

            done = 8 * G1 + 4 * G2
            rest = w4_work(done, 16 * NC - done)
            ahead = mlp_in(0)
            for b in range(5, NB):
                unit(b, 1, pre(b + 1, 1, b + 1) if b + 1 < NB else _share(rest, 2, 4),
                     post(b - 1, 1, b - 1), _share(ahead, b - 5, 3),
                     _share(rest, (0, 1, 3)[b - 5], 4))
            for _, task in post(1, 1, NB - 1):
                task()

        def mlp(ta0, ta1, pd, ob):
            ta = [ta0.at[c] for c in range(NC - 1)] + [ta1]

            def mid(c, g, j):
                r = pl.ds(8 * g, 8)
                m = [pu[c][p1 + here, j, r, :] for p1 in range(7)]
                y = [_gelu2(_res(q, m.__getitem__)) for q in range(4)]
                for p1 in range(7):
                    v = _lhs(p1, y.__getitem__)
                    ta[c][p1, j, r, :] = v
                return v

            def down(b, m, p, c):
                p1, p0 = divmod(p, 7)
                lhs = _lhs(p0, lambda j: ta[c][p1 + here, j]).astype(bf16)
                tot = _dot(lhs, jnp.concatenate(
                    [_get(w4t, p, rows=(C4 * c + 128 * k, 128)) for k in range(2)],
                    axis=1))
                m[p] = m[p] + tot if c else tot
                if c == NC - 1 and p0 >= 3:
                    j = (2, 1, 3, 0)[p0 - 3]
                    v = _res(j, lambda k: m[7 * p1 + k])
                    if p1 < 6:
                        pd[p1, j] = v
                    if p1 >= 3:
                        q = (2, 1, 3, 0)[p1 - 3]
                        i, n = _pos(q, j)
                        r0, cols = _mult(b * RB + i * R, R), pl.ds(n * C4, C4)
                        v = _res(q, lambda k: v if k == p1 else pd[k + here, j])
                        ob[pl.ds(r0, R), cols] = (
                            _cols(*[xg[2 * n + k, pl.ds(r0, R), :] for k in range(2)]) + 0.5 * v).astype(bf16)
                return tot

            def out_copy(b):
                rows = pl.ds(_mult(b * RB, RB), RB)
                return pltpu.make_async_copy(ob.at[rows], out_hbm.at[rows],
                                             sems.at[SEM_OUT + b])

            @pl.loop(0, NB)
            def _(b):
                mids = lambda c: _held(pu[c].at[7, 0, pl.ds(0, 8)], _tasks(
                    functools.partial(mid, c), range(R // 8), range(4)))
                task = functools.partial(down, b, {})
                early = _tasks(task, range(EARLY), range(NC - 1))
                ahead = mlp_in(jnp.minimum(b + 1, NB - 1))
                _overlap(ups(0), ahead[:A0], 0)
                for c in range(NC):
                    _overlap(ups(c + 1) if c + 1 < NC else early,
                             _merge(mids(c), _share(ahead[A0:AH], c, NC - 1)), UP_LAG)

                _overlap(_tasks(task, range(EARLY), [NC - 1])
                         + _tasks(task, range(EARLY, 49), range(NC)),
                         ahead[AH:], DN_LAG)
                out_copy(b).start()

            for b in range(NB):
                out_copy(b).wait()

        pl.run_scoped(mixer, pltpu.VMEM((NC + 1, 4, 64, D), u32),
                      *[pltpu.VMEM((49, 2, R, DH), bf16)] * 2,
                      *[pltpu.VMEM((8, 4, R, DH), f32)] * 4)
        pl.run_scoped(mlp, pltpu.VMEM((NC - 1, 7, 4, R, DH), f32),
                      pltpu.VMEM((7, 4, R, DH), f32),
                      pltpu.VMEM((6, 4, R, C4), f32), pltpu.VMEM((S, D), bf16))

    pl.run_scoped(
        block_b,
        pltpu.VMEM((49, C4 * NC, DH), bf16),
        pltpu.VMEM((S, D), f32),
        pltpu.VMEM((RB + 8, D), f32),
        pltpu.VMEM((49, 2, R, DH), bf16),
        *[pltpu.VMEM((8, 4, R, 128), f32)] * 3)


@jax.jit
def pallas_sequential_preLN__memory_aug_recurrent_mem_tr__mixer_s_mlp__prompt_kernel(
    A_x: jax.Array,
    A_mem0: jax.Array,
    A_Wq: jax.Array,
    A_Wk: jax.Array,
    A_Wv: jax.Array,
    A_Wo: jax.Array,
    A_seg_len: jax.Array,
    B_x: jax.Array,
    B_w1: jax.Array,
    B_w2: jax.Array,
    B_w3: jax.Array,
    B_w4: jax.Array,
):
    del A_seg_len, B_x
    hbm = pl.BlockSpec(memory_space=pl.ANY)
    scratch = [
        pltpu.VMEM((PAD + S, D), f32),
        pltpu.VMEM((8, S + 3 * HALO, DH), f32),
        pltpu.VMEM((7, NP, 4, DH, DH), bf16),
        pltpu.VMEM((6, NP, HS, DH), bf16),
        pltpu.VMEM((NP, 3 * HS, DH), f32),
        pltpu.VMEM((49, S, DH), bf16),
        pltpu.VMEM((49, D, DH), bf16),
        pltpu.SemaphoreType.DMA((NSEM,)),
    ]
    out = pl.pallas_call(
        _kernel,
        out_shape=jax.ShapeDtypeStruct((S, D), A_x.dtype),
        in_specs=[hbm] * 10,
        out_specs=hbm,
        scratch_shapes=scratch,
        compiler_params=pltpu.CompilerParams(vmem_limit_bytes=127 * 1024 * 1024),
    )(A_x.reshape(S, D), A_mem0.reshape(MEM, D),
      A_Wq.reshape(D // 2, 2 * H, DH), A_Wk.reshape(D // 2, 2 * H, DH),
      A_Wv.reshape(D // 2, 2 * H, DH),
      A_Wo.reshape(H * DH, D), B_w1.reshape(4, C4, D), B_w2.reshape(4, C4, D),
      B_w3.reshape(4, C4, F), B_w4.reshape(NC, 4, FC // 4, D))
    return out.reshape(A_x.shape)
```

```python
import functools

import jax
import jax.numpy as jnp
from jax import lax
import jax.experimental.pallas as pl
import jax.experimental.pallas.tpu as pltpu

S = 2048
D = 1024
H = 32
DH = 128
MEM = 8
SEG = 32
F = 3584
NSEG = S // SEG
L = MEM + SEG
HS = SEG // 2
NP = H // 2
HD = D // 2
PAD = 8
C4 = D // 4
HALO = 8
R = 64
RB = 4 * R
NB = S // RB
FC = 512
NC = F // FC
EPS = 1e-5
NEG = -1000000000.0

LAG_QK = 2
LAG_PV = 4
LAG_WO = 6
FILL_AT = 19
CUTS = (0, 2, 4, 8, 10, 14, 16, 16)
CH0 = 20
DUE = 15
M1_CUT = 16
G1 = 8
G2 = 11
A0 = 32
AH = 80
EARLY = 14
MX_LAG = 5
UP_LAG = 10
DN_LAG = 20

GROUPS = ((1, 3), (2, 4), (5, 6))
TARGETS = (((0, 1), (3, 1)), ((2, 1), (3, -1)), ((1, 1), (3, 1)), ((0, 1), (2, 1)),
           ((0, -1), (1, 1)), ((3, 1),), ((0, 1),))

bf16 = jnp.bfloat16
f32 = jnp.float32
u32 = jnp.uint32

SEM_X, SEM_W, SEM_WO, SEM_B, SEM_OUT = 0, 4, 16, 20, 24
NSEM = SEM_OUT + NB


def _mult(i, n):
    return i if isinstance(i, int) else pl.multiple_of(i, n)


def _ln(x):
    m = jnp.mean(x, axis=-1, keepdims=True)
    d = x - m
    v = jnp.mean(d * d, axis=-1, keepdims=True)
    return d * lax.rsqrt(v + EPS)


def _gelu2(x):
    c = 0.7978845608028654
    return x + x * jnp.tanh(x * (c + (c * 0.044715) * (x * x)))


def _get(ref, *idx, rows=None):
    rows = slice(None) if rows is None else pl.ds(rows[0] // 2, rows[1] // 2)
    return _unpack(ref.bitcast(u32)[idx + (rows, slice(None))])


def _cols(*xs):
    return jnp.concatenate(xs, axis=1)


def _unpack(x):
    return pltpu.bitcast(x, bf16)


def _dot(a, b):
    return jnp.dot(a, b, preferred_element_type=f32)


def _rows(*xs):
    return jnp.concatenate(xs, axis=0)


def _lhs(p, a):
    return (lambda: a(0) + a(3), lambda: a(2) + a(3), lambda: a(0), lambda: a(3),
            lambda: a(0) + a(1), lambda: a(2) - a(0), lambda: a(1) - a(3))[p]()


def _rhs(p, b):
    return (lambda: b(0) + b(3), lambda: b(0), lambda: b(1) - b(3), lambda: b(2) - b(0),
            lambda: b(3), lambda: b(0) + b(1), lambda: b(2) + b(3))[p]()


def _res(q, m):
    return (lambda: m(0) + m(3) - m(4) + m(6), lambda: m(2) + m(4),
            lambda: m(1) + m(3), lambda: m(0) - m(1) + m(2) + m(5))[q]()


def _pos(q, j):
    return 2 * (q >> 1) + (j >> 1), 2 * (q & 1) + (j & 1)


def _twice(side, blk, p1):
    outer = [side(p1, lambda q: blk(*_pos(q, j))) for j in range(4)]
    return [side(p0, outer.__getitem__) for p0 in range(7)]


def _ln_tasks(load, store, twice=False, keep=None):
    st = {}

    def fold(x):
        return functools.reduce(
            lambda u, v: u + v, [x[:, c:c + DH] for c in range(0, D, DH)])

    def part():
        st["s"] = fold(load())

    def mean():
        st["m"] = jnp.sum(st["s"], axis=-1, keepdims=True) * (1.0 / D)

    def square():
        d = load() - st["m"]
        st["s"] = fold(d * d)
        if keep:
            keep[...] = d

    def var():
        st["v"] = jnp.sum(st["s"], axis=-1, keepdims=True) * (1.0 / D)

    def scale():
        st["r"] = lax.rsqrt(st["v"] + EPS)

    def again():
        st["r"] = st["r"] * lax.rsqrt(st["v"] * st["r"] * st["r"] + EPS)

    def apply():
        store((keep[...] if keep else load() - st["m"]) * st["r"])

    if twice:
        return [part, mean, square, var, scale, again, apply]
    return [lambda: (part(), mean()), lambda: (square(), var(), scale()), apply]


def _abreast(chains, n):
    return [t for i in range(0, len(chains), n) for ts in zip(*chains[i:i + n]) for t in ts]


def _row_lhs(p, a1, a2):
    return a1 + a2 if p in (1, 4) else a1 if p in (2, 5) else a2


def _row_res(t):
    if 0 not in t:
        return t[2] - t[1], t[1]
    if 1 not in t:
        return t[0], t[2] - t[0]
    return t[0], t[1]


def _merge(*lists):
    order = sorted(((i + 0.5) / len(l), n, i)
                   for n, l in enumerate(lists) for i in range(len(l)))
    return [lists[n][i] for _, n, i in order]


def _interleave(*lists):
    for task in _merge(*lists):
        task()


def _held(spare, tasks):
    return [(spare, task) for task in tasks]


def _overlap(dots, side, lag):
    for i, dot in enumerate(dots):
        _release(dot(), _share(side, i, len(dots) - lag))


def _release(result, mine):
    for spare in {id(spare): spare for spare, _ in mine}.values():
        spare[...] = pltpu.bitcast(result[-8:, -DH:], spare.dtype)
    for _, task in mine:
        task()


def _share(tasks, k, n):
    return tasks[len(tasks) * k // n:len(tasks) * (k + 1) // n] if k >= 0 else []


def _tasks(fn, *ranges):
    if len(ranges) == 2:
        return [functools.partial(fn, i, j) for i in ranges[0] for j in ranges[1]]
    return [functools.partial(fn, i) for i in ranges[0]]


def _start(copies):
    for c in copies:
        c.start()


def _wait(copies):
    for c in copies:
        c.wait()


def _scores(q, k):
    return lax.dot_general(q, k, (((1,), (1,)), ((), ())), preferred_element_type=f32)


def _attend(sc, v):
    ri = lax.broadcasted_iota(jnp.int32, (L, L), 0)
    ci = lax.broadcasted_iota(jnp.int32, (L, L), 1)
    sc = jnp.where((ri < MEM) | (ri >= ci), sc, NEG * DH ** 0.5)
    mx = jnp.max(sc, axis=1, keepdims=True)
    e = jnp.exp2((sc - mx) * (DH ** -0.5 * 1.4426950408889634))
    den = jnp.sum(e, axis=1, keepdims=True)
    inv = pl.reciprocal(den, approx=True)
    inv = inv * (2.0 - den * inv)
    return _dot(e, v) * inv


def _kernel(x_hbm, mem0_hbm, wq_hbm, wk_hbm, wv_hbm, wo_hbm, w1_hbm, w2_hbm,
            w3_hbm, w4_hbm, out_hbm, hbuf, xg, wo_t, o1, late, ocar, m1, w12, sems):
    w_hbm = (wq_hbm, wk_hbm, wv_hbm)
    here = lax.fori_loop(0, 2, lambda i, z: z + (i >> 1), jnp.int32(0))

    def b_copies(raw):
        tile = lambda w, i: w.bitcast(u32).at[:, :, pl.ds(128 * i, 128)]
        for n in range(4):
            slabs = pl.ds(4 * n, 4)
            for i, w in enumerate((w1_hbm, w2_hbm)):
                for c in range(2):
                    yield pltpu.make_async_copy(
                        tile(w, 2 * n + c),
                        raw.at[slabs, pl.ds(128 * (NC + 2 * i + c), 128)],
                        sems.at[SEM_B])
            for c in range(NC):
                yield pltpu.make_async_copy(
                    tile(w3_hbm, 4 * c + n), raw.at[slabs, pl.ds(128 * c, 128)],
                    sems.at[SEM_B])

    def b_operands(raw, dst, r1, p1):
        for p0, v in enumerate(_twice(_rhs, lambda k, n: _unpack(raw(k, n)).astype(f32), p1)):
            if p1 in (1, 4) and p0 in (1, 4):
                k = 2 * (p1 // 4) + p0 // 4
                dst.bitcast(u32)[7 * p1 + p0, pl.ds(r1, 8), :] = raw(k, k)
            else:
                dst[7 * p1 + p0, pl.ds(_mult(2 * r1, 16), 16), :] = v.astype(bf16)

    def rows_of(r0, n):
        return pl.ds(pl.multiple_of(r0 + here, 8), n)

    def put(rows, x):
        for c in range(8):
            xg[c, rows, :] = x[:, DH * c:DH * (c + 1)]

    def wo_tile(p, a):
        return _cols(*[_get(wo_t, p, a, c) for c in range(4)])

    def seg_quads(s):
        r0 = HALO + s * SEG
        return [jnp.concatenate(
            [xg[4 * (q & 1) + c, pl.ds(_mult(r0 + (q >> 1) * HS, 8), HS), :]
             for c in range(4)], axis=1) for q in range(4)]

    def heads_of(c_mem, m):
        return [_rows(c_mem[n], _res(n, m.__getitem__), _res(2 + n, m.__getitem__))
                for n in range(2)]

    def wo_pass(phase, a, o, prev, o1_slot):
        whole, part = GROUPS[(phase + 1) % 3], GROUPS[(phase + 2) % 3]
        quad = lambda q: o[q & 1][MEM + (q >> 1) * HS:MEM + (q >> 1) * HS + HS]
        x = [_lhs(p, quad) for p in range(7)]
        o1[o1_slot, a] = x[0].astype(bf16)
        ocar[a] = _rows(*[x[p] for p in GROUPS[phase]], *[x[p][8:] for p in part])
        res = {}
        for k in range(2):
            for p, riders in ((whole[k], (prev[SEG + 8 * k:SEG + 8 * k + 8], x[whole[k]])),
                              (part[k], (x[part[k]][:8], prev[HS * k:HS * k + HS]))):
                lhs = _rows(_row_lhs(p, o[0][:MEM], o[1][:MEM]), *riders)
                res[p] = lhs.astype(bf16)
        return res

    def add_h(s, terms):
        for q in range(4):
            for z in range(2):
                mine = [(sign, v) for p, zz, v in terms if zz == z
                        for qq, sign in TARGETS[p] if qq == q]
                if mine:
                    at = (pl.ds(_mult(PAD + s * SEG + (q >> 1) * HS + 8 * z, 8), 8),
                          pl.ds((q & 1) * HD, HD))
                    acc = hbuf[at]
                    for sign, v in mine:
                        acc = acc + v if sign > 0 else acc - v
                    hbuf[at] = acc

    def wo_tokens(phase, s, rows):
        whole, part = GROUPS[(phase + 1) % 3], GROUPS[(phase + 2) % 3]
        for k, one, two in ((jnp.maximum(s - 1, 0), whole, part), (s, part, whole)):
            add_h(k, [(p, int(one is whole), rows(p, 0)) for p in one]
                  + [(p, z, rows(p, 8 + 8 * z)) for p in two for z in range(2)])

    def wo_finish(phase, s, tot):
        if phase:
            wo_tokens(phase, s, lambda p, r0: tot[p][MEM + r0:MEM + r0 + 8])
        else:
            for p in tot:
                late[p] = tot[p][MEM:]
        return _row_res({g: tot[GROUPS[g][0]][:MEM] + tot[GROUPS[g][1]][:MEM]
                         for g in range(3) if g != phase})

    def wo_late(s):
        wo_tokens(0, s, lambda p, r0: late[p + here, pl.ds(r0, 8), :])

    def wo_m1(slot, pairs):
        lhs = jnp.concatenate(
            [_rows(*[_get(o1, slot + k, a) for k in range(3)]) for a in pairs], axis=1)
        return _dot(lhs, _rows(*[wo_tile(0, a) for a in pairs]))

    def add_m1(s, r):
        for k in range(3):
            add_h(jnp.maximum(s + k, 0),
                  [(0, z, r[HS * k + 8 * z:HS * k + 8 * z + 8]) for z in range(2)])

    def mixer_norm(r0, keep=None):
        return _ln_tasks(lambda: hbuf[rows_of(PAD + r0, HS), :],
                         functools.partial(put, rows_of(HALO + r0, HS)), True, keep)

    def prologue(wt, qcar, stg, words, lhs1, lhs0, qkv0, mem0):
        def row_copy(src, i, n, sem):
            rows = pl.ds(_mult(i * n, n), n)
            return pltpu.make_async_copy(src.bitcast(u32).at[rows], words.at[rows],
                                         sems.at[sem + i])

        x_copy = lambda i: row_copy(x_hbm, i, S // 8, SEM_X)
        wo_copy = lambda g: row_copy(wo_hbm, g, 512, SEM_WO)

        def start_chunk(g, m):
            src = w_hbm[m].bitcast(u32)
            dst = stg.reshape(3 * HD, 8, DH)
            for par in range(2):
                pltpu.make_async_copy(
                    src.at[:, pl.ds(_mult(16 * par + 4 * g, 4), 4), :],
                    dst.at[pl.ds(HD * m, HD), pl.ds(4 * par, 4), :],
                    sems.at[SEM_W + 3 * g + m]).start()

        def wait_chunk(g, m):
            part = stg.at[pl.ds(_mult(4 * D * m, 4 * D), 4 * D)]
            pltpu.make_async_copy(part, part, sems.at[SEM_W + 3 * g + m]).wait()

        def operands(g, m, pair, i):
            w = [stg[pl.ds(4 * (D * m + HD * k + 16 * i) + pair, 16, stride=4), :]
                 for k in range(2)]
            quad = [pltpu.bitcast(w[q >> 1] & jnp.uint32(0xFFFF0000) if q & 1
                                  else w[q >> 1] << 16, f32) for q in range(4)]
            wt[3 * NP + m, pair, pl.ds(_mult(16 * i, 16), 16), :] = _rhs(0, quad.__getitem__).astype(bf16)
            for p in range(1, 7):
                wt[NP * m + 4 * g + pair, p - 1, pl.ds(_mult(16 * i, 16), 16), :] = _rhs(
                    p, quad.__getitem__).astype(bf16)

        def wo_operands(g, pair, i):
            c, r0 = i & 3, 8 * (i >> 2)
            w = [words[rows_of(DH * (4 * g + pair) + DH // 2 * (q >> 1) + r0, 8),
                       pl.ds(HD * (q & 1) + DH * c, DH)] for q in range(4)]
            quad = [_unpack(v).astype(f32) for v in w]
            for p in range(7):
                v = _rhs(p, quad.__getitem__).astype(bf16)
                wo_t[p, 4 * g + pair, c, pl.ds(2 * r0, 16), :] = v

        for i in range(4):
            if i == 3:
                start_chunk(0, 0)
            x_copy(i).start()
        mem_copy = pltpu.make_async_copy(mem0_hbm, mem0, sems.at[SEM_B + 3])
        mem_copy.start()
        start_chunk(0, 1)
        start_chunk(0, 2)
        for r0 in (0, HALO + S):
            put(pl.ds(r0, HALO), jnp.zeros((HALO, D), f32))
        for k in range(2):
            o1[k] = jnp.zeros((NP, HS, DH), bf16)
        @pl.loop(0, 4)
        def _(i):
            x_copy(i).wait()

            @pl.loop(0, 4, unroll=4)
            def _(k):
                r0 = pl.multiple_of(i * (S // 4) + k * 128, 128)
                xv = _unpack(words[pl.ds(pl.multiple_of(r0 // 2, 64), 64), :]).astype(f32)
                hbuf[pl.ds(PAD + r0, 128), :] = xv
                xn = _ln(xv)
                put(pl.ds(HALO + r0, 128), xn)
                v = _rows(*[xn[z:z + HS, :HD] + xn[z + HS:z + SEG, HD:]
                            for z in range(0, 128, SEG)])
                for c in range(4):
                    lhs1[c, pl.ds(pl.multiple_of(r0 // 2, 64), 64), :] = (
                        v[:, DH * c:DH * (c + 1)].astype(bf16))

        wait_chunk(0, 0)

        @pl.loop(0, HD // 16, step=4)
        def _(i):
            for k in range(4):
                for pair in range(4):
                    operands(0, 0, pair, i + k)

        mem_copy.wait()
        mem = mem0[...].astype(f32)
        cur, nxt = seg_quads(0), seg_quads(1)
        for p in range(1, 7):
            x0, x1 = _lhs(p, cur.__getitem__), _lhs(p, nxt.__getitem__)
            v = (_rows(x0, x1) if p in GROUPS[1]
                 else _rows(_row_lhs(p, mem[:, :HD], mem[:, HD:]), x1[:8], x0))
            for c in range(4):
                lhs0[p - 1, c] = v[:, DH * c:DH * (c + 1)].astype(bf16)

        def first(g, m, pair, i):
            n = S // 2 // M1_CUT
            lhs = _cols(*[_get(lhs1, c, rows=(n * i, n)) for c in range(4)])
            r = pltpu.bitcast(_dot(lhs, _get(wt, 3 * NP + m + here, pair)), u32)
            m1.bitcast(u32)[NP * m + 4 * g + pair, pl.ds(n * i, n), :] = r
            return r

        def project(g, m, pair):
            a = 4 * g + pair
            r = {p: _dot(_cols(*[_get(lhs0, p - 1, c) for c in range(4)]),
                         _get(wt, NP * m + a, p - 1))
                 for p in range(1, 7)}
            prod = {p: r[p][:HS] if p in GROUPS[1] else r[p][HS:] for p in r}
            prod[0] = pltpu.bitcast(m1.bitcast(u32)[NP * m + a, pl.ds(0, HS), :], f32)
            qcar[m, a] = _rows(*[r[p][HS:] for p in GROUPS[1]],
                               *[r[p][8:16] for p in GROUPS[2]])
            c_mem = _row_res({k: r[GROUPS[k][0]][:MEM] + r[GROUPS[k][1]][:MEM]
                              for k in (0, 2)})
            for n, v in enumerate(heads_of(c_mem, prod)):
                qkv0[m, a, n] = v

        def wo_tasks(g):
            return _held(words.at[pl.ds(H * DH // 2, 8), pl.ds(0, DH)],
                         _tasks(functools.partial(wo_operands, g), range(4), range(32)))

        @pl.loop(0, 11)
        def _(c):
            g, g2 = lax.div(c, 3), lax.div(c + 1, 3)
            m, m2 = c - 3 * g, c + 1 - 3 * g2
            for k in range(3):
                pl.when((m == k) & (g < 3))(functools.partial(start_chunk, g + 1, k))
            pl.when(c == 9)(lambda: _start([wo_copy(k) for k in range(4)]))
            wait_chunk(g2, m2)
            _interleave(_tasks(functools.partial(operands, g2, m2), range(4), range(HD // 16)),
                        _tasks(functools.partial(first, g, m), range(4), range(M1_CUT)))
            for pair in range(4):
                project(g, m, pair)

        @pl.loop(0, 2)
        def _(k):
            wo_copy(k).wait()
            _overlap(_tasks(lambda j, i: first(3, 2, 2 * k + j, i), range(2), range(M1_CUT)),
                     wo_tasks(k), 2)

        scores, outs, tot = {}, {}, {}
        none = jnp.zeros((3 * HS, DH), f32)

        def step0(t):
            if t < NP:
                scores[t] = [_scores(qkv0[0, t, n], qkv0[1, t, n]) for n in range(2)]
            if 0 <= t - 2 < NP:
                outs[t - 2] = [_attend(scores[t - 2][n], qkv0[2, t - 2, n]) for n in range(2)]
            if 0 <= t - 4 < NP:
                for p, v in wo_pass(0, t - 4, outs[t - 4], none, 2).items():
                    r = _dot(v, wo_tile(p, t - 4))
                    tot[p] = tot[p] + r if p in tot else r
                return r
            project(3, 2, t)
            return qkv0[0, t, 0]

        for k, slots in ((2, range(12)), (3, range(12, 16))):
            wo_copy(k).wait()
            _overlap(_tasks(step0, slots), wo_tasks(k), 1)
        _interleave(_tasks(step0, range(16, 20)))
        return wo_finish(0, 0, tot)

    def step(wt, qcar, s, phase, cur, nxt, first, mem, o1_slot, fillers, chores):
        gw, gp = (phase + 1) % 3, (phase + 2) % 3
        ahead, now = GROUPS[gw], GROUPS[gp]
        lhs = {}
        for p in ahead + now:
            x0, x1 = _lhs(p, cur.__getitem__), _lhs(p, nxt.__getitem__)
            riders = (x0[8:], x1) if p in ahead else (x1[:8], x0)
            lhs[p] = _rows(_row_lhs(p, *mem), *riders).astype(bf16)
        heads, scores, outs, tot = {}, {}, {}, {}

        def qkv(m, a):
            r = {p: _dot(lhs[p], _get(wt, NP * m + a, p - 1)) for p in lhs}
            _release(r[now[1]], _share(chores, len(heads), 3 * NP - CH0))
            old = qcar[m, a]
            prod = {0: pltpu.bitcast(first(NP * m + a), f32)}
            for k in range(2):
                prod[GROUPS[phase][k]] = old[HS * k:HS * k + HS]
                prod[ahead[k]] = _rows(old[SEG + 8 * k:SEG + 8 * k + 8],
                                       r[ahead[k]][8:16])
                prod[now[k]] = r[now[k]][HS:]
            qcar[m, a] = _rows(*[r[p][HS:] for p in ahead], *[r[p][8:16] for p in now])
            c_mem = _row_res({g: r[GROUPS[g][0]][:MEM] + r[GROUPS[g][1]][:MEM]
                              for g in (gw, gp)})
            heads[m, a] = heads_of(c_mem, prod)

        for t in range(NP + LAG_WO):
            a = t - LAG_QK
            if 0 <= a < NP:
                scores[a] = [_scores(heads[0, a][n], heads[1, a][n]) for n in range(2)]
            a = t - LAG_PV
            if 0 <= a < NP:
                outs[a] = [_attend(scores[a][n], heads[2, a][n]) for n in range(2)]
            if t < NP:
                for m in range(3):
                    qkv(m, t)
            if t == FILL_AT:
                fillers[0]()
            a = t - LAG_WO
            if 0 <= a < NP:
                for p, v in wo_pass(phase, a, outs[a], ocar[a], o1_slot).items():
                    r = _dot(v, wo_tile(p, a))
                    tot[p] = tot[p] + r if p in tot else r
        fillers[1]()
        return wo_finish(phase, s, tot)

    def recurrence(wt, qcar, mem, raw, fin):
        _start(b_copies(raw))
        spare = 128 * (NC + 4)
        raw[pl.ds(0, 16), pl.ds(spare, 8), :] = jnp.zeros((16, 8, DH), u32)

        def chores(i):
            def convert(dst, base, per, groups):
                tasks = []
                for k in range(per):
                    r = pl.multiple_of(8 * jnp.clip(per * (i - 2) + k, 0, groups - 1), 8)
                    r0 = pl.multiple_of(jnp.where(i > 1, base + r, spare), 8)
                    tasks += _tasks(functools.partial(
                        b_operands, lambda k, n, r0=r0: raw[4 * n + k, pl.ds(r0, 8), :],
                        dst, r), range(7))
                return _held(raw.at[16, pl.ds(0, 8)], tasks)
            rest = convert(w12, 128 * NC, 4, 64)
            norm = _abreast(
                [mixer_norm(jnp.maximum(3 * i - 5 + (k >> 1), 0) * SEG + (k & 1) * HS,
                            fin.at[rows_of(HS * k, HS)])
                 for k in range(6)], 6)
            in_h = hbuf.at[pl.ds(0, 8), pl.ds(0, DH)]
            norm = (_held(in_h, norm[:36])
                    + _held(fin.at[pl.ds(3 * SEG, 8), pl.ds(0, DH)], norm[36:]))

            def due():
                m1.bitcast(u32)[3 * NP + here, pl.ds(S // 2 - 8, 8), :] = pltpu.bitcast(
                    xg[here, pl.ds(0, 8), :], u32)
            last = _merge(convert(m1, 0, 6, 16 * NC), norm[36:] + [(norm[-1][0], due)])
            return _merge(rest[:14], norm[:12]), _merge(rest[14:], norm[12:36]), last

        def steps(i, mem):
            pl.when(i == 2)(lambda: _wait(b_copies(raw)))
            src = 3 * (i & 1)
            acc = []

            def filler(n):
                if CUTS[n] < CUTS[n + 1]:
                    acc.append(wo_m1(src, range(CUTS[n], CUTS[n + 1])))
                    if CUTS[n + 1] == NP:
                        add_m1(3 * i - 2, functools.reduce(lambda u, v: u + v, acc))

            todo = chores(i)
            filler(0)
            wo_late(3 * i)
            nxt = seg_quads(3 * i + 1)
            for k in range(3):
                fillers = _tasks(filler, (2 * k + 1, 2 * k + 2))
                rows = pl.ds(pl.multiple_of((3 * i + 1 + k) * HS, HS), HS)
                first = lambda j: m1.bitcast(u32)[j, rows, :]
                if k == 2:
                    early = {j: first(j) for j in range(3 * NP) if j % NP < DUE}
                    first = lambda j, late=first: early[j] if j in early else late(j)
                cur, nxt = nxt, seg_quads(jnp.minimum(3 * i + 2 + k, NSEG - 1))
                mem = step(wt, qcar, 3 * i + 1 + k, (1 + k) % 3, cur, nxt, first, mem,
                           3 - src + k, fillers, todo[k])
            return mem

        lax.fori_loop(0, NSEG // 3, steps, mem)

    def block_a(wt, qcar):
        mem = pl.run_scoped(
            functools.partial(prologue, wt, qcar),
            pltpu.VMEM((12 * D, DH), u32),
            pltpu.VMEM((H * DH // 2 + 8, D), u32),
            pltpu.VMEM((4, S // 2, DH), bf16),
            pltpu.VMEM((6, 4, SEG, DH), bf16),
            pltpu.VMEM((3, NP, 2, L, DH), f32),
            pltpu.VMEM((MEM, D), bf16))

        pl.run_scoped(functools.partial(recurrence, wt, qcar, mem),
                      pltpu.VMEM((17, 128 * (NC + 4) + 8, DH), u32),
                      pltpu.VMEM((3 * SEG + 8, D), f32))

    pl.run_scoped(block_a, pltpu.VMEM((3 * NP + 3, 6, HD, DH), bf16),
                  pltpu.VMEM((3, NP, 3 * HS, DH), f32))

    def block_b(w4t, x1b, yn, ya, *pu):
        in_h = hbuf.at[pl.ds(0, 8), pl.ds(0, DH)]
        in_y = yn.at[pl.ds(RB, 8), pl.ds(0, DH)]
        pu = [pu[c % 3] for c in range(NC)]
        def wo_last():
            phase = NSEG % 3
            tot = {}
            wo_late(NSEG - 1)

            def task(a0, p, r0=0, n=0):
                pairs = range(a0, a0 + 2)
                if p == 0:
                    r = wo_m1(3 * (NSEG // 3 & 1), pairs)
                else:
                    lhs = _cols(*[ocar[a, pl.ds(r0, n), :] for a in pairs])
                    r = _dot(lhs.astype(bf16), _rows(*[wo_tile(p, a) for a in pairs]))
                tot[p] = tot[p] + r if a0 else r
                if a0 == NP - 2 and p == 0:
                    add_m1(NSEG - 3, tot[p])
                elif a0 == NP - 2:
                    add_h(NSEG - 1, [(p, 1, tot[p][-8:])] + [(p, 0, tot[p][:8])] * (n > 8))
                return r

            todo = [(0,)] + [t for k in range(2) for t in (
                (GROUPS[(phase + 2) % 3][k], HS * k, HS),
                (GROUPS[(phase + 1) % 3][k], SEG + 8 * k, 8))]
            return [functools.partial(task, a0, *t) for t in todo for a0 in range(0, NP, 2)]

        def a_operands(load, dst):
            def task(g, p1):
                r0, c = 16 * (g >> 1), g & 1
                for p0, v in enumerate(_twice(
                        _lhs, lambda i, k: load(i * R + r0, 2 * k + c), p1)):
                    dst[7 * p1 + p0, c, pl.ds(r0, 16), :] = v.astype(bf16)
            return _tasks(task, range(R // 8), range(7))

        def products(src, w, r0, dst):
            m = {}

            def task(p1, p0):
                p = 7 * p1 + p0
                m[p0] = _dot(_cols(*[_get(src, p + here, k) for k in range(2)]),
                             _get(w, p, rows=(r0, C4)))
                if p0 >= 3:
                    j = (2, 1, 3, 0)[p0 - 3]
                    dst[p1, j] = _res(j, m.__getitem__)
                return m[p0]
            return _tasks(task, range(7), range(7))

        def mlp_in(b):
            def residual(r0, y):
                x1 = y + x1b[rows_of(b * RB + r0, 16), :]
                yn[pl.ds(r0, 16), :] = x1
                put(rows_of(b * RB + r0, 16), hbuf[rows_of(PAD + b * RB + r0, 16), :] + x1)

            def store(r0, y):
                yn[pl.ds(r0, 16), :] = y
                return y

            return _held(in_h, _abreast([
                _ln_tasks(lambda r0=r0: hbuf[rows_of(PAD + b * RB + r0, 16), :],
                          functools.partial(residual, r0)) for r0 in range(0, RB, 16)], RB // 16)
            ) + _held(in_y, _abreast([
                _ln_tasks(lambda r0=r0: yn[rows_of(r0, 16), :],
                          functools.partial(store, r0)) for r0 in range(0, RB, 16)], RB // 16)
                + a_operands(
                lambda r0, c: yn[rows_of(r0, 16), pl.ds(DH * c, DH)], ya))

        def ups(c):
            return products(ya, m1, C4 * c, pu[c])

        def mixer(raw, *bufs):
            sa, sp = bufs[:2], (bufs[2:4], bufs[4:])
            in_g = xg.at[0, pl.ds(S + 2 * HALO, 8)]
            w4_copies = [pltpu.make_async_copy(
                w4_hbm.bitcast(u32).at[pl.ds(c, n)], raw.at[pl.ds(c, n)], sems.at[SEM_B + s])
                for c, n, s in ((0, 2, 1), (2, NC - 2, 2))]
            _start(w4_copies)

            def pre(n, w, b):
                shift = lambda c: w * (-1, 1, -2, 2)[c >> 1]
                return _held(in_g, a_operands(lambda r0, c: xg[c + here, pl.ds(
                    HALO + b * RB + r0 + shift(c), 16), :], sa[n & 1]))

            def post(n, w, b):
                def task(g, j):
                    c, g = divmod(g, R // 8)
                    m = [sp[n & 1][c][p1 + here, j, pl.ds(8 * g, 8), :]
                         for p1 in range(7)]
                    for q in range(4):
                        i, k = _pos(q, j)
                        r0 = _mult(b * RB + i * R + 8 * g, 8)
                        v = _res(q, m.__getitem__)
                        if w == 0:
                            xg[2 * k + c, pl.ds(HALO + r0, 8), :] = _gelu2(v)
                        else:
                            x1b[pl.ds(r0, 8), pl.ds(DH * (2 * k + c), DH)] = 0.5 * v
                return [t for c in range(2) for t in _held(
                    sp[n & 1][c].at[7, 0, pl.ds(0, 8)],
                    _tasks(task, range(R // 8 * c, R // 8 * (c + 1)), range(4)))]

            def unit(n, w, *side):
                dots = [t for c in range(2) for t in products(
                    sa[n & 1], w12, C4 * (2 * w + c), sp[n & 1][c])]
                _overlap(dots, _merge(*side), MX_LAG)

            def w4_work(k, n, half=0):
                def task(i, p1):
                    g, c = half + (i >> 1), i & 1
                    r0 = _mult(8 * (g & 7), 8)
                    b_operands(lambda q, j: raw[(g >> 3) + here, q, pl.ds(r0, 8),
                                                pl.ds(DH * (2 * j + c), DH)],
                               w4t, _mult(DH * (g >> 3) + 64 * c + r0, 8), p1)
                return _held(raw.at[NC, 0, pl.ds(0, 8), pl.ds(0, DH)],
                             _tasks(task, range(k, k + n), range(7)))

            norms = lambda s: _held(in_h, _abreast(
                [mixer_norm(s * SEG + k * HS) for k in range(6)], 3))
            _overlap(wo_last(), _merge(pre(0, 0, 0), norms(NSEG - 6)), MX_LAG)
            unit(0, 0, pre(1, 0, 1), norms(NSEG - 3))
            _wait(w4_copies[:1])

            @pl.loop(0, 3)
            def _(i):
                pl.when(i == 2)(lambda: _wait(w4_copies[1:]))
                for n in range(2):
                    b = 2 * i + 1 + n
                    unit(n + 1, 0, pre(n, 0, b + 1), post(n, 0, b - 1),
                         w4_work(G1 * n, G1, G1 * i))

            unit(1, 0, pre(0, 1, 0), post(0, 0, 6), w4_work(6 * G1, G1))
            unit(0, 1, pre(1, 1, 1), post(1, 0, 7), w4_work(7 * G1, G1))

            @pl.loop(0, 2)
            def _(i):
                for n in range(2):
                    b = 2 * i + 1 + n
                    unit(n + 1, 1, pre(n, 1, b + 1), post(n, 1, b - 1),
                         w4_work(8 * G1 + G2 * n, G2, G2 * i))

            done = 8 * G1 + 4 * G2
            rest = w4_work(done, 16 * NC - done)
            ahead = mlp_in(0)
            for b in range(5, NB):
                unit(b, 1, pre(b + 1, 1, b + 1) if b + 1 < NB else _share(rest, 2, 4),
                     post(b - 1, 1, b - 1), _share(ahead, b - 5, 3),
                     _share(rest, (0, 1, 3)[b - 5], 4))
            for _, task in post(1, 1, NB - 1):
                task()

        def mlp(ta0, ta1, pd, ob):
            ta = [ta0.at[c] for c in range(NC - 1)] + [ta1]

            def mid(c, g, j):
                r = pl.ds(8 * g, 8)
                m = [pu[c][p1 + here, j, r, :] for p1 in range(7)]
                y = [_gelu2(_res(q, m.__getitem__)) for q in range(4)]
                for p1 in range(7):
                    v = _lhs(p1, y.__getitem__)
                    ta[c][p1, j, r, :] = v
                return v

            def down(b, m, p, c):
                p1, p0 = divmod(p, 7)
                lhs = _lhs(p0, lambda j: ta[c][p1 + here, j]).astype(bf16)
                tot = _dot(lhs, jnp.concatenate(
                    [_get(w4t, p, rows=(C4 * c + 128 * k, 128)) for k in range(2)],
                    axis=1))
                m[p] = m[p] + tot if c else tot
                if c == NC - 1 and p0 >= 3:
                    j = (2, 1, 3, 0)[p0 - 3]
                    v = _res(j, lambda k: m[7 * p1 + k])
                    if p1 < 6:
                        pd[p1, j] = v
                    if p1 >= 3:
                        q = (2, 1, 3, 0)[p1 - 3]
                        i, n = _pos(q, j)
                        r0, cols = _mult(b * RB + i * R, R), pl.ds(n * C4, C4)
                        v = _res(q, lambda k: v if k == p1 else pd[k + here, j])
                        ob[pl.ds(r0, R), cols] = (
                            _cols(*[xg[2 * n + k, pl.ds(r0, R), :] for k in range(2)]) + 0.5 * v).astype(bf16)
                return tot

            def out_copy(b):
                rows = pl.ds(_mult(b * RB, RB), RB)
                return pltpu.make_async_copy(ob.at[rows], out_hbm.at[rows],
                                             sems.at[SEM_OUT + b])

            @pl.loop(0, NB)
            def _(b):
                mids = lambda c: _held(pu[c].at[7, 0, pl.ds(0, 8)], _tasks(
                    functools.partial(mid, c), range(R // 8), range(4)))
                task = functools.partial(down, b, {})
                early = _tasks(task, range(EARLY), range(NC - 1))
                ahead = mlp_in(jnp.minimum(b + 1, NB - 1))
                _overlap(ups(0), ahead[:A0], 0)
                for c in range(NC):
                    _overlap(ups(c + 1) if c + 1 < NC else early,
                             _merge(mids(c), _share(ahead[A0:AH], c, NC - 1)), UP_LAG)

                _overlap(_tasks(task, range(EARLY), [NC - 1])
                         + _tasks(task, range(EARLY, 49), range(NC)),
                         ahead[AH:], DN_LAG)
                out_copy(b).start()

            for b in range(NB):
                out_copy(b).wait()

        pl.run_scoped(mixer, pltpu.VMEM((NC + 1, 4, 64, D), u32),
                      *[pltpu.VMEM((49, 2, R, DH), bf16)] * 2,
                      *[pltpu.VMEM((8, 4, R, DH), f32)] * 4)
        pl.run_scoped(mlp, pltpu.VMEM((NC - 1, 7, 4, R, DH), f32),
                      pltpu.VMEM((7, 4, R, DH), f32),
                      pltpu.VMEM((6, 4, R, C4), f32), pltpu.VMEM((S, D), bf16))

    pl.run_scoped(
        block_b,
        pltpu.VMEM((49, C4 * NC, DH), bf16),
        pltpu.VMEM((S, D), f32),
        pltpu.VMEM((RB + 8, D), f32),
        pltpu.VMEM((49, 2, R, DH), bf16),
        *[pltpu.VMEM((8, 4, R, 128), f32)] * 3)


@jax.jit
def pallas_sequential_preLN__memory_aug_recurrent_mem_tr__mixer_s_mlp__prompt_kernel(
    A_x: jax.Array,
    A_mem0: jax.Array,
    A_Wq: jax.Array,
    A_Wk: jax.Array,
    A_Wv: jax.Array,
    A_Wo: jax.Array,
    A_seg_len: jax.Array,
    B_x: jax.Array,
    B_w1: jax.Array,
    B_w2: jax.Array,
    B_w3: jax.Array,
    B_w4: jax.Array,
):
    del A_seg_len, B_x
    hbm = pl.BlockSpec(memory_space=pl.ANY)
    scratch = [
        pltpu.VMEM((PAD + S, D), f32),
        pltpu.VMEM((8, S + 3 * HALO, DH), f32),
        pltpu.VMEM((7, NP, 4, DH, DH), bf16),
        pltpu.VMEM((6, NP, HS, DH), bf16),
        pltpu.VMEM((7, 24, HD), f32),
        pltpu.VMEM((NP, 3 * HS, DH), f32),
        pltpu.VMEM((49, S, DH), bf16),
        pltpu.VMEM((49, D, DH), bf16),
        pltpu.SemaphoreType.DMA((NSEM,)),
    ]
    out = pl.pallas_call(
        _kernel,
        out_shape=jax.ShapeDtypeStruct((S, D), A_x.dtype),
        in_specs=[hbm] * 10,
        out_specs=hbm,
        scratch_shapes=scratch,
        compiler_params=pltpu.CompilerParams(vmem_limit_bytes=127 * 1024 * 1024),
    )(A_x.reshape(S, D), A_mem0.reshape(MEM, D),
      A_Wq.reshape(D // 2, 2 * H, DH), A_Wk.reshape(D // 2, 2 * H, DH),
      A_Wv.reshape(D // 2, 2 * H, DH),
      A_Wo.reshape(H * DH, D), B_w1.reshape(4, C4, D), B_w2.reshape(4, C4, D),
      B_w3.reshape(4, C4, F), B_w4.reshape(NC, 4, FC // 4, D))
    return out.reshape(A_x.shape)
```

```python
import functools

import jax
import jax.numpy as jnp
from jax import lax
import jax.experimental.pallas as pl
import jax.experimental.pallas.tpu as pltpu

S = 2048
D = 1024
H = 32
DH = 128
MEM = 8
SEG = 32
F = 3584
NSEG = S // SEG
L = MEM + SEG
HS = SEG // 2
NP = H // 2
HD = D // 2
PAD = 8
C4 = D // 4
HALO = 8
R = 64
RB = 4 * R
NB = S // RB
FC = 512
NC = F // FC
EPS = 1e-5
NEG = -1000000000.0

LAG_QK = 2
LAG_PV = 4
LAG_WO = 6
FILL_AT = 19
CUTS = (0, 2, 4, 8, 10, 14, 16, 16)
CH0 = 20
DUE = 15
M1_CUT = 16
G1 = 8
G2 = 11
A0 = 32
AH = 80
EARLY = 14
MX_LAG = 5
UP_LAG = 10
DN_LAG = 20

GROUPS = ((1, 3), (2, 4), (5, 6))
TARGETS = (((0, 1), (3, 1)), ((2, 1), (3, -1)), ((1, 1), (3, 1)), ((0, 1), (2, 1)),
           ((0, -1), (1, 1)), ((3, 1),), ((0, 1),))

bf16 = jnp.bfloat16
f32 = jnp.float32
u32 = jnp.uint32

SEM_X, SEM_W, SEM_WO, SEM_B, SEM_OUT = 0, 4, 16, 20, 24
NSEM = SEM_OUT + NB


def _mult(i, n):
    return i if isinstance(i, int) else pl.multiple_of(i, n)


def _ln(x):
    m = jnp.mean(x, axis=-1, keepdims=True)
    d = x - m
    v = jnp.mean(d * d, axis=-1, keepdims=True)
    return d * lax.rsqrt(v + EPS)


def _gelu2(x):
    c = 0.7978845608028654
    return x + x * jnp.tanh(x * (c + (c * 0.044715) * (x * x)))


def _get(ref, *idx, rows=None):
    rows = slice(None) if rows is None else pl.ds(rows[0] // 2, rows[1] // 2)
    return _unpack(ref.bitcast(u32)[idx + (rows, slice(None))])


def _cols(*xs):
    return jnp.concatenate(xs, axis=1)


def _unpack(x):
    return pltpu.bitcast(x, bf16)


def _dot(a, b):
    return jnp.dot(a, b, preferred_element_type=f32)


def _rows(*xs):
    return jnp.concatenate(xs, axis=0)


def _lhs(p, a):
    return (lambda: a(0) + a(3), lambda: a(2) + a(3), lambda: a(0), lambda: a(3),
            lambda: a(0) + a(1), lambda: a(2) - a(0), lambda: a(1) - a(3))[p]()


def _rhs(p, b):
    return (lambda: b(0) + b(3), lambda: b(0), lambda: b(1) - b(3), lambda: b(2) - b(0),
            lambda: b(3), lambda: b(0) + b(1), lambda: b(2) + b(3))[p]()


def _res(q, m):
    return (lambda: m(0) + m(3) - m(4) + m(6), lambda: m(2) + m(4),
            lambda: m(1) + m(3), lambda: m(0) - m(1) + m(2) + m(5))[q]()


def _pos(q, j):
    return 2 * (q >> 1) + (j >> 1), 2 * (q & 1) + (j & 1)


def _twice(side, blk, p1):
    outer = [side(p1, lambda q: blk(*_pos(q, j))) for j in range(4)]
    return [side(p0, outer.__getitem__) for p0 in range(7)]


def _ln_tasks(load, store, twice=False, keep=None):
    st = {}

    def fold(x):
        return functools.reduce(
            lambda u, v: u + v, [x[:, c:c + DH] for c in range(0, D, DH)])

    def part():
        st["s"] = fold(load())

    def mean():
        st["m"] = jnp.sum(st["s"], axis=-1, keepdims=True) * (1.0 / D)

    def square():
        d = load() - st["m"]
        st["s"] = fold(d * d)
        if keep:
            keep[...] = d

    def var():
        st["v"] = jnp.sum(st["s"], axis=-1, keepdims=True) * (1.0 / D)

    def scale():
        st["r"] = lax.rsqrt(st["v"] + EPS)

    def again():
        st["r"] = st["r"] * lax.rsqrt(st["v"] * st["r"] * st["r"] + EPS)

    def apply():
        store((keep[...] if keep else load() - st["m"]) * st["r"])

    if twice:
        return [part, mean, square, var, scale, again, apply]
    return [lambda: (part(), mean()), lambda: (square(), var(), scale()), apply]


def _abreast(chains, n):
    return [t for i in range(0, len(chains), n) for ts in zip(*chains[i:i + n]) for t in ts]


def _row_lhs(p, a1, a2):
    return a1 + a2 if p in (1, 4) else a1 if p in (2, 5) else a2


def _row_res(t):
    if 0 not in t:
        return t[2] - t[1], t[1]
    if 1 not in t:
        return t[0], t[2] - t[0]
    return t[0], t[1]


def _merge(*lists):
    order = sorted(((i + 0.5) / len(l), n, i)
                   for n, l in enumerate(lists) for i in range(len(l)))
    return [lists[n][i] for _, n, i in order]


def _interleave(*lists):
    for task in _merge(*lists):
        task()


def _held(spare, tasks):
    return [(spare, task) for task in tasks]


def _overlap(dots, side, lag):
    for i, dot in enumerate(dots):
        _release(dot(), _share(side, i, len(dots) - lag))


def _release(result, mine):
    for spare in {id(spare): spare for spare, _ in mine}.values():
        spare[...] = pltpu.bitcast(result[-8:, -DH:], spare.dtype)
    for _, task in mine:
        task()


def _share(tasks, k, n):
    return tasks[len(tasks) * k // n:len(tasks) * (k + 1) // n] if k >= 0 else []


def _tasks(fn, *ranges):
    if len(ranges) == 2:
        return [functools.partial(fn, i, j) for i in ranges[0] for j in ranges[1]]
    return [functools.partial(fn, i) for i in ranges[0]]


def _start(copies):
    for c in copies:
        c.start()


def _wait(copies):
    for c in copies:
        c.wait()


def _scores(q, k):
    return lax.dot_general(q, k, (((1,), (1,)), ((), ())), preferred_element_type=f32)


def _attend(sc, v):
    ri = lax.broadcasted_iota(jnp.int32, (L, L), 0)
    ci = lax.broadcasted_iota(jnp.int32, (L, L), 1)
    sc = jnp.where((ri < MEM) | (ri >= ci), sc, NEG * DH ** 0.5)
    mx = jnp.max(sc, axis=1, keepdims=True)
    e = jnp.exp2((sc - mx) * (DH ** -0.5 * 1.4426950408889634))
    den = jnp.sum(e, axis=1, keepdims=True)
    inv = pl.reciprocal(den, approx=True)
    inv = inv * (2.0 - den * inv)
    return _dot(e, v) * inv


def _kernel(x_hbm, mem0_hbm, wq_hbm, wk_hbm, wv_hbm, wo_hbm, w1_hbm, w2_hbm,
            w3_hbm, w4_hbm, out_hbm, hbuf, xg, wo_t, o1, late, ocar, m1, w12, sems):
    w_hbm = (wq_hbm, wk_hbm, wv_hbm)
    here = lax.fori_loop(0, 2, lambda i, z: z + (i >> 1), jnp.int32(0))

    def b_copies(raw):
        tile = lambda w, i: w.bitcast(u32).at[:, :, pl.ds(128 * i, 128)]
        for n in range(4):
            slabs = pl.ds(4 * n, 4)
            for i, w in enumerate((w1_hbm, w2_hbm)):
                for c in range(2):
                    yield pltpu.make_async_copy(
                        tile(w, 2 * n + c),
                        raw.at[slabs, pl.ds(128 * (NC + 2 * i + c), 128)],
                        sems.at[SEM_B])
            for c in range(NC):
                yield pltpu.make_async_copy(
                    tile(w3_hbm, 4 * c + n), raw.at[slabs, pl.ds(128 * c, 128)],
                    sems.at[SEM_B])

    def b_operands(raw, dst, r1, p1):
        for p0, v in enumerate(_twice(_rhs, lambda k, n: _unpack(raw(k, n)).astype(f32), p1)):
            if p1 in (1, 4) and p0 in (1, 4):
                k = 2 * (p1 // 4) + p0 // 4
                dst.bitcast(u32)[7 * p1 + p0, pl.ds(r1, 8), :] = raw(k, k)
            else:
                dst[7 * p1 + p0, pl.ds(_mult(2 * r1, 16), 16), :] = v.astype(bf16)

    def rows_of(r0, n):
        return pl.ds(pl.multiple_of(r0 + here, 8), n)

    def put(rows, x):
        for c in range(8):
            xg[c, rows, :] = x[:, DH * c:DH * (c + 1)]

    def wo_tile(p, a):
        return _cols(*[_get(wo_t, p, a, c) for c in range(4)])

    def seg_quads(s):
        r0 = HALO + s * SEG
        return [jnp.concatenate(
            [xg[4 * (q & 1) + c, pl.ds(_mult(r0 + (q >> 1) * HS, 8), HS), :]
             for c in range(4)], axis=1) for q in range(4)]

    def heads_of(c_mem, m):
        return [_rows(c_mem[n], _res(n, m.__getitem__), _res(2 + n, m.__getitem__))
                for n in range(2)]

    def wo_pass(phase, a, o, prev, o1_slot):
        whole, part = GROUPS[(phase + 1) % 3], GROUPS[(phase + 2) % 3]
        quad = lambda q: o[q & 1][MEM + (q >> 1) * HS:MEM + (q >> 1) * HS + HS]
        x = [_lhs(p, quad) for p in range(7)]
        o1[o1_slot, a] = x[0].astype(bf16)
        ocar[a] = _rows(*[x[p] for p in GROUPS[phase]], *[x[p][8:] for p in part])
        res = {}
        for k in range(2):
            for p, riders in ((whole[k], (prev[SEG + 8 * k:SEG + 8 * k + 8], x[whole[k]])),
                              (part[k], (x[part[k]][:8], prev[HS * k:HS * k + HS]))):
                lhs = _rows(_row_lhs(p, o[0][:MEM], o[1][:MEM]), *riders)
                res[p] = lhs.astype(bf16)
        return res

    def add_h(s, terms):
        for q in range(4):
            for z in range(2):
                mine = [(sign, v) for p, zz, v in terms if zz == z
                        for qq, sign in TARGETS[p] if qq == q]
                if mine:
                    at = (pl.ds(_mult(PAD + s * SEG + (q >> 1) * HS + 8 * z, 8), 8),
                          pl.ds((q & 1) * HD, HD))
                    acc = hbuf[at]
                    for sign, v in mine:
                        acc = acc + v if sign > 0 else acc - v
                    hbuf[at] = acc

    def wo_tokens(phase, s, rows):
        whole, part = GROUPS[(phase + 1) % 3], GROUPS[(phase + 2) % 3]
        for k, one, two in ((jnp.maximum(s - 1, 0), whole, part), (s, part, whole)):
            add_h(k, [(p, int(one is whole), rows(p, 0)) for p in one]
                  + [(p, z, rows(p, 8 + 8 * z)) for p in two for z in range(2)])

    def wo_finish(phase, s, tot):
        if phase:
            wo_tokens(phase, s, lambda p, r0: tot[p][MEM + r0:MEM + r0 + 8])
        else:
            for p in tot:
                late[p] = tot[p][MEM:]
        return _row_res({g: tot[GROUPS[g][0]][:MEM] + tot[GROUPS[g][1]][:MEM]
                         for g in range(3) if g != phase})

    def wo_late(s):
        wo_tokens(0, s, lambda p, r0: late[p + here, pl.ds(r0, 8), :])

    def wo_m1(slot, pairs):
        lhs = jnp.concatenate(
            [_rows(*[_get(o1, slot + k, a) for k in range(3)]) for a in pairs], axis=1)
        return _dot(lhs, _rows(*[wo_tile(0, a) for a in pairs]))

    def add_m1(s, r):
        for k in range(3):
            add_h(jnp.maximum(s + k, 0),
                  [(0, z, r[HS * k + 8 * z:HS * k + 8 * z + 8]) for z in range(2)])

    def mixer_norm(r0, keep=None):
        return _ln_tasks(lambda: hbuf[rows_of(PAD + r0, HS), :],
                         functools.partial(put, rows_of(HALO + r0, HS)), True, keep)

    def prologue(wt, qcar, stg, words, lhs1, lhs0, qkv0, mem0):
        def row_copy(src, i, n, sem):
            rows = pl.ds(_mult(i * n, n), n)
            return pltpu.make_async_copy(src.bitcast(u32).at[rows], words.at[rows],
                                         sems.at[sem + i])

        x_copy = lambda i: row_copy(x_hbm, i, S // 8, SEM_X)
        wo_copy = lambda g: row_copy(wo_hbm, g, 512, SEM_WO)

        def start_chunk(g, m):
            src = w_hbm[m].bitcast(u32)
            dst = stg.reshape(3 * (HD + 1), 8, DH)
            for par in range(2):
                pltpu.make_async_copy(
                    src.at[:, pl.ds(_mult(16 * par + 4 * g, 4), 4), :],
                    dst.at[pl.ds((HD + 1) * m, HD), pl.ds(4 * par, 4), :],
                    sems.at[SEM_W + 3 * g + m]).start()

        def wait_chunk(g, m):
            part = stg.at[pl.ds(_mult((4 * D + 8) * m, 8), 4 * D)]
            pltpu.make_async_copy(part, part, sems.at[SEM_W + 3 * g + m]).wait()

        def operands(g, m, pair, i):
            w = [stg[pl.ds(4 * ((D + 2) * m + HD * k + 16 * i) + pair, 16, stride=4), :]
                 for k in range(2)]
            quad = [pltpu.bitcast(w[q >> 1] & jnp.uint32(0xFFFF0000) if q & 1
                                  else w[q >> 1] << 16, f32) for q in range(4)]
            wt[3 * NP + m, pair, pl.ds(_mult(16 * i, 16), 16), :] = _rhs(0, quad.__getitem__).astype(bf16)
            for p in range(1, 7):
                wt[NP * m + 4 * g + pair, p - 1, pl.ds(_mult(16 * i, 16), 16), :] = _rhs(
                    p, quad.__getitem__).astype(bf16)

        def wo_operands(g, pair, i):
            c, r0 = i & 3, 8 * (i >> 2)
            w = [words[rows_of(DH * (4 * g + pair) + DH // 2 * (q >> 1) + r0, 8),
                       pl.ds(HD * (q & 1) + DH * c, DH)] for q in range(4)]
            quad = [_unpack(v).astype(f32) for v in w]
            for p in range(7):
                v = _rhs(p, quad.__getitem__).astype(bf16)
                wo_t[p, 4 * g + pair, c, pl.ds(2 * r0, 16), :] = v

        for i in range(4):
            if i == 3:
                start_chunk(0, 0)
            x_copy(i).start()
        mem_copy = pltpu.make_async_copy(mem0_hbm, mem0, sems.at[SEM_B + 3])
        mem_copy.start()
        start_chunk(0, 1)
        start_chunk(0, 2)
        for r0 in (0, HALO + S):
            put(pl.ds(r0, HALO), jnp.zeros((HALO, D), f32))
        for k in range(2):
            o1[k] = jnp.zeros((NP, HS, DH), bf16)
        @pl.loop(0, 4)
        def _(i):
            x_copy(i).wait()

            @pl.loop(0, 4, unroll=4)
            def _(k):
                r0 = pl.multiple_of(i * (S // 4) + k * 128, 128)
                xv = _unpack(words[pl.ds(pl.multiple_of(r0 // 2, 64), 64), :]).astype(f32)
                hbuf[pl.ds(PAD + r0, 128), :] = xv
                xn = _ln(xv)
                put(pl.ds(HALO + r0, 128), xn)
                v = _rows(*[xn[z:z + HS, :HD] + xn[z + HS:z + SEG, HD:]
                            for z in range(0, 128, SEG)])
                for c in range(4):
                    lhs1[c, pl.ds(pl.multiple_of(r0 // 2, 64), 64), :] = (
                        v[:, DH * c:DH * (c + 1)].astype(bf16))

        wait_chunk(0, 0)

        @pl.loop(0, HD // 16, step=4)
        def _(i):
            for k in range(4):
                for pair in range(4):
                    operands(0, 0, pair, i + k)

        mem_copy.wait()
        mem = mem0[...].astype(f32)
        cur, nxt = seg_quads(0), seg_quads(1)
        for p in range(1, 7):
            x0, x1 = _lhs(p, cur.__getitem__), _lhs(p, nxt.__getitem__)
            v = (_rows(x0, x1) if p in GROUPS[1]
                 else _rows(_row_lhs(p, mem[:, :HD], mem[:, HD:]), x1[:8], x0))
            for c in range(4):
                lhs0[p - 1, c] = v[:, DH * c:DH * (c + 1)].astype(bf16)

        def first(g, m, pair, i):
            n = S // 2 // M1_CUT
            lhs = _cols(*[_get(lhs1, c, rows=(n * i, n)) for c in range(4)])
            r = pltpu.bitcast(_dot(lhs, _get(wt, 3 * NP + m + here, pair)), u32)
            m1.bitcast(u32)[NP * m + 4 * g + pair, pl.ds(n * i, n), :] = r
            return r

        def project(g, m, pair):
            a = 4 * g + pair
            r = {p: _dot(_cols(*[_get(lhs0, p - 1, c) for c in range(4)]),
                         _get(wt, NP * m + a, p - 1))
                 for p in range(1, 7)}
            prod = {p: r[p][:HS] if p in GROUPS[1] else r[p][HS:] for p in r}
            prod[0] = pltpu.bitcast(m1.bitcast(u32)[NP * m + a, pl.ds(0, HS), :], f32)
            qcar[m, a] = _rows(*[r[p][HS:] for p in GROUPS[1]],
                               *[r[p][8:16] for p in GROUPS[2]])
            c_mem = _row_res({k: r[GROUPS[k][0]][:MEM] + r[GROUPS[k][1]][:MEM]
                              for k in (0, 2)})
            for n, v in enumerate(heads_of(c_mem, prod)):
                qkv0[m, a, n] = v

        def wo_tasks(g):
            return _held(words.at[pl.ds(H * DH // 2, 8), pl.ds(0, DH)],
                         _tasks(functools.partial(wo_operands, g), range(4), range(32)))

        @pl.loop(0, 11)
        def _(c):
            g, g2 = lax.div(c, 3), lax.div(c + 1, 3)
            m, m2 = c - 3 * g, c + 1 - 3 * g2
            for k in range(3):
                pl.when((m == k) & (g < 3))(functools.partial(start_chunk, g + 1, k))
            pl.when(c == 9)(lambda: _start([wo_copy(k) for k in range(4)]))
            wait_chunk(g2, m2)
            _interleave(_tasks(functools.partial(operands, g2, m2), range(4), range(HD // 16)),
                        _tasks(functools.partial(first, g, m), range(4), range(M1_CUT)))
            for pair in range(4):
                project(g, m, pair)

        @pl.loop(0, 2)
        def _(k):
            wo_copy(k).wait()
            _overlap(_tasks(lambda j, i: first(3, 2, 2 * k + j, i), range(2), range(M1_CUT)),
                     wo_tasks(k), 2)

        scores, outs, tot = {}, {}, {}
        none = jnp.zeros((3 * HS, DH), f32)

        def step0(t):
            if t < NP:
                scores[t] = [_scores(qkv0[0, t, n], qkv0[1, t, n]) for n in range(2)]
            if 0 <= t - 2 < NP:
                outs[t - 2] = [_attend(scores[t - 2][n], qkv0[2, t - 2, n]) for n in range(2)]
            if 0 <= t - 4 < NP:
                for p, v in wo_pass(0, t - 4, outs[t - 4], none, 2).items():
                    r = _dot(v, wo_tile(p, t - 4))
                    tot[p] = tot[p] + r if p in tot else r
                return r
            project(3, 2, t)
            return qkv0[0, t, 0]

        for k, slots in ((2, range(12)), (3, range(12, 16))):
            wo_copy(k).wait()
            _overlap(_tasks(step0, slots), wo_tasks(k), 1)
        _interleave(_tasks(step0, range(16, 20)))
        return wo_finish(0, 0, tot)

    def step(wt, qcar, s, phase, cur, nxt, first, mem, o1_slot, fillers, chores):
        gw, gp = (phase + 1) % 3, (phase + 2) % 3
        ahead, now = GROUPS[gw], GROUPS[gp]
        lhs = {}
        for p in ahead + now:
            x0, x1 = _lhs(p, cur.__getitem__), _lhs(p, nxt.__getitem__)
            riders = (x0[8:], x1) if p in ahead else (x1[:8], x0)
            lhs[p] = _rows(_row_lhs(p, *mem), *riders).astype(bf16)
        heads, scores, outs, tot = {}, {}, {}, {}

        def qkv(m, a):
            r = {p: _dot(lhs[p], _get(wt, NP * m + a, p - 1)) for p in lhs}
            _release(r[now[1]], _share(chores, len(heads), 3 * NP - CH0))
            old = qcar[m, a]
            prod = {0: pltpu.bitcast(first(NP * m + a), f32)}
            for k in range(2):
                prod[GROUPS[phase][k]] = old[HS * k:HS * k + HS]
                prod[ahead[k]] = _rows(old[SEG + 8 * k:SEG + 8 * k + 8],
                                       r[ahead[k]][8:16])
                prod[now[k]] = r[now[k]][HS:]
            qcar[m, a] = _rows(*[r[p][HS:] for p in ahead], *[r[p][8:16] for p in now])
            c_mem = _row_res({g: r[GROUPS[g][0]][:MEM] + r[GROUPS[g][1]][:MEM]
                              for g in (gw, gp)})
            heads[m, a] = heads_of(c_mem, prod)

        for t in range(NP + LAG_WO):
            a = t - LAG_QK
            if 0 <= a < NP:
                scores[a] = [_scores(heads[0, a][n], heads[1, a][n]) for n in range(2)]
            a = t - LAG_PV
            if 0 <= a < NP:
                outs[a] = [_attend(scores[a][n], heads[2, a][n]) for n in range(2)]
            if t < NP:
                for m in range(3):
                    qkv(m, t)
            if t == FILL_AT:
                fillers[0]()
            a = t - LAG_WO
            if 0 <= a < NP:
                for p, v in wo_pass(phase, a, outs[a], ocar[a], o1_slot).items():
                    r = _dot(v, wo_tile(p, a))
                    tot[p] = tot[p] + r if p in tot else r
        fillers[1]()
        return wo_finish(phase, s, tot)

    def recurrence(wt, qcar, mem, raw, fin):
        _start(b_copies(raw))
        spare = 128 * (NC + 4)
        raw[pl.ds(0, 16), pl.ds(spare, 8), :] = jnp.zeros((16, 8, DH), u32)

        def chores(i):
            def convert(dst, base, per, groups):
                tasks = []
                for k in range(per):
                    r = pl.multiple_of(8 * jnp.clip(per * (i - 2) + k, 0, groups - 1), 8)
                    r0 = pl.multiple_of(jnp.where(i > 1, base + r, spare), 8)
                    tasks += _tasks(functools.partial(
                        b_operands, lambda k, n, r0=r0: raw[4 * n + k, pl.ds(r0, 8), :],
                        dst, r), range(7))
                return _held(raw.at[16, pl.ds(0, 8)], tasks)
            rest = convert(w12, 128 * NC, 4, 64)
            norm = _abreast(
                [mixer_norm(jnp.maximum(3 * i - 5 + (k >> 1), 0) * SEG + (k & 1) * HS,
                            fin.at[rows_of(HS * k, HS)])
                 for k in range(6)], 6)
            in_h = hbuf.at[pl.ds(0, 8), pl.ds(0, DH)]
            norm = (_held(in_h, norm[:36])
                    + _held(fin.at[pl.ds(3 * SEG, 8), pl.ds(0, DH)], norm[36:]))

            def due():
                m1.bitcast(u32)[3 * NP + here, pl.ds(S // 2 - 8, 8), :] = pltpu.bitcast(
                    xg[here, pl.ds(0, 8), :], u32)
            last = _merge(convert(m1, 0, 6, 16 * NC), norm[36:] + [(norm[-1][0], due)])
            return _merge(rest[:14], norm[:12]), _merge(rest[14:], norm[12:36]), last

        def steps(i, mem):
            pl.when(i == 2)(lambda: _wait(b_copies(raw)))
            src = 3 * (i & 1)
            acc = []

            def filler(n):
                if CUTS[n] < CUTS[n + 1]:
                    acc.append(wo_m1(src, range(CUTS[n], CUTS[n + 1])))
                    if CUTS[n + 1] == NP:
                        add_m1(3 * i - 2, functools.reduce(lambda u, v: u + v, acc))

            todo = chores(i)
            filler(0)
            wo_late(3 * i)
            nxt = seg_quads(3 * i + 1)
            for k in range(3):
                fillers = _tasks(filler, (2 * k + 1, 2 * k + 2))
                rows = pl.ds(pl.multiple_of((3 * i + 1 + k) * HS, HS), HS)
                first = lambda j: m1.bitcast(u32)[j, rows, :]
                if k == 2:
                    early = {j: first(j) for j in range(3 * NP) if j % NP < DUE}
                    first = lambda j, late=first: early[j] if j in early else late(j)
                cur, nxt = nxt, seg_quads(jnp.minimum(3 * i + 2 + k, NSEG - 1))
                mem = step(wt, qcar, 3 * i + 1 + k, (1 + k) % 3, cur, nxt, first, mem,
                           3 - src + k, fillers, todo[k])
            return mem

        lax.fori_loop(0, NSEG // 3, steps, mem)

    def block_a(wt, qcar):
        mem = pl.run_scoped(
            functools.partial(prologue, wt, qcar),
            pltpu.VMEM((12 * D + 24, DH), u32),
            pltpu.VMEM((H * DH // 2 + 8, D), u32),
            pltpu.VMEM((4, S // 2, DH), bf16),
            pltpu.VMEM((6, 4, SEG, DH), bf16),
            pltpu.VMEM((3, NP, 2, L, DH), f32),
            pltpu.VMEM((MEM, D), bf16))

        pl.run_scoped(functools.partial(recurrence, wt, qcar, mem),
                      pltpu.VMEM((17, 128 * (NC + 4) + 8, DH), u32),
                      pltpu.VMEM((3 * SEG + 8, D), f32))

    pl.run_scoped(block_a, pltpu.VMEM((3 * NP + 3, 6, HD, DH), bf16),
                  pltpu.VMEM((3, NP, 3 * HS, DH), f32))

    def block_b(w4t, x1b, yn, ya, *pu):
        in_h = hbuf.at[pl.ds(0, 8), pl.ds(0, DH)]
        in_y = yn.at[pl.ds(RB, 8), pl.ds(0, DH)]
        pu = [pu[c % 3] for c in range(NC)]
        def wo_last():
            phase = NSEG % 3
            tot = {}
            wo_late(NSEG - 1)

            def task(a0, p, r0=0, n=0):
                pairs = range(a0, a0 + 2)
                if p == 0:
                    r = wo_m1(3 * (NSEG // 3 & 1), pairs)
                else:
                    lhs = _cols(*[ocar[a, pl.ds(r0, n), :] for a in pairs])
                    r = _dot(lhs.astype(bf16), _rows(*[wo_tile(p, a) for a in pairs]))
                tot[p] = tot[p] + r if a0 else r
                if a0 == NP - 2 and p == 0:
                    add_m1(NSEG - 3, tot[p])
                elif a0 == NP - 2:
                    add_h(NSEG - 1, [(p, 1, tot[p][-8:])] + [(p, 0, tot[p][:8])] * (n > 8))
                return r

            todo = [(0,)] + [t for k in range(2) for t in (
                (GROUPS[(phase + 2) % 3][k], HS * k, HS),
                (GROUPS[(phase + 1) % 3][k], SEG + 8 * k, 8))]
            return [functools.partial(task, a0, *t) for t in todo for a0 in range(0, NP, 2)]

        def a_operands(load, dst):
            def task(g, p1):
                r0, c = 16 * (g >> 1), g & 1
                for p0, v in enumerate(_twice(
                        _lhs, lambda i, k: load(i * R + r0, 2 * k + c), p1)):
                    dst[7 * p1 + p0, c, pl.ds(r0, 16), :] = v.astype(bf16)
            return _tasks(task, range(R // 8), range(7))

        def products(src, w, r0, dst):
            m = {}

            def task(p1, p0):
                p = 7 * p1 + p0
                m[p0] = _dot(_cols(*[_get(src, p + here, k) for k in range(2)]),
                             _get(w, p, rows=(r0, C4)))
                if p0 >= 3:
                    j = (2, 1, 3, 0)[p0 - 3]
                    dst[p1, j] = _res(j, m.__getitem__)
                return m[p0]
            return _tasks(task, range(7), range(7))

        def mlp_in(b):
            def residual(r0, y):
                x1 = y + x1b[rows_of(b * RB + r0, 16), :]
                yn[pl.ds(r0, 16), :] = x1
                put(rows_of(b * RB + r0, 16), hbuf[rows_of(PAD + b * RB + r0, 16), :] + x1)

            def store(r0, y):
                yn[pl.ds(r0, 16), :] = y
                return y

            return _held(in_h, _abreast([
                _ln_tasks(lambda r0=r0: hbuf[rows_of(PAD + b * RB + r0, 16), :],
                          functools.partial(residual, r0)) for r0 in range(0, RB, 16)], RB // 16)
            ) + _held(in_y, _abreast([
                _ln_tasks(lambda r0=r0: yn[rows_of(r0, 16), :],
                          functools.partial(store, r0)) for r0 in range(0, RB, 16)], RB // 16)
                + a_operands(
                lambda r0, c: yn[rows_of(r0, 16), pl.ds(DH * c, DH)], ya))

        def ups(c):
            return products(ya, m1, C4 * c, pu[c])

        def mixer(raw, *bufs):
            sa, sp = bufs[:2], (bufs[2:4], bufs[4:])
            in_g = xg.at[0, pl.ds(S + 2 * HALO, 8)]
            w4_copies = [pltpu.make_async_copy(
                w4_hbm.bitcast(u32).at[pl.ds(c, n)], raw.at[pl.ds(c, n)], sems.at[SEM_B + s])
                for c, n, s in ((0, 2, 1), (2, NC - 2, 2))]
            _start(w4_copies)

            def pre(n, w, b):
                shift = lambda c: w * (-1, 1, -2, 2)[c >> 1]
                return _held(in_g, a_operands(lambda r0, c: xg[c + here, pl.ds(
                    HALO + b * RB + r0 + shift(c), 16), :], sa[n & 1]))

            def post(n, w, b):
                def task(g, j):
                    c, g = divmod(g, R // 8)
                    m = [sp[n & 1][c][p1 + here, j, pl.ds(8 * g, 8), :]
                         for p1 in range(7)]
                    for q in range(4):
                        i, k = _pos(q, j)
                        r0 = _mult(b * RB + i * R + 8 * g, 8)
                        v = _res(q, m.__getitem__)
                        if w == 0:
                            xg[2 * k + c, pl.ds(HALO + r0, 8), :] = _gelu2(v)
                        else:
                            x1b[pl.ds(r0, 8), pl.ds(DH * (2 * k + c), DH)] = 0.5 * v
                return [t for c in range(2) for t in _held(
                    sp[n & 1][c].at[7, 0, pl.ds(0, 8)],
                    _tasks(task, range(R // 8 * c, R // 8 * (c + 1)), range(4)))]

            def unit(n, w, *side):
                dots = [t for c in range(2) for t in products(
                    sa[n & 1], w12, C4 * (2 * w + c), sp[n & 1][c])]
                _overlap(dots, _merge(*side), MX_LAG)

            def w4_work(k, n, half=0):
                def task(i, p1):
                    g, c = half + (i >> 1), i & 1
                    r0 = _mult(8 * (g & 7), 8)
                    b_operands(lambda q, j: raw[(g >> 3) + here, q, pl.ds(r0, 8),
                                                pl.ds(DH * (2 * j + c), DH)],
                               w4t, _mult(DH * (g >> 3) + 64 * c + r0, 8), p1)
                return _held(raw.at[NC, 0, pl.ds(0, 8), pl.ds(0, DH)],
                             _tasks(task, range(k, k + n), range(7)))

            norms = lambda s: _held(in_h, _abreast(
                [mixer_norm(s * SEG + k * HS) for k in range(6)], 3))
            _overlap(wo_last(), _merge(pre(0, 0, 0), norms(NSEG - 6)), MX_LAG)
            unit(0, 0, pre(1, 0, 1), norms(NSEG - 3))
            _wait(w4_copies[:1])

            @pl.loop(0, 3)
            def _(i):
                pl.when(i == 2)(lambda: _wait(w4_copies[1:]))
                for n in range(2):
                    b = 2 * i + 1 + n
                    unit(n + 1, 0, pre(n, 0, b + 1), post(n, 0, b - 1),
                         w4_work(G1 * n, G1, G1 * i))

            unit(1, 0, pre(0, 1, 0), post(0, 0, 6), w4_work(6 * G1, G1))
            unit(0, 1, pre(1, 1, 1), post(1, 0, 7), w4_work(7 * G1, G1))

            @pl.loop(0, 2)
            def _(i):
                for n in range(2):
                    b = 2 * i + 1 + n
                    unit(n + 1, 1, pre(n, 1, b + 1), post(n, 1, b - 1),
                         w4_work(8 * G1 + G2 * n, G2, G2 * i))

            done = 8 * G1 + 4 * G2
            rest = w4_work(done, 16 * NC - done)
            ahead = mlp_in(0)
            for b in range(5, NB):
                unit(b, 1, pre(b + 1, 1, b + 1) if b + 1 < NB else _share(rest, 2, 4),
                     post(b - 1, 1, b - 1), _share(ahead, b - 5, 3),
                     _share(rest, (0, 1, 3)[b - 5], 4))
            for _, task in post(1, 1, NB - 1):
                task()

        def mlp(ta0, ta1, pd, ob):
            ta = [ta0.at[c] for c in range(NC - 1)] + [ta1]

            def mid(c, g, j):
                r = pl.ds(8 * g, 8)
                m = [pu[c][p1 + here, j, r, :] for p1 in range(7)]
                y = [_gelu2(_res(q, m.__getitem__)) for q in range(4)]
                for p1 in range(7):
                    v = _lhs(p1, y.__getitem__)
                    ta[c][p1, j, r, :] = v
                return v

            def down(b, m, p, c):
                p1, p0 = divmod(p, 7)
                lhs = _lhs(p0, lambda j: ta[c][p1 + here, j]).astype(bf16)
                tot = _dot(lhs, jnp.concatenate(
                    [_get(w4t, p, rows=(C4 * c + 128 * k, 128)) for k in range(2)],
                    axis=1))
                m[p] = m[p] + tot if c else tot
                if c == NC - 1 and p0 >= 3:
                    j = (2, 1, 3, 0)[p0 - 3]
                    v = _res(j, lambda k: m[7 * p1 + k])
                    if p1 < 6:
                        pd[p1, j] = v
                    if p1 >= 3:
                        q = (2, 1, 3, 0)[p1 - 3]
                        i, n = _pos(q, j)
                        r0, cols = _mult(b * RB + i * R, R), pl.ds(n * C4, C4)
                        v = _res(q, lambda k: v if k == p1 else pd[k + here, j])
                        ob[pl.ds(r0, R), cols] = (
                            _cols(*[xg[2 * n + k, pl.ds(r0, R), :] for k in range(2)]) + 0.5 * v).astype(bf16)
                return tot

            def out_copy(b):
                rows = pl.ds(_mult(b * RB, RB), RB)
                return pltpu.make_async_copy(ob.at[rows], out_hbm.at[rows],
                                             sems.at[SEM_OUT + b])

            @pl.loop(0, NB)
            def _(b):
                mids = lambda c: _held(pu[c].at[7, 0, pl.ds(0, 8)], _tasks(
                    functools.partial(mid, c), range(R // 8), range(4)))
                task = functools.partial(down, b, {})
                early = _tasks(task, range(EARLY), range(NC - 1))
                ahead = mlp_in(jnp.minimum(b + 1, NB - 1))
                _overlap(ups(0), ahead[:A0], 0)
                for c in range(NC):
                    _overlap(ups(c + 1) if c + 1 < NC else early,
                             _merge(mids(c), _share(ahead[A0:AH], c, NC - 1)), UP_LAG)

                _overlap(_tasks(task, range(EARLY), [NC - 1])
                         + _tasks(task, range(EARLY, 49), range(NC)),
                         ahead[AH:], DN_LAG)
                out_copy(b).start()

            for b in range(NB):
                out_copy(b).wait()

        pl.run_scoped(mixer, pltpu.VMEM((NC + 1, 4, 64, D), u32),
                      *[pltpu.VMEM((49, 2, R, DH), bf16)] * 2,
                      *[pltpu.VMEM((8, 4, R, DH), f32)] * 4)
        pl.run_scoped(mlp, pltpu.VMEM((NC - 1, 7, 4, R, DH), f32),
                      pltpu.VMEM((7, 4, R, DH), f32),
                      pltpu.VMEM((6, 4, R, C4), f32), pltpu.VMEM((S, D), bf16))

    pl.run_scoped(
        block_b,
        pltpu.VMEM((49, C4 * NC, DH), bf16),
        pltpu.VMEM((S, D), f32),
        pltpu.VMEM((RB + 8, D), f32),
        pltpu.VMEM((49, 2, R, DH), bf16),
        *[pltpu.VMEM((8, 4, R, 128), f32)] * 3)


@jax.jit
def pallas_sequential_preLN__memory_aug_recurrent_mem_tr__mixer_s_mlp__prompt_kernel(
    A_x: jax.Array,
    A_mem0: jax.Array,
    A_Wq: jax.Array,
    A_Wk: jax.Array,
    A_Wv: jax.Array,
    A_Wo: jax.Array,
    A_seg_len: jax.Array,
    B_x: jax.Array,
    B_w1: jax.Array,
    B_w2: jax.Array,
    B_w3: jax.Array,
    B_w4: jax.Array,
):
    del A_seg_len, B_x
    hbm = pl.BlockSpec(memory_space=pl.ANY)
    scratch = [
        pltpu.VMEM((PAD + S, D), f32),
        pltpu.VMEM((8, S + 3 * HALO, DH), f32),
        pltpu.VMEM((7, NP, 4, DH, DH), bf16),
        pltpu.VMEM((6, NP, HS, DH), bf16),
        pltpu.VMEM((7, 24, HD), f32),
        pltpu.VMEM((NP, 3 * HS, DH), f32),
        pltpu.VMEM((49, S, DH), bf16),
        pltpu.VMEM((49, D, DH), bf16),
        pltpu.SemaphoreType.DMA((NSEM,)),
    ]
    out = pl.pallas_call(
        _kernel,
        out_shape=jax.ShapeDtypeStruct((S, D), A_x.dtype),
        in_specs=[hbm] * 10,
        out_specs=hbm,
        scratch_shapes=scratch,
        compiler_params=pltpu.CompilerParams(vmem_limit_bytes=127 * 1024 * 1024),
    )(A_x.reshape(S, D), A_mem0.reshape(MEM, D),
      A_Wq.reshape(D // 2, 2 * H, DH), A_Wk.reshape(D // 2, 2 * H, DH),
      A_Wv.reshape(D // 2, 2 * H, DH),
      A_Wo.reshape(H * DH, D), B_w1.reshape(4, C4, D), B_w2.reshape(4, C4, D),
      B_w3.reshape(4, C4, F), B_w4.reshape(NC, 4, FC // 4, D))
    return out.reshape(A_x.shape)
```
